```python
import jax
import jax.numpy as jnp

def _softmax(x, axis=-1):
    return jax.nn.softmax(x, axis=axis)
def _gelu(x):
    return jax.nn.gelu(x, approximate=True)
def _silu(x):
    return jax.nn.silu(x)
def _sigmoid(x):
    return jax.nn.sigmoid(x)
def _layernorm(x, axis=-1, eps=1e-5):
    m = jnp.mean(x, axis=axis, keepdims=True)
    v = jnp.var(x, axis=axis, keepdims=True)
    return (x - m) / jnp.sqrt(v + eps)
def _scatter_add(tgt, idx, src, axis=0):
    return tgt.at[idx].add(src)
def _segment_sum(src, seg, n):
    return jax.ops.segment_sum(src, seg, n)
class _Rng:
    def __init__(self, key):
        self._k = key
    def _next(self):
        self._k, sub = jax.random.split(self._k)
        return sub
    def normal(self, shape):
        return jax.random.normal(self._next(), shape, dtype=jnp.bfloat16)
    def randint(self, lo, hi, shape):
        return jax.random.randint(self._next(), shape, lo, hi, dtype=jnp.int32)
    def uniform(self, shape, lo=0.0, hi=1.0):
        return jax.random.uniform(self._next(), shape, jnp.bfloat16, lo, hi)
    def permutation(self, n):
        return jax.random.permutation(self._next(), n)


kernel_name = 'standalone__layernorm_linear__sampling'

def setup_inputs():
    _rng = _Rng(jax.random.key(int.from_bytes(__import__("os").urandom(4), "little")))
    _w = (lambda a: (lambda t: t.astype(jnp.bfloat16) if jnp.issubdtype(t.dtype, jnp.floating) else t)(jnp.asarray(a)))
    B, S, D = 1024, 32, 576
    return {
        "x": _w((lambda *s: _rng.normal(s) * 0.05)(B, S, D)),
        "g": _w((lambda *s: _rng.normal(s) * 0.05)(D) + 1.0),
        "b": _w((lambda *s: _rng.normal(s) * 0.05)(D)),
        "w": _w((lambda *s: _rng.normal(s) * 0.05)(D, D)),
    }

def reference(x, g, b, w):
    return (_layernorm(x, axis=-1) * g + b) @ w
```

```python
import jax
import jax.numpy as jnp
from jax import lax
import jax.experimental.pallas as pl
import jax.experimental.pallas.tpu as pltpu

EPS = 1e-5
F32 = jnp.float32
BF16 = jnp.bfloat16
U32 = jnp.uint32

LANES = 128
AUG = 16
PLAN = ((1, 4), (4, 7))
SWITCH = 13
OUT_PIECE = 256


def _split_hi_lo(v):
    hi = v.astype(BF16).astype(F32)
    lo = (v - hi).astype(BF16).astype(F32)
    return hi, lo


def _prep_weights(g_ref, b_ref, w_ref, wa_ref, d_model):
    wt = w_ref[...].astype(F32).T
    g = g_ref[...].astype(F32).reshape(1, d_model)
    b = b_ref[...].astype(F32).reshape(1, d_model)
    wg = (wt * g).astype(BF16)
    c = jnp.sum(wg.astype(F32), axis=1, keepdims=True)
    d = jnp.sum(wt * b, axis=1, keepdims=True)
    c_hi, c_lo = _split_hi_lo(c)
    d_hi, d_lo = _split_hi_lo(d)
    lane = lax.broadcasted_iota(jnp.int32, (d_model, 64), 1)
    aug = jnp.where(lane < 2, -c_hi,
                    jnp.where(lane == 2, -c_lo,
                              jnp.where(lane < 5, d_hi,
                                        jnp.where(lane == 5, d_lo, 0.0))))
    full = jnp.concatenate([wg, aug.astype(BF16)], axis=1)
    wa_ref[...] = pltpu.bitcast(full, U32)


def _column_stats(x_ref, d_model):
    rows = 16
    x0 = x_ref[0:rows, :].astype(F32)[0:1, :]
    a1 = None
    a2 = None
    for i in range(d_model // rows):
        t = x_ref[i * rows:(i + 1) * rows, :].astype(F32) - x0
        for r in range(rows // 8):
            tt = t[r * 8:(r + 1) * 8]
            a1 = tt if a1 is None else a1 + tt
            a2 = tt * tt if a2 is None else a2 + tt * tt
    s1 = jnp.sum(a1, axis=0, keepdims=True) * (1.0 / d_model)
    s2 = jnp.sum(a2, axis=0, keepdims=True) * (1.0 / d_model)
    mean = x0 + s1
    var = jnp.maximum(s2 - s1 * s1, 0.0)
    ve = var + EPS
    rstd = lax.rsqrt(ve)
    std = ve * rstd
    return mean, rstd, std


def _aug_rows(mean, std):
    m_hi, m_lo = _split_hi_lo(mean)
    s_hi, s_lo = _split_hi_lo(std)
    row = lax.broadcasted_iota(jnp.int32, (AUG, LANES), 0)
    return jnp.where((row == 0) | (row == 2), m_hi,
                     jnp.where(row == 1, m_lo,
                               jnp.where((row == 3) | (row == 5), s_hi,
                                         jnp.where(row == 4, s_lo, 0.0)))).astype(BF16)


@jax.jit
def pallas_standalone__layernorm_linear__sampling_kernel(
    x: jax.Array,
    g: jax.Array,
    b: jax.Array,
    w: jax.Array,
):
    B, S, D = x.shape
    assert sum(u * n for u, n in PLAN) == S
    xt = jnp.transpose(x, (1, 2, 0))

    def kernel(x_hbm, g_hbm, b_hbm, w_hbm, o_hbm,
               xbuf, obuf, wbuf, gbuf, bbuf, wa_ref, isem, osem, wsem):
        def in_copy(s):
            return pltpu.make_async_copy(x_hbm.at[s], xbuf.at[s], isem.at[s])

        def out_piece(s, p):
            cols = pl.ds(p * OUT_PIECE, OUT_PIECE)
            return pltpu.make_async_copy(obuf.at[s, :, cols], o_hbm.at[s, :, cols], osem.at[0])

        cg = pltpu.make_async_copy(g_hbm, gbuf, wsem.at[1])
        cb = pltpu.make_async_copy(b_hbm, bbuf, wsem.at[2])
        cw = pltpu.make_async_copy(w_hbm, wbuf, wsem.at[0])
        cg.start()
        cb.start()
        cw.start()
        cg.wait()
        cb.wait()
        for s in range(S):
            in_copy(s).start()
        cw.wait()
        _prep_weights(gbuf, bbuf, wbuf, wa_ref, D)

        def do_slice(s):
            @pl.when(s == SWITCH)
            def _():
                pltpu.make_async_copy(obuf.at[pl.ds(0, SWITCH)],
                                      o_hbm.at[pl.ds(0, SWITCH)], osem.at[0]).start()

            for c0 in range(0, B, LANES):
                mean, rstd, std = _column_stats(xbuf.at[s, :, pl.ds(c0, LANES)], D)
                xa = jnp.concatenate([xbuf[s, :, c0:c0 + LANES], _aug_rows(mean, std)], axis=0)
                wfull = pltpu.bitcast(wa_ref[...], BF16)[:, 0:D + AUG]
                acc = jnp.dot(wfull, xa, preferred_element_type=F32)
                obuf[s, :, c0:c0 + LANES] = (acc * rstd).astype(BF16)
                if (c0 + LANES) % OUT_PIECE == 0:
                    @pl.when(s >= SWITCH)
                    def _():
                        out_piece(s, c0 // OUT_PIECE).start()

        base = 0
        for unroll, count in PLAN:
            def body(it, carry, unroll=unroll, base=base):
                s0 = base + it * unroll
                for u in range(unroll):
                    in_copy(s0 + u).wait()
                for u in range(unroll):
                    do_slice(s0 + u)
                return carry
            lax.fori_loop(0, count, body, 0)
            base += unroll * count
        pltpu.make_async_copy(obuf, o_hbm, osem.at[0]).wait()

    out = pl.pallas_call(
        kernel,
        in_specs=[pl.BlockSpec(memory_space=pl.ANY)] * 4,
        out_specs=pl.BlockSpec(memory_space=pl.ANY),
        out_shape=jax.ShapeDtypeStruct((S, D, B), x.dtype),
        scratch_shapes=[
            pltpu.VMEM((S, D, B), BF16),
            pltpu.VMEM((S, D, B), BF16),
            pltpu.VMEM((D, D), BF16),
            pltpu.VMEM((D,), BF16),
            pltpu.VMEM((D,), BF16),
            pltpu.VMEM((D // 2, D + 64), U32),
            pltpu.SemaphoreType.DMA((S,)),
            pltpu.SemaphoreType.DMA((1,)),
            pltpu.SemaphoreType.DMA((3,)),
        ],
        compiler_params=pltpu.CompilerParams(
            vmem_limit_bytes=110 * 1024 * 1024,
            disable_bounds_checks=True,
        ),
    )(xt, g, b, w)
    return jnp.transpose(out, (2, 0, 1))
```

```python
import functools

import jax
import jax.numpy as jnp
from jax import lax
import jax.experimental.pallas as pl
import jax.experimental.pallas.tpu as pltpu

EPS = 1e-5
F32 = jnp.float32
BF16 = jnp.bfloat16
U32 = jnp.uint32

L = 128
H = 288
KH = 256
KM = 2 * KH
KT = 80
UNIT = 512
PLAN = ((1, 1), (2, 1), (5, 1), (8, 7))
SWITCH = 14
ORDER = ("M2", "T21", "M4", "M3", "T12", "M5", "M1", "M6t", "M7t")
USES = {
    "M1": (("11", 1), ("22", 1)), "M2": (("21", 1), ("22", -1)),
    "M3": (("12", 1), ("22", 1)), "M4": (("11", 1), ("21", 1)),
    "M5": (("11", -1), ("12", 1)), "M6t": (("22", 1),), "M7t": (("11", 1),),
    "T12": (("12", 1),), "T21": (("21", 1),),
}
TERMS = {"11": 4, "12": 3, "21": 3, "22": 4}


def _prep_weights(g_ref, b_ref, w_ref, a_ref, t_ref, d_model):
    rows, cols = 32, L
    w = w_ref[...]
    g = g_ref[...].astype(F32).reshape(1, d_model)
    wt = w[0:KM].T
    for i in range(H // rows):
        for c in range(0, KH, cols):
            def blk(hh, kk):
                k0 = kk * KH + c
                r0 = hh * H + i * rows
                return wt[r0:r0 + rows, k0:k0 + cols].astype(F32) * g[:, k0:k0 + cols]
            a11, a12, a21, a22 = blk(0, 0), blk(0, 1), blk(1, 0), blk(1, 1)
            xs = (a11 + a22, a21 + a22, a11, a22, a11 + a12, a21 - a11, a12 - a22)
            for k in range(7):
                a_ref[k, i * rows // 2:(i + 1) * rows // 2, c:c + cols] = (
                    pltpu.bitcast(xs[k].astype(BF16), U32))
    brow = jnp.broadcast_to(b_ref[...].astype(F32).reshape(1, d_model), (16, d_model))
    drow = jnp.dot(brow.astype(BF16), w, preferred_element_type=F32)
    row = lax.broadcasted_iota(jnp.int32, (16, d_model), 0)
    lo = drow - drow.astype(BF16).astype(F32)
    e = jnp.where(row == 0, drow, jnp.where(row == 1, lo, 0.0))
    e = jnp.concatenate([e, jnp.zeros((48, d_model), F32)], axis=0).astype(BF16)
    wtail = jnp.concatenate([w[KM:d_model], e], axis=0)
    gt = jnp.concatenate([g[:, KM:d_model], jnp.ones((1, 64), F32)], axis=1)
    at = pltpu.bitcast((wtail.T.astype(F32) * gt).astype(BF16), U32)
    t_ref[0] = at[0:H // 2]
    t_ref[1] = at[H // 2:]


def _column_stats(x_ref, d_model, chains):
    rows = 16
    x0 = x_ref[0:rows, :].astype(F32)[0:1, :]
    a1 = [None] * chains
    a2 = [None] * chains
    n = 0
    for i in range(d_model // rows):
        t = x_ref[i * rows:(i + 1) * rows, :].astype(F32) - x0
        for r in range(rows // 8):
            tt = t[r * 8:(r + 1) * 8]
            c = n % chains
            n += 1
            a1[c] = tt if a1[c] is None else a1[c] + tt
            a2[c] = tt * tt if a2[c] is None else a2[c] + tt * tt
    a1 = functools.reduce(lambda u, v: u + v, a1)
    a2 = functools.reduce(lambda u, v: u + v, a2)
    s1 = jnp.sum(a1, axis=0, keepdims=True) * (1.0 / d_model)
    s2 = jnp.sum(a2, axis=0, keepdims=True) * (1.0 / d_model)
    mean = x0 + s1
    var = jnp.maximum(s2 - s1 * s1, 0.0)
    return mean, lax.rsqrt(var + EPS)


def _pair(xs_ref, os_ref, a_ref, t_ref, c0, d_model, first):
    cc = (c0, c0 + L)
    cache = {}

    def x(k, j):
        return xs_ref[k * KH:(k + 1) * KH, cc[j]:cc[j] + L].astype(F32)

    def lhs(i):
        return pltpu.bitcast(a_ref[i - 1], BF16)

    def lhs_tail(h):
        return pltpu.bitcast(t_ref[h - 1], BF16)

    def stats(j):
        if j not in cache:
            chains = 2 if (first and j == 0) else 1
            cache[j] = _column_stats(xs_ref.at[:, pl.ds(cc[j], L)], d_model, chains)
        return cache[j]

    def rhs_tail(j):
        if ("t", j) not in cache:
            m, r = stats(j)
            row = lax.broadcasted_iota(jnp.int32, (16, L), 0)
            ones = jnp.where(row < 2, 1.0, 0.0)
            xt = xs_ref[KM:d_model, cc[j]:cc[j] + L].astype(F32)
            cache["t", j] = jnp.concatenate([(xt - m) * r, ones], axis=0)
        return cache["t", j]

    def cross(ka, kb):
        (m1, r1), (m2, r2) = stats(0), stats(1)
        if "mr" not in cache:
            cache["mr"] = m1 * r1 + m2 * r2
        return x(ka, 0) * r1 + x(kb, 1) * r2 - cache["mr"]

    def rhs(i):
        if i == 1:
            return cross(0, 1)
        if i == 2:
            return (x(0, 0) - stats(0)[0]) * stats(0)[1]
        if i == 3:
            return (x(0, 1) - x(1, 1)) * stats(1)[1]
        if i == 4:
            return (x(1, 0) - x(0, 0)) * stats(0)[1]
        if i == 5:
            return (x(1, 1) - stats(1)[0]) * stats(1)[1]
        if i == 6:
            return cross(0, 0)
        return cross(1, 1)

    def dot(p, q):
        return jnp.dot(p, q.astype(BF16), preferred_element_type=F32)

    acc = {}
    count = dict.fromkeys(TERMS, 0)
    for name in ORDER:
        if name[0] == "T":
            v = dot(lhs_tail(int(name[1]))[:, 0:KT], rhs_tail(int(name[2]) - 1))
        elif name.endswith("t"):
            i = int(name[1])
            h, j = (2, 1) if i == 6 else (1, 0)
            v = dot(jnp.concatenate([lhs(i), lhs_tail(h)], axis=1)[:, 0:KH + KT],
                    jnp.concatenate([rhs(i), rhs_tail(j)], axis=0))
        else:
            i = int(name[1])
            v = dot(lhs(i), rhs(i))
        for key, sign in USES[name]:
            if key not in acc:
                acc[key] = (v, sign)
            else:
                cur, cur_sign = acc[key]
                if cur_sign == 1:
                    acc[key] = (cur + v if sign == 1 else cur - v, 1)
                else:
                    acc[key] = (v - cur, 1) if sign == 1 else (cur + v, -1)
            count[key] += 1
            if count[key] == TERMS[key]:
                val, val_sign = acc[key]
                assert val_sign == 1
                r0 = 0 if key[0] == "1" else H
                col = cc[int(key[1]) - 1]
                os_ref[r0:r0 + H, col:col + L] = val.astype(BF16)


def _when(cond, fn):
    if isinstance(cond, bool):
        if cond:
            fn()
    else:
        pl.when(cond)(fn)


@jax.jit
def pallas_standalone__layernorm_linear__sampling_kernel(
    x: jax.Array,
    g: jax.Array,
    b: jax.Array,
    w: jax.Array,
):
    B, S, D = x.shape
    assert D == 2 * H == KM + 64
    ups = B // UNIT
    assert sum(u * n for u, n in PLAN) == S * ups
    n_chunks = sum(n for _, n in PLAN)
    xt = jnp.transpose(x, (1, 2, 0))

    def kernel(x_hbm, g_hbm, b_hbm, w_hbm, o_hbm,
               xbuf, obuf, wbuf, gbuf, bbuf, a_ref, t_ref, isem, osem, wsem):
        def chunk_copies(j, u0, nu, shift):
            res = []
            u, end = u0, u0 + nu
            while u < end:
                s, r = divmod(u, ups)
                if r == 0 and end - u >= ups:
                    ns = (end - u) // ups
                    sl = pl.ds(s + shift, ns)
                    res.append(pltpu.make_async_copy(x_hbm.at[sl], xbuf.at[sl], isem.at[j]))
                    u += ns * ups
                else:
                    k = min(ups - r, end - u)
                    cols = pl.ds(r * UNIT, k * UNIT)
                    res.append(pltpu.make_async_copy(
                        x_hbm.at[s + shift, :, cols], xbuf.at[s + shift, :, cols], isem.at[j]))
                    u += k
            return res

        cg = pltpu.make_async_copy(g_hbm, gbuf, wsem.at[1])
        cb = pltpu.make_async_copy(b_hbm, bbuf, wsem.at[2])
        cw = pltpu.make_async_copy(w_hbm, wbuf, wsem.at[0])
        cg.start()
        cb.start()
        cw.start()
        cg.wait()
        cb.wait()
        j = u0 = 0
        for nu, count in PLAN:
            for _ in range(count):
                for c in chunk_copies(j, u0, nu, 0):
                    c.start()
                j += 1
                u0 += nu
        cw.wait()
        _prep_weights(gbuf, bbuf, wbuf, a_ref, t_ref, D)

        def do_chunk(j, u0, nu, shift):
            for c in chunk_copies(j, u0, nu, shift):
                c.wait()
            first = True
            for u in range(u0, u0 + nu):
                s = u // ups + shift
                for c0 in range((u % ups) * UNIT, (u % ups + 1) * UNIT, 2 * L):
                    if c0 == 0:
                        _when(s == SWITCH, lambda: pltpu.make_async_copy(
                            obuf.at[pl.ds(0, SWITCH)], o_hbm.at[pl.ds(0, SWITCH)],
                            osem.at[0]).start())
                    _pair(xbuf.at[s], obuf.at[s], a_ref, t_ref, c0, D, first)
                    first = False
                    cols = pl.ds(c0, 2 * L)
                    _when(s >= SWITCH, lambda: pltpu.make_async_copy(
                        obuf.at[s, :, cols], o_hbm.at[s, :, cols], osem.at[0]).start())

        j = u0 = 0
        for nu, count in PLAN:
            if count == 1:
                do_chunk(j, u0, nu, 0)
            else:
                assert nu % ups == 0 and u0 % ups == 0

                def body(it, carry, j=j, u0=u0, nu=nu):
                    do_chunk(j + it, u0, nu, it * (nu // ups))
                    return carry
                lax.fori_loop(0, count, body, 0)
            j += count
            u0 += nu * count
        pltpu.make_async_copy(obuf, o_hbm, osem.at[0]).wait()

    out = pl.pallas_call(
        kernel,
        in_specs=[pl.BlockSpec(memory_space=pl.ANY)] * 4,
        out_specs=pl.BlockSpec(memory_space=pl.ANY),
        out_shape=jax.ShapeDtypeStruct((S, D, B), x.dtype),
        scratch_shapes=[
            pltpu.VMEM((S, D, B), BF16),
            pltpu.VMEM((S, D, B), BF16),
            pltpu.VMEM((D, D), BF16),
            pltpu.VMEM((D,), BF16),
            pltpu.VMEM((D,), BF16),
            pltpu.VMEM((7, H // 2, KH), U32),
            pltpu.VMEM((2, H // 2, L), U32),
            pltpu.SemaphoreType.DMA((n_chunks,)),
            pltpu.SemaphoreType.DMA((1,)),
            pltpu.SemaphoreType.DMA((3,)),
        ],
        compiler_params=pltpu.CompilerParams(
            vmem_limit_bytes=110 * 1024 * 1024,
            disable_bounds_checks=True,
            disable_semaphore_checks=True,
        ),
    )(xt, g, b, w)
    return jnp.transpose(out, (2, 0, 1))
```

```python
import functools

import jax
import jax.numpy as jnp
from jax import lax
import jax.experimental.pallas as pl
import jax.experimental.pallas.tpu as pltpu

EPS = 1e-5
F32 = jnp.float32
BF16 = jnp.bfloat16
U32 = jnp.uint32

L = 128
H = 288
KH = 256
KS = 192
KM = 2 * KH
UNIT = 512
PLAN = ((1, 1), (2, 1), (5, 1), (8, 7))
SWITCH = 15
BULK_ROWS = 24

TILES = ("S1a", "S1b", "S2a", "S2b", "S3a", "S3b", "S4a", "S4b", "S5a", "S5b",
         "S6a", "S6b", "S7a", "S7b", "R1", "R6", "R7")
USES = {
    "S1": (("11", 1), ("22", 1)), "S2": (("21", 1), ("22", -1)),
    "S3": (("12", 1), ("22", 1)), "S4": (("11", 1), ("21", 1)),
    "S5": (("11", -1), ("12", 1)), "S6": (("22", 1),), "S7": (("11", 1),),
    "R1": (("12", 1), ("21", 1)), "R6": (("12", 1),), "R7": (("21", 1),),
    "D": (("21", 1), ("22", 1)),
}
TERMS = {"11": 4, "12": 4, "21": 5, "22": 5}
ORDER = ("S4a", "S4b", "S2a", "S3a", "S3b", "S5a", "D", "S2b", "R7", "S5b+a",
         "R1", "R6", "S1a", "S1b", "S7a+b", "S7b", "S6a", "S6b")


def _prep_weights(g_ref, b_ref, w_ref, tile_refs, dl_ref, d_model):
    rows = 32
    ref = dict(zip(TILES, tile_refs))
    w = w_ref[...]
    g = g_ref[...].astype(F32).reshape(1, d_model)
    wt = w[0:KM].T
    gt = jnp.concatenate([g[:, KM:d_model]] * 2, axis=1)
    at = jnp.concatenate([w[KM:d_model]] * 2, axis=0).T
    brow = jnp.broadcast_to(b_ref[...].astype(F32).reshape(1, d_model), (16, d_model))
    drow = jnp.dot(brow.astype(BF16), w, preferred_element_type=F32)
    row = lax.broadcasted_iota(jnp.int32, (16, d_model), 0)
    lo = drow - drow.astype(BF16).astype(F32)
    e = jnp.where(row == 0, drow, jnp.where(row == 1, lo, 0.0))
    z = jnp.zeros((48, d_model), F32)
    et = jnp.concatenate([e, z, e, z], axis=0).astype(BF16).T

    low = lax.broadcasted_iota(jnp.int32, (rows, L), 1) < 64

    def sel(p, q):
        return jnp.where(low, p, q)

    for i in range(H // rows):
        r0 = i * rows

        def put(name, v):
            ref[name][r0 // 2:(r0 + rows) // 2, :] = pltpu.bitcast(v.astype(BF16), U32)

        def blocks(c):
            return [wt[h * H + r0:h * H + r0 + rows, k * KH + c:k * KH + c + L].astype(F32)
                    * g[:, k * KH + c:k * KH + c + L] for h in range(2) for k in range(2)]

        a11, a12, a21, a22 = blocks(0)
        xs = (a11 + a22, a21 + a22, a11, a22, a11 + a12, a21 - a11, a12 - a22)
        for k in range(7):
            put("S%da" % (k + 1), xs[k])
        a11, a12, a21, a22 = blocks(L)
        at1 = at[r0:r0 + rows].astype(F32) * gt
        at2 = at[H + r0:H + r0 + rows].astype(F32) * gt
        e1 = et[r0:r0 + rows].astype(F32)
        s2, s5, s6, s7 = a21 + a22, a11 + a12, a21 - a11, a12 - a22
        xs = (sel(a11 + a22, e1), sel(s2, -s2), sel(a11, a21), sel(a22, a12),
              sel(s5, -s5), sel(s6, at2), sel(s7, at1))
        for k in range(7):
            put("S%db" % (k + 1), xs[k])
        put("R1", sel(e1, a21 + a12))
        put("R6", sel(at1, -s6))
        put("R7", sel(at2, -s7))
    low2 = lax.broadcasted_iota(jnp.int32, (H, L), 1) < 64
    lhs = jnp.where(low2, et[H:d_model].astype(F32), -et[0:H].astype(F32)).astype(BF16)
    dl_ref[...] = jnp.dot(lhs, jnp.ones((L, L), BF16), preferred_element_type=F32)


def _column_stats(x_ref, d_model, chains):
    rows = 16
    x0 = x_ref[0:rows, :].astype(F32)[0:1, :]
    a1 = [None] * chains
    a2 = [None] * chains
    n = 0
    for i in range(d_model // rows):
        t = x_ref[i * rows:(i + 1) * rows, :].astype(F32) - x0
        for r in range(rows // 8):
            tt = t[r * 8:(r + 1) * 8]
            c = n % chains
            n += 1
            a1[c] = tt if a1[c] is None else a1[c] + tt
            a2[c] = tt * tt if a2[c] is None else a2[c] + tt * tt
    a1 = functools.reduce(lambda u, v: u + v, a1)
    a2 = functools.reduce(lambda u, v: u + v, a2)
    s1 = jnp.sum(a1, axis=0, keepdims=True) * (1.0 / d_model)
    s2 = jnp.sum(a2, axis=0, keepdims=True) * (1.0 / d_model)
    mean = x0 + s1
    var = jnp.maximum(s2 - s1 * s1, 0.0)
    return mean, lax.rsqrt(var + EPS)


class _Pair:
    def __init__(self, xs_ref, os_ref, tile_refs, dl_ref, c0, d_model, first):
        self.xs_ref, self.os_ref, self.dl_ref = xs_ref, os_ref, dl_ref
        self.lhs = dict(zip(TILES, tile_refs))
        self.cc = (c0, c0 + L)
        self.d_model = d_model
        self.first = first
        self.cache = {}

    def stats(self, j):
        if j not in self.cache:
            chains = 2 if (self.first and j == 0) else 1
            self.cache[j] = _column_stats(
                self.xs_ref.at[:, pl.ds(self.cc[j], L)], self.d_model, chains)
        return self.cache[j]

    def x(self, k, j, r0, r1):
        return self.xs_ref[k * KH + r0:k * KH + r1, self.cc[j]:self.cc[j] + L].astype(F32)

    def rhs(self, name, dep):
        def late(v):
            return v if dep is None else v + dep

        def hat(k, j, r0, r1):
            m, r = self.stats(j)
            return (self.x(k, j, r0, r1) - late(m)) * r

        def tail(j):
            if ("t", j) not in self.cache:
                self.cache["t", j] = hat(2, j, 0, 64)
            return self.cache["t", j]

        def cross(ka, kb, r0, r1):
            (m1, ra), (m2, rb) = self.stats(0), self.stats(1)
            if "mr" not in self.cache:
                self.cache["mr"] = m1 * ra + m2 * rb
            return (self.x(ka, 0, r0, r1) * ra + self.x(kb, 1, r0, r1) * rb
                    - late(self.cache["mr"]))

        def ones():
            row = lax.broadcasted_iota(jnp.int32, (16, L), 0)
            return jnp.where(row < 2, 1.0, 0.0)

        def cat(*parts):
            return jnp.concatenate(parts, axis=0)

        if name == "R1":
            return cat(ones(), jnp.zeros((48, L), F32), cross(0, 1, KS, KH))
        if name == "R6":
            return cat(tail(1), cross(0, 0, KS, KH))
        if name == "R7":
            return cat(tail(0), cross(1, 1, KS, KH))
        prod, r0 = name[:2], (0 if name[2] == "a" else L)
        if prod in ("S3", "S4"):
            j = 1 if prod == "S3" else 0
            diff = self.x(1 - j, j, r0, r0 + L) - self.x(j, j, r0, r0 + L)
            if self.first and j == 1:
                return diff + self.stats(0)[1] * 0.0 if r0 == 0 else diff
            return diff * self.stats(j)[1]
        main = {"S1": lambda a, b: cross(0, 1, a, b), "S2": lambda a, b: hat(0, 0, a, b),
                "S5": lambda a, b: hat(1, 1, a, b), "S6": lambda a, b: cross(0, 0, a, b),
                "S7": lambda a, b: cross(1, 1, a, b)}[prod]
        if r0 == 0:
            return main(0, L)
        rest = {"S1": ones, "S2": lambda: hat(1, 1, KS, KH), "S5": lambda: hat(0, 0, KS, KH),
                "S6": lambda: tail(1), "S7": lambda: tail(0)}[prod]
        return cat(main(L, KS), rest())

    def run(self, nxt):
        acc = {}
        count = dict.fromkeys(TERMS, 0)
        part = {}

        def add(name, v):
            for key, sign in USES[name]:
                if key not in acc:
                    acc[key] = (v, sign)
                else:
                    cur, cur_sign = acc[key]
                    if cur_sign == 1:
                        acc[key] = (cur + v if sign == 1 else cur - v, 1)
                    else:
                        acc[key] = (v - cur, 1) if sign == 1 else (cur + v, -1)
                count[key] += 1
                if count[key] == TERMS[key]:
                    val, val_sign = acc[key]
                    assert val_sign == 1
                    r0 = 0 if key[0] == "1" else H
                    col = self.cc[int(key[1]) - 1]
                    self.os_ref[r0:r0 + H, col:col + L] = val.astype(BF16)

        held = None
        for token in ORDER:
            name, _, wait_for = token.partition("+")
            if name == "D":
                if held is not None:
                    add("S3", held * self.stats(1)[1])
                add("D", self.dl_ref[...])
                continue
            dep = None
            if wait_for and nxt is not None:
                dep = nxt.stats("ab".index(wait_for))[1] * 0.0
            q = self.rhs(name, dep)
            p = pltpu.bitcast(self.lhs[name][...], BF16)[:, 0:q.shape[0]]
            v = jnp.dot(p, q.astype(BF16), preferred_element_type=F32)
            prod = name[:2]
            if prod[0] == "R":
                add(prod, v)
            elif prod not in part:
                part[prod] = v
            elif self.first and prod == "S3":
                held = v + part.pop(prod)
            else:
                add(prod, v + part.pop(prod))
        assert count == TERMS


def _when(cond, fn):
    if isinstance(cond, bool):
        if cond:
            fn()
    else:
        pl.when(cond)(fn)


@jax.jit
def pallas_standalone__layernorm_linear__sampling_kernel(
    x: jax.Array,
    g: jax.Array,
    b: jax.Array,
    w: jax.Array,
):
    B, S, D = x.shape
    assert D == 2 * H == KM + 64
    ups = B // UNIT
    assert sum(u * n for u, n in PLAN) == S * ups
    n_chunks = sum(n for _, n in PLAN)
    bulk_per_pair = D // BULK_ROWS // (B // (2 * L))
    xt = jnp.transpose(x, (1, 2, 0))

    def kernel(x_hbm, g_hbm, b_hbm, w_hbm, o_hbm, xbuf, obuf, wbuf, gbuf, bbuf, *rest):
        tile_refs = rest[:len(TILES)]
        dl_ref, isem, osem, wsem = rest[len(TILES):]

        def chunk_copies(j, u0, nu, shift):
            res = []
            u, end = u0, u0 + nu
            while u < end:
                s, r = divmod(u, ups)
                if r == 0 and end - u >= ups:
                    ns = (end - u) // ups
                    sl = pl.ds(s + shift, ns)
                    res.append(pltpu.make_async_copy(x_hbm.at[sl], xbuf.at[sl], isem.at[j]))
                    u += ns * ups
                else:
                    k = min(ups - r, end - u)
                    cols = pl.ds(r * UNIT, k * UNIT)
                    res.append(pltpu.make_async_copy(
                        x_hbm.at[s + shift, :, cols], xbuf.at[s + shift, :, cols], isem.at[j]))
                    u += k
            return res

        def write_back(*idx):
            pltpu.make_async_copy(obuf.at[idx], o_hbm.at[idx], osem.at[0]).start()

        cg = pltpu.make_async_copy(g_hbm, gbuf, wsem.at[1])
        cb = pltpu.make_async_copy(b_hbm, bbuf, wsem.at[2])
        cw = pltpu.make_async_copy(w_hbm, wbuf, wsem.at[0])
        cg.start()
        cb.start()
        cw.start()
        cg.wait()
        cb.wait()
        j = u0 = 0
        for nu, count in PLAN:
            for _ in range(count):
                for c in chunk_copies(j, u0, nu, 0):
                    c.start()
                j += 1
                u0 += nu
        cw.wait()
        _prep_weights(gbuf, bbuf, wbuf, tile_refs, dl_ref, D)

        def do_chunk(j, u0, nu, shift):
            for c in chunk_copies(j, u0, nu, shift):
                c.wait()
            where = [(u // ups + shift, c0) for u in range(u0, u0 + nu)
                     for c0 in range((u % ups) * UNIT, (u % ups + 1) * UNIT, 2 * L)]
            pairs = [_Pair(xbuf.at[s], obuf.at[s], tile_refs, dl_ref, c0, D, p == 0)
                     for p, (s, c0) in enumerate(where)]
            for p, (s, c0) in enumerate(where):
                r0 = c0 // (2 * L) * bulk_per_pair * BULK_ROWS
                for r in range(r0, r0 + bulk_per_pair * BULK_ROWS, BULK_ROWS):
                    _when(s == SWITCH, functools.partial(
                        write_back, pl.ds(0, SWITCH), pl.ds(r, BULK_ROWS)))
                pairs[p].run(pairs[p + 1] if p + 1 < len(pairs) else None)

                def both_tiles(s=s, c0=c0):
                    write_back(s, slice(None), pl.ds(c0, L))
                    write_back(s, slice(None), pl.ds(c0 + L, L))
                _when(s >= SWITCH, both_tiles)

        j = u0 = 0
        for nu, count in PLAN:
            if count == 1:
                do_chunk(j, u0, nu, 0)
            else:
                assert nu % ups == 0 and u0 % ups == 0

                def body(it, carry, j=j, u0=u0, nu=nu):
                    do_chunk(j + it, u0, nu, it * (nu // ups))
                    return carry
                lax.fori_loop(0, count, body, 0)
            j += count
            u0 += nu * count
        pltpu.make_async_copy(obuf, o_hbm, osem.at[0]).wait()

    out = pl.pallas_call(
        kernel,
        in_specs=[pl.BlockSpec(memory_space=pl.ANY)] * 4,
        out_specs=pl.BlockSpec(memory_space=pl.ANY),
        out_shape=jax.ShapeDtypeStruct((S, D, B), x.dtype),
        scratch_shapes=[
            pltpu.VMEM((S, D, B), BF16),
            pltpu.VMEM((S, D, B), BF16),
            pltpu.VMEM((D, D), BF16),
            pltpu.VMEM((D,), BF16),
            pltpu.VMEM((D,), BF16),
            *[pltpu.VMEM((H // 2, L), U32)] * len(TILES),
            pltpu.VMEM((H, L), F32),
            pltpu.SemaphoreType.DMA((n_chunks,)),
            pltpu.SemaphoreType.DMA((1,)),
            pltpu.SemaphoreType.DMA((3,)),
        ],
        compiler_params=pltpu.CompilerParams(
            vmem_limit_bytes=110 * 1024 * 1024,
            disable_bounds_checks=True,
            disable_semaphore_checks=True,
        ),
    )(xt, g, b, w)
    return jnp.transpose(out, (2, 0, 1))
```

```python
import functools

import jax
import jax.numpy as jnp
from jax import lax
import jax.experimental.pallas as pl
import jax.experimental.pallas.tpu as pltpu

EPS = 1e-5
F32 = jnp.float32
BF16 = jnp.bfloat16
U32 = jnp.uint32

L = 128
H = 288
Q = 144
KH = 256
KS = 192
KM = 2 * KH
UNIT = 512
STEPS = 72

LONG = tuple("S%d%s" % (i, h) for i in range(1, 8) for h in "ab") + ("R1", "R6", "R7")
LEVEL2 = ("S2", "S3", "S4", "S5")
SHORT = tuple("%sm%d" % (p, k) for p in LEVEL2 for k in range(1, 8))
USES = {
    "S1": (("11", 1), ("22", 1)), "S2": (("21", 1), ("22", -1)),
    "S3": (("12", 1), ("22", 1)), "S4": (("11", 1), ("21", 1)),
    "S5": (("11", -1), ("12", 1)), "S6": (("22", 1),), "S7": (("11", 1),),
    "R1": (("12", 1), ("21", 1)), "R6": (("12", 1),), "R7": (("21", 1),),
    "D": (("21", 1), ("22", 1)),
}
TERMS = {"11": 4, "12": 4, "21": 5, "22": 5}
USES2 = {1: ((0, 0, 1), (1, 1, 1)), 2: ((1, 0, 1), (1, 1, -1)), 3: ((0, 1, 1), (1, 1, 1)),
         4: ((0, 0, 1), (1, 0, 1)), 5: ((0, 0, -1), (0, 1, 1)), 6: ((1, 1, 1),),
         7: ((0, 0, 1),)}
TERMS2 = {(0, 0): 4, (0, 1): 2, (1, 0): 2, (1, 1): 4}
TILE_ORDER = ((0, 0), (1, 0), (0, 1), (1, 1))

_ROWS = ("S4m1 S4m7 S4m6 S4m2", "S4m4 S4m3 S4m5 S2m1", "S2m6 S2m2 S2m4 S2m3",
         "S2m5 S2m7 S3m4 S3m2", "S3m5 S3m3 S3m1 S3m6", "S3m7 S5m1 S5m7 S5m6",
         "A:D B:D A:R7 B:R7 S5m2 S5m4", "S5m3 S5m5", "A:S1a A:S1b B:S1a B:S1b",
         "A:R1 B:R1 A:R6 B:R6", "A:S7a A:S7b B:S7a B:S7b", "A:S6a A:S6b B:S6a B:S6b")
_ROWS_COLD = ("A:S4a A:S4b A:S2a A:Q3a", "A:P3b A:S5a A:V3 A:D A:S2b A:R7",
              "A:S5b A:R1 A:R6 A:S1a", "A:S1b A:S7a A:S7b A:S6a", "A:S6b B:S4a B:S4b B:S2a",
              "B:S3a B:S3b B:S5a B:D B:S2b", "B:R7 B:S5b B:R1 B:R6",
              "B:S1a B:S1b B:S7a B:S7b", "B:S6a B:S6b")
_ROWS_COLD0 = ("A:S4a A:S4b A:Q3a A:Q3b", "A:V3 A:D A:R7 A:R1 B:S4a B:S4b",
               "A:R6 A:S1a A:S1b B:P3a", "B:P3b A:S7a A:S7b A:S6a",
               "A:S6b B:V3 B:D B:R7 B:R1 B:R6", "S2m2 S2m4 S2m3 S2m5", "S2m6 S2m1 S2m7 S5m1",
               "S5m7 S5m6 S5m2 S5m4", "B:S1a B:S1b S5m3 S5m5", "B:S7a B:S7b B:S6a B:S6b")


def _schedule(rows, weights):
    out = []
    for row, steps in zip(rows, weights, strict=True):
        toks = row.split()
        passes = [t for t in toks if not (t.endswith(":D") or ":V" in t)]
        for t in toks:
            n = 0
            if t in passes:
                k = passes.index(t)
                n = steps * (k + 1) // len(passes) - steps * k // len(passes)
            out.append((t, n))
    return tuple(out)


CONFIG = dict(
    plan=((1, 1, False), (2, 1, False), (4, 1, True), (7, 1, True), (10, 5, True)),
    steady=_schedule(_ROWS, (16, 36, 24, 4, 28, 12, 8, 8, 28, 36, 36, 52)),
    warm=_schedule(_ROWS, (0, 28, 16, 12, 40, 8, 8, 32, 20, 36, 48, 40)),
    last=_schedule(_ROWS, (4, 36, 36, 16, 28, 16, 12, 12, 8, 36, 32, 52)),
    cold=(_schedule(_ROWS_COLD0, (0, 24, 28, 76, 0, 0, 0, 4, 0, 12)),
          _schedule(_ROWS_COLD, (0, 12, 60, 60, 40, 88, 64, 76, 32)),
          _schedule(_ROWS_COLD, (0, 36, 52, 36, 84, 68, 60, 84, 12))),
    gate_row=112,
    write_start=30,
    write_fine=48,
    bulk_slices=4,
    bulk_rows=24,
    bulk_per_unit=12,
)


def _pack(v):
    return pltpu.bitcast(v.astype(BF16), U32)


def _prep_first(g_ref, w_ref, ref, used, d_model, rows=16):
    g = g_ref[...].astype(F32).reshape(1, d_model)
    wt = jnp.concatenate([w_ref[0:L, :], w_ref[KH:KH + L, :]], axis=0).T
    keep = {}
    for r0 in range(0, H, rows):
        a11, a12, a21, a22 = [
            wt[h * H + r0:h * H + r0 + rows, k * L:(k + 1) * L].astype(F32)
            * g[:, k * KH:k * KH + L] for h in range(2) for k in range(2)]
        xs = (a11 + a22, a21 + a22, a11, a22, a11 + a12, a21 - a11, a12 - a22)
        for k in range(7):
            name = "S%da" % (k + 1)
            if name in used:
                ref[name][r0 // 2:(r0 + rows) // 2, :] = _pack(xs[k])
            keep[name, r0] = xs[k]
    for r0 in range(0, Q, rows):
        for p in LEVEL2:
            x11, x21 = keep[p + "a", r0], keep[p + "a", Q + r0]
            ref[p + "m3"][r0 // 2:(r0 + rows) // 2, :] = _pack(x11)
            ref[p + "m6"][r0 // 2:(r0 + rows) // 2, :] = _pack(x21 - x11)
    return keep


def _prep_rest(g_ref, b_ref, w_ref, ref, dl_ref, used, keep, d_model, rows=16):
    w = w_ref[...]
    g = g_ref[...].astype(F32).reshape(1, d_model)
    wt = jnp.concatenate([w[L:KH], w[KH + L:KM]], axis=0).T
    gt = jnp.concatenate([g[:, KM:d_model]] * 2, axis=1)
    at = jnp.concatenate([w[KM:d_model]] * 2, axis=0).T
    brow = jnp.broadcast_to(b_ref[...].astype(F32).reshape(1, d_model), (16, d_model))
    drow = jnp.dot(brow.astype(BF16), w, preferred_element_type=F32)
    row = lax.broadcasted_iota(jnp.int32, (16, d_model), 0)
    lo = drow - drow.astype(BF16).astype(F32)
    e = jnp.where(row == 0, drow, jnp.where(row == 1, lo, 0.0))
    z = jnp.zeros((48, d_model), F32)
    et = jnp.concatenate([e, z, e, z], axis=0).astype(BF16).T
    low = lax.broadcasted_iota(jnp.int32, (rows, L), 1) < 64

    def sel(p, q):
        return jnp.where(low, p, q)

    def level1(r0):
        a11, a12, a21, a22 = [
            wt[h * H + r0:h * H + r0 + rows, k * L:(k + 1) * L].astype(F32)
            * g[:, k * KH + L:(k + 1) * KH] for h in range(2) for k in range(2)]
        at1 = at[r0:r0 + rows].astype(F32) * gt
        at2 = at[H + r0:H + r0 + rows].astype(F32) * gt
        e1 = et[r0:r0 + rows].astype(F32)
        s2, s5, s6, s7 = a21 + a22, a11 + a12, a21 - a11, a12 - a22
        xs = (sel(a11 + a22, e1), sel(s2, -s2), sel(a11, a21), sel(a22, a12),
              sel(s5, -s5), sel(s6, at2), sel(s7, at1))
        res = {"S%db" % (k + 1): xs[k] for k in range(7)}
        res["R1"] = sel(e1, a21 + a12)
        res["R6"] = sel(at1, -s6)
        res["R7"] = sel(at2, -s7)
        for name in res:
            if name in used:
                ref[name][r0 // 2:(r0 + rows) // 2, :] = _pack(res[name])
        return res

    for r0 in range(0, Q, rows):
        u, v = level1(r0), level1(Q + r0)
        for p in LEVEL2:
            x11, x12 = keep[p + "a", r0], u[p + "b"]
            x21, x22 = keep[p + "a", Q + r0], v[p + "b"]
            xs = {1: x11 + x22, 2: x21 + x22, 4: x22, 5: x11 + x12, 7: x12 - x22}
            for k in xs:
                ref["%sm%d" % (p, k)][r0 // 2:(r0 + rows) // 2, :] = _pack(xs[k])
    low2 = lax.broadcasted_iota(jnp.int32, (H, L), 1) < 64
    lhs = jnp.where(low2, et[H:d_model].astype(F32), -et[0:H].astype(F32)).astype(BF16)
    dl_ref[...] = jnp.dot(lhs, jnp.ones((L, L), BF16), preferred_element_type=F32)


class _Stats:
    def __init__(self, x_ref, d_model, chains=1):
        self.x_ref, self.d_model = x_ref, d_model
        self.pos = 0
        self.x0 = None
        self.a1 = [None] * chains
        self.a2 = [None] * chains
        self.pending = []
        self.result = None

    def left(self):
        return STEPS - self.pos

    def advance(self, n):
        if self.x0 is None:
            self.x0 = self.x_ref[0:16, :].astype(F32)[0:1, :]
        for _ in range(n):
            if not self.pending:
                r0 = self.pos * 8
                t = self.x_ref[r0:r0 + 16, :].astype(F32) - self.x0
                self.pending = [t[0:8], t[8:16]]
            t = self.pending.pop(0)
            c = self.pos % len(self.a1)
            self.a1[c] = t if self.a1[c] is None else self.a1[c] + t
            self.a2[c] = t * t if self.a2[c] is None else self.a2[c] + t * t
            self.pos += 1
        return self.a2[0]

    def finish(self):
        if self.result is None:
            self.advance(self.left())
            a1 = functools.reduce(lambda u, v: u + v, self.a1)
            a2 = functools.reduce(lambda u, v: u + v, self.a2)
            s1 = jnp.sum(a1, axis=0, keepdims=True) * (1.0 / self.d_model)
            s2 = jnp.sum(a2, axis=0, keepdims=True) * (1.0 / self.d_model)
            var = jnp.maximum(s2 - s1 * s1, 0.0)
            self.result = (self.x0 + s1, lax.rsqrt(var + EPS))
        return self.result


def _signed_add(cur, v, sign):
    if cur is None:
        return v, sign
    val, cur_sign = cur
    if cur_sign == 1:
        return (val + v if sign == 1 else val - v), 1
    return (v - val, 1) if sign == 1 else (val + v, -1)


class _Unit:
    def __init__(self, xs_ref, os_ref, ref, dl_ref, c0, d_model, gate_row):
        self.xs_ref, self.os_ref, self.ref, self.dl_ref = xs_ref, os_ref, ref, dl_ref
        self.c0, self.d_model, self.gate_row = c0, d_model, gate_row
        self.stats = {}
        self.cache = {}
        self.queue = []
        self.on_store = None

    def col(self, pair, j):
        return self.c0 + (pair + 2 * j) * L

    def tile_stats(self, pair, j, chains=1):
        if (pair, j) not in self.stats:
            self.stats[pair, j] = _Stats(
                self.xs_ref.at[:, pl.ds(self.col(pair, j), L)], self.d_model, chains)
        return self.stats[pair, j]

    def norm(self, pair, j):
        return self.tile_stats(pair, j).finish()

    def x(self, pair, k, j, r0, r1):
        c = self.col(pair, j)
        return self.xs_ref[k * KH + r0:k * KH + r1, c:c + L].astype(F32)

    def hat(self, pair, k, j, r0, r1):
        m, r = self.norm(pair, j)
        return (self.x(pair, k, j, r0, r1) - m) * r

    def tail(self, pair, j):
        if ("tail", pair, j) not in self.cache:
            self.cache["tail", pair, j] = self.hat(pair, 2, j, 0, 64)
        return self.cache["tail", pair, j]

    def cross(self, pair, ka, kb, r0, r1):
        (ma, ra), (mb, rb) = self.norm(pair, 0), self.norm(pair, 1)
        if ("mr", pair) not in self.cache:
            self.cache["mr", pair] = ma * ra + mb * rb
        return (self.x(pair, ka, 0, r0, r1) * ra + self.x(pair, kb, 1, r0, r1) * rb
                - self.cache["mr", pair])

    def rhs(self, pair, name, raw=None):
        row = lax.broadcasted_iota(jnp.int32, (16, L), 0)
        ones = jnp.where(row < 2, 1.0, 0.0)

        def cat(*parts):
            return jnp.concatenate(parts, axis=0)

        if name == "R1":
            return cat(ones, jnp.zeros((48, L), F32), self.cross(pair, 0, 1, KS, KH))
        if name == "R6":
            return cat(self.tail(pair, 1), self.cross(pair, 0, 0, KS, KH))
        if name == "R7":
            return cat(self.tail(pair, 0), self.cross(pair, 1, 1, KS, KH))
        prod, r0 = name[:2], (0 if name[2] == "a" else L)
        if prod in ("S3", "S4"):
            j = 1 if prod == "S3" else 0
            diff = self.x(pair, 1 - j, j, r0, r0 + L) - self.x(pair, j, j, r0, r0 + L)
            if raw == "P":
                return diff
            if raw == "Q":
                return diff + self.norm(pair, 0)[1] * 0.0
            return diff * self.norm(pair, j)[1]
        main = {"S1": lambda a, b: self.cross(pair, 0, 1, a, b),
                "S2": lambda a, b: self.hat(pair, 0, 0, a, b),
                "S5": lambda a, b: self.hat(pair, 1, 1, a, b),
                "S6": lambda a, b: self.cross(pair, 0, 0, a, b),
                "S7": lambda a, b: self.cross(pair, 1, 1, a, b)}[prod]
        if r0 == 0:
            return main(0, L)
        rest = {"S1": lambda: ones,
                "S2": lambda: self.hat(pair, 1, 1, KS, KH),
                "S5": lambda: self.hat(pair, 0, 0, KS, KH),
                "S6": lambda: self.tail(pair, 1),
                "S7": lambda: self.tail(pair, 0)}[prod]
        return cat(main(L, KS), rest())

    def rhs2(self, prod, k):
        def h(kk, pair):
            if ("h", prod, kk, pair) not in self.cache:
                self.cache["h", prod, kk, pair] = self.rhs(pair, prod + "ab"[kk])
            return self.cache["h", prod, kk, pair]

        return {1: lambda: h(0, 0) + h(1, 1), 2: lambda: h(0, 0),
                3: lambda: h(0, 1) - h(1, 1), 4: lambda: h(1, 0) - h(0, 0),
                5: lambda: h(1, 1), 6: lambda: h(0, 0) + h(0, 1),
                7: lambda: h(1, 0) + h(1, 1)}[k]()

    def run(self, schedule, before_token):
        acc, count, done = {}, {}, {}
        acc2, count2, part = {}, {}, {}

        def add(pair, half, name, v):
            for key, sign in USES[name]:
                k = (pair, half, key)
                acc[k] = _signed_add(acc.get(k), v, sign)
                count[k] = count.get(k, 0) + 1
                if count[k] == TERMS[key]:
                    val, val_sign = acc[k]
                    assert val_sign == 1
                    done[k] = val
                    if (1 - pair, half, key) in done:
                        r0 = (0 if key[0] == "1" else H) + half * Q
                        c = self.col(0, int(key[1]) - 1)
                        both = jnp.concatenate(
                            [done[0, half, key], done[1, half, key]], axis=1)
                        self.os_ref[r0:r0 + Q, c:c + 2 * L] = both.astype(BF16)
                        if self.on_store is not None:
                            self.on_store(r0, c)

        def add_full(pair, name, v):
            add(pair, 0, name, v[0:Q])
            add(pair, 1, name, v[Q:H])

        for pos, (token, steps) in enumerate(schedule):
            before_token(pos)
            gate = None
            while steps > 0 and self.queue:
                n = min(steps, self.queue[0].left())
                gate = self.queue[0].advance(n)
                steps -= n
                if self.queue[0].left() == 0:
                    gate = jnp.broadcast_to(self.queue.pop(0).finish()[1], (8, L))

            def dot(name, q, gate=gate):
                if gate is not None:
                    g0 = self.gate_row if q.shape[0] > self.gate_row else 0
                    parts = [q[0:g0]] if g0 else []
                    parts.append(q[g0:g0 + 8] + gate * 0.0)
                    if g0 + 8 < q.shape[0]:
                        parts.append(q[g0 + 8:])
                    q = jnp.concatenate(parts, axis=0)
                p = pltpu.bitcast(self.ref[name][...], BF16)[:, 0:q.shape[0]]
                return jnp.dot(p, q.astype(BF16), preferred_element_type=F32)

            if ":" not in token:
                prod, k = token[:2], int(token[3])
                v = dot(token, self.rhs2(prod, k))
                for half, pair, sign in USES2[k]:
                    kk = (prod, half, pair)
                    acc2[kk] = _signed_add(acc2.get(kk), v, sign)
                    count2[kk] = count2.get(kk, 0) + 1
                    if count2[kk] == TERMS2[half, pair]:
                        val, val_sign = acc2[kk]
                        assert val_sign == 1
                        add(pair, half, prod, val)
                continue
            pair, name = "AB".index(token[0]), token[2:]
            if name == "D":
                add_full(pair, "D", self.dl_ref[...])
                continue
            if name == "V3":
                add_full(pair, "S3", part.pop((pair, "S3")) * self.norm(pair, 1)[1])
                continue
            raw = name[0] if name[0] in "PQ" else None
            name = "S" + name[1:] if raw else name
            v = dot(name, self.rhs(pair, name, raw))
            prod = name[:2]
            if prod[0] == "R":
                add_full(pair, prod, v)
            elif (pair, prod) not in part:
                part[pair, prod] = v
            elif raw:
                part[pair, prod] = v + part[pair, prod]
            else:
                add_full(pair, prod, v + part.pop((pair, prod)))
        assert len(done) == 16


def _forward(cfg, x, g, b, w):
    B, S, D = x.shape
    assert D == 2 * H == KM + 64 == 8 * STEPS
    plan = cfg["plan"]
    ups = B // UNIT
    n_units = S * ups
    assert sum(u * n for u, n, _ in plan) == n_units
    n_chunks = sum(n for _, n, _ in plan)
    names = LONG + SHORT
    used = {t[2:].replace("P", "S").replace("Q", "S")
            for sched in (cfg["steady"], *cfg["cold"]) for t, _ in sched if ":" in t}
    fine, per_unit = cfg["write_fine"], cfg["bulk_per_unit"]
    gs, rb = cfg["bulk_slices"], cfg["bulk_rows"]
    nrb = D // rb

    def issued(u, lo=jnp.minimum, hi=jnp.maximum):
        def ready(v):
            return nrb * (lo(v, fine) // (gs * ups))
        n = lo(per_unit * (u - cfg["write_start"] + 1), ready(u))
        for back in range(1, -(-nrb // per_unit)):
            n = lo(n, ready(u - back) + per_unit * back)
        return hi(n, 0)

    loop_start = sum(u * n for u, n, _ in plan[:-1])
    table = [issued(u, min, max) for u in range(n_units)]
    assert table[loop_start - 1] == 0 and fine >= loop_start and fine % (gs * ups) == 0
    assert all(0 <= table[u] - table[u - 1] <= per_unit for u in range(1, n_units))
    assert all(table[u] <= nrb * (u // (gs * ups)) for u in range(n_units))
    assert table[-1] == nrb * fine // (gs * ups)
    assert all(n == 1 for _, n, _ in plan[:-1]) and plan[-1][2] and plan[-2][2]

    xt = jnp.transpose(x, (1, 2, 0))

    def kernel(x_hbm, g_hbm, b_hbm, w_hbm, o_hbm, xbuf, obuf, wbuf, gbuf, bbuf, *rest):
        ref = dict(zip(names, rest))
        dl_ref, isem, nsem, osem, wsem = rest[len(names):]

        def copies(sem, u, end, shift=0):
            res = []
            while u < end:
                s, r = divmod(u, ups)
                if r == 0 and end - u >= ups:
                    idx = (pl.ds(s + shift, (end - u) // ups),)
                    u += (end - u) // ups * ups
                else:
                    idx = (s + shift, slice(None), pl.ds(r * UNIT, UNIT))
                    u += 1
                res.append(pltpu.make_async_copy(x_hbm.at[idx], xbuf.at[idx], sem))
            return res

        def write_back(*idx):
            pltpu.make_async_copy(obuf.at[idx], o_hbm.at[idx], osem.at[0]).start()

        def w_rows(r0, r1, k):
            rows = pl.ds(r0, r1 - r0)
            return pltpu.make_async_copy(w_hbm.at[rows], wbuf.at[rows], wsem.at[k])

        cg = pltpu.make_async_copy(g_hbm, gbuf, wsem.at[1])
        cb = pltpu.make_async_copy(b_hbm, bbuf, wsem.at[2])
        w_first = [w_rows(0, L, 0), w_rows(KH, KH + L, 0)]
        w_rest = [w_rows(L, KH, 3), w_rows(KH + L, D, 3)]
        for c in [cg, cb] + w_first + w_rest:
            c.start()
        cg.wait()
        cb.wait()
        j = u0 = 0
        handed = False
        for nu, count, hand in plan:
            for _ in range(count):
                for c in copies(isem.at[j], u0 + handed, u0 + nu):
                    c.start()
                if hand and u0 + nu < n_units:
                    for c in copies(nsem.at[j], u0 + nu, u0 + nu + 1):
                        c.start()
                j += 1
                u0 += nu
                handed = hand
        for c in w_first:
            c.wait()
        keep = _prep_first(gbuf, wbuf, ref, used, D)
        for c in w_rest:
            c.wait()
        _prep_rest(gbuf, bbuf, wbuf, ref, dl_ref, used, keep, D)

        def make_unit(s, c0):
            return _Unit(xbuf.at[s], obuf.at[s], ref, dl_ref, c0, D, cfg["gate_row"])

        def do_chunk(j, u0, nu, shift, stats_in, hand, in_loop):
            for c in copies(isem.at[j], u0 + (stats_in is not None), u0 + nu, shift):
                c.wait()
            if hand:
                s_next, r_next = divmod(u0 + nu, ups)
                if in_loop:
                    exists = s_next + shift < S
                    s_next = jnp.minimum(s_next + shift, S - 1)

                    @pl.when(exists)
                    def _():
                        copies(nsem.at[j], r_next, r_next + 1, s_next)[0].wait()
                else:
                    copies(nsem.at[j], u0 + nu, u0 + nu + 1)[0].wait()
            where = [(u // ups + shift, (u % ups) * UNIT) for u in range(u0, u0 + nu)]
            units = [make_unit(s, c0) for s, c0 in where]
            if stats_in is None:
                units[0].tile_stats(0, 0, chains=2)
                units[0].queue = [units[0].tile_stats(1, 0), units[0].tile_stats(1, 1)]
            else:
                for n, key in enumerate(TILE_ORDER[1:]):
                    units[0].tile_stats(*key).result = stats_in[2 * n:2 * n + 2]
                head = units[0].tile_stats(*TILE_ORDER[0])
                head.x0, head.a1, head.a2 = stats_in[6], [stats_in[7]], [stats_in[8]]
                head.pos = STEPS
            for p in range(nu - 1):
                units[p].queue += [units[p + 1].tile_stats(*key) for key in TILE_ORDER]
            if hand:
                ahead = make_unit(s_next, r_next * UNIT)
                units[-1].queue += [ahead.tile_stats(*key)
                                    for key in TILE_ORDER[1:] + TILE_ORDER[:1]]

            for p, (s, c0) in enumerate(where):
                if p == 0:
                    schedule = cfg["cold"][j] if stats_in is None else cfg["warm"]
                else:
                    schedule = cfg["last"] if (hand and p == nu - 1) else cfg["steady"]
                if not in_loop:
                    units[p].run(schedule, lambda pos: None)
                    continue
                u = u0 + p + shift * ups
                k0, k1 = issued(u - 1), issued(u)
                groups = -(-per_unit // 6)
                slots = {len(schedule) * i // groups: i for i in range(groups)}

                def delayed(pos, k0=k0, k1=k1, slots=slots):
                    if pos in slots:
                        for i in range(slots[pos] * 6, min(slots[pos] * 6 + 6, per_unit)):
                            k = k0 + i
                            pl.when(k < k1)(functools.partial(
                                write_back, pl.ds(k // nrb * gs, gs),
                                pl.ds(pl.multiple_of(k % nrb * rb, 8), rb)))

                now = u >= fine
                if p == nu - 1:
                    now = now & (u < n_units - 1)

                    def on_store(r0, c, s=s, u=u):
                        pl.when(u == n_units - 1)(functools.partial(
                            write_back, s, pl.ds(r0, Q), pl.ds(c, 2 * L)))
                    units[p].on_store = on_store
                units[p].run(schedule, delayed)

                @pl.when(now)
                def _(s=s, c0=c0):
                    for c in range(c0, c0 + UNIT, L):
                        write_back(s, slice(None), pl.ds(c, L))

            if not hand:
                return None
            head = ahead.tile_stats(*TILE_ORDER[0])
            assert head.left() == 0
            return (*[v for key in TILE_ORDER[1:] for v in ahead.norm(*key)],
                    head.x0, head.a1[0], head.a2[0])

        j = u0 = 0
        stats = None
        for nu, count, hand in plan:
            if count == 1:
                stats = do_chunk(j, u0, nu, 0, stats, hand, False)
            else:
                assert nu % ups == 0 and u0 % ups == 0

                def body(it, carry, j=j, u0=u0, nu=nu):
                    return do_chunk(j + it, u0, nu, it * (nu // ups), carry, True, True)
                lax.fori_loop(0, count, body, stats)
            j += count
            u0 += nu * count
        pltpu.make_async_copy(obuf, o_hbm, osem.at[0]).wait()

    out = pl.pallas_call(
        kernel,
        in_specs=[pl.BlockSpec(memory_space=pl.ANY)] * 4,
        out_specs=pl.BlockSpec(memory_space=pl.ANY),
        out_shape=jax.ShapeDtypeStruct((S, D, B), x.dtype),
        scratch_shapes=[
            pltpu.VMEM((S, D, B), BF16),
            pltpu.VMEM((S, D, B), BF16),
            pltpu.VMEM((D, D), BF16),
            pltpu.VMEM((D,), BF16),
            pltpu.VMEM((D,), BF16),
            *[pltpu.VMEM(((H if n in LONG else Q) // 2, L), U32) for n in names],
            pltpu.VMEM((H, L), F32),
            pltpu.SemaphoreType.DMA((n_chunks,)),
            pltpu.SemaphoreType.DMA((n_chunks,)),
            pltpu.SemaphoreType.DMA((1,)),
            pltpu.SemaphoreType.DMA((4,)),
        ],
        compiler_params=pltpu.CompilerParams(
            vmem_limit_bytes=110 * 1024 * 1024,
            disable_bounds_checks=True,
            disable_semaphore_checks=True,
        ),
    )(xt, g, b, w)
    return jnp.transpose(out, (2, 0, 1))


@jax.jit
def pallas_standalone__layernorm_linear__sampling_kernel(
    x: jax.Array,
    g: jax.Array,
    b: jax.Array,
    w: jax.Array,
):
    return _forward(CONFIG, x, g, b, w)
```

```python
import functools

import jax
import jax.numpy as jnp
from jax import lax
import jax.experimental.pallas as pl
import jax.experimental.pallas.tpu as pltpu

EPS = 1e-5
F32 = jnp.float32
BF16 = jnp.bfloat16
U32 = jnp.uint32

L = 128
H = 288
Q = 144
KH = 256
KS = 192
KM = 2 * KH
UNIT = 512
STEPS = 72

LONG = tuple("S%d%s" % (i, h) for i in range(1, 8) for h in "ab") + ("R1", "R6", "R7")
LEVEL2 = ("S2", "S3", "S4", "S5")
SHORT = tuple("%sm%d" % (p, k) for p in LEVEL2 for k in range(1, 8))
USES = {
    "S1": (("11", 1), ("22", 1)), "S2": (("21", 1), ("22", -1)),
    "S3": (("12", 1), ("22", 1)), "S4": (("11", 1), ("21", 1)),
    "S5": (("11", -1), ("12", 1)), "S6": (("22", 1),), "S7": (("11", 1),),
    "R1": (("12", 1), ("21", 1)), "R6": (("12", 1),), "R7": (("21", 1),),
    "D": (("21", 1), ("22", 1)),
}
TERMS = {"11": 4, "12": 4, "21": 5, "22": 5}
USES2 = {1: ((0, 0, 1), (1, 1, 1)), 2: ((1, 0, 1), (1, 1, -1)), 3: ((0, 1, 1), (1, 1, 1)),
         4: ((0, 0, 1), (1, 0, 1)), 5: ((0, 0, -1), (0, 1, 1)), 6: ((1, 1, 1),),
         7: ((0, 0, 1),)}
TERMS2 = {(0, 0): 4, (0, 1): 2, (1, 0): 2, (1, 1): 4}
TILE_ORDER = ((0, 0), (1, 0), (0, 1), (1, 1))

_ROWS = ("S4m1 S4m7 S4m6 S4m2", "S4m4 S4m3 S4m5 S2m1", "S2m6 S2m2 S2m4 S2m3",
         "S2m5 S2m7 S3m4 S3m2", "S3m5 S3m3 S3m1 S3m6", "A:D B:D S3m7 S5m1 S5m7 S5m6",
         "A:R7 B:R7 S5m2 S5m4", "S5m3 S5m5", "A:S1a A:S1b B:S1a B:S1b",
         "A:R1 B:R1 A:R6 B:R6", "A:S7a A:S7b B:S7a B:S7b", "A:S6a A:S6b B:S6a B:S6b")
_ROWS_COLD = ("A:S4a A:S4b A:S2a A:Q3a", "A:P3b A:S5a A:V3 A:D A:S2b A:R7",
              "A:S5b A:R1 A:R6 A:S1a", "A:S1b A:S7a A:S7b A:S6a", "A:S6b B:S4a B:S4b B:S2a",
              "B:S3a B:S3b B:S5a B:D B:S2b", "B:R7 B:S5b B:R1 B:R6",
              "B:S1a B:S1b B:S7a B:S7b", "B:S6a B:S6b")
_ROWS_COLD0 = ("A:S4a A:S4b A:Q3a A:Q3b", "A:V3 A:D A:R7 A:R1 B:S4a B:S4b",
               "A:R6 A:S1a A:S1b B:P3a", "B:P3b A:S7a A:S7b A:S6a",
               "A:S6b B:V3 B:D B:R7 B:R1 B:R6", "S2m2 S2m4 S2m3 S2m5", "S2m6 S2m1 S2m7 S5m1",
               "S5m7 S5m6 S5m2 S5m4", "B:S1a B:S1b S5m3 S5m5", "B:S7a B:S7b B:S6a B:S6b")


def _schedule(rows, weights):
    out = []
    for row, steps in zip(rows, weights, strict=True):
        toks = row.split()
        passes = [t for t in toks if not (t.endswith(":D") or ":V" in t)]
        for t in toks:
            n = 0
            if t in passes:
                k = passes.index(t)
                n = steps * (k + 1) // len(passes) - steps * k // len(passes)
            out.append((t, n))
    return tuple(out)


CONFIG = dict(
    plan=((1, 1, False), (2, 1, False), (4, 1, True), (7, 1, True), (10, 5, True)),
    steady=_schedule(_ROWS, (12, 20, 36, 12, 20, 12, 24, 8, 24, 36, 32, 52)),
    warm=_schedule(_ROWS, (0, 28, 16, 12, 28, 20, 8, 32, 20, 36, 48, 40)),
    last=_schedule(_ROWS, (12, 36, 28, 12, 28, 20, 12, 16, 16, 28, 28, 52)),
    cold=(_schedule(_ROWS_COLD0, (0, 24, 28, 76, 0, 0, 0, 4, 0, 12)),
          _schedule(_ROWS_COLD, (0, 12, 60, 60, 40, 88, 64, 76, 32)),
          _schedule(_ROWS_COLD, (0, 36, 52, 36, 84, 68, 60, 84, 12))),
    gate_row=112,
    write_start=30,
    write_fine=48,
    bulk_slices=4,
    bulk_rows=24,
    bulk_per_unit=12,
    bulk_at=(4, 8, 20, 32, 36, 41),
)


def _pack(v):
    return pltpu.bitcast(v.astype(BF16), U32)


def _prep_first(g_ref, w_ref, ref, used, d_model, rows=16):
    g = g_ref[...].astype(F32).reshape(1, d_model)
    wt = jnp.concatenate([w_ref[0:L, :], w_ref[KH:KH + L, :]], axis=0).T
    keep = {}
    for r0 in range(0, H, rows):
        a11, a12, a21, a22 = [
            wt[h * H + r0:h * H + r0 + rows, k * L:(k + 1) * L].astype(F32)
            * g[:, k * KH:k * KH + L] for h in range(2) for k in range(2)]
        xs = (a11 + a22, a21 + a22, a11, a22, a11 + a12, a21 - a11, a12 - a22)
        for k in range(7):
            name = "S%da" % (k + 1)
            if name in used:
                ref[name][r0 // 2:(r0 + rows) // 2, :] = _pack(xs[k])
            keep[name, r0] = xs[k]
    for r0 in range(0, Q, rows):
        for p in LEVEL2:
            x11, x21 = keep[p + "a", r0], keep[p + "a", Q + r0]
            ref[p + "m3"][r0 // 2:(r0 + rows) // 2, :] = _pack(x11)
            ref[p + "m6"][r0 // 2:(r0 + rows) // 2, :] = _pack(x21 - x11)
    return keep


def _prep_rest(g_ref, b_ref, w_ref, ref, dl_ref, used, keep, d_model, rows=16):
    w = w_ref[...]
    g = g_ref[...].astype(F32).reshape(1, d_model)
    wt = jnp.concatenate([w[L:KH], w[KH + L:KM]], axis=0).T
    gt = jnp.concatenate([g[:, KM:d_model]] * 2, axis=1)
    at = jnp.concatenate([w[KM:d_model]] * 2, axis=0).T
    brow = jnp.broadcast_to(b_ref[...].astype(F32).reshape(1, d_model), (16, d_model))
    drow = jnp.dot(brow.astype(BF16), w, preferred_element_type=F32)
    row = lax.broadcasted_iota(jnp.int32, (16, d_model), 0)
    lo = drow - drow.astype(BF16).astype(F32)
    e = jnp.where(row == 0, drow, jnp.where(row == 1, lo, 0.0))
    z = jnp.zeros((48, d_model), F32)
    et = jnp.concatenate([e, z, e, z], axis=0).astype(BF16).T
    low = lax.broadcasted_iota(jnp.int32, (rows, L), 1) < 64

    def sel(p, q):
        return jnp.where(low, p, q)

    def level1(r0):
        a11, a12, a21, a22 = [
            wt[h * H + r0:h * H + r0 + rows, k * L:(k + 1) * L].astype(F32)
            * g[:, k * KH + L:(k + 1) * KH] for h in range(2) for k in range(2)]
        at1 = at[r0:r0 + rows].astype(F32) * gt
        at2 = at[H + r0:H + r0 + rows].astype(F32) * gt
        e1 = et[r0:r0 + rows].astype(F32)
        s2, s5, s6, s7 = a21 + a22, a11 + a12, a21 - a11, a12 - a22
        xs = (sel(a11 + a22, e1), sel(s2, -s2), sel(a11, a21), sel(a22, a12),
              sel(s5, -s5), sel(s6, at2), sel(s7, at1))
        res = {"S%db" % (k + 1): xs[k] for k in range(7)}
        res["R1"] = sel(e1, a21 + a12)
        res["R6"] = sel(at1, -s6)
        res["R7"] = sel(at2, -s7)
        for name in res:
            if name in used:
                ref[name][r0 // 2:(r0 + rows) // 2, :] = _pack(res[name])
        return res

    for r0 in range(0, Q, rows):
        u, v = level1(r0), level1(Q + r0)
        for p in LEVEL2:
            x11, x12 = keep[p + "a", r0], u[p + "b"]
            x21, x22 = keep[p + "a", Q + r0], v[p + "b"]
            xs = {1: x11 + x22, 2: x21 + x22, 4: x22, 5: x11 + x12, 7: x12 - x22}
            for k in xs:
                ref["%sm%d" % (p, k)][r0 // 2:(r0 + rows) // 2, :] = _pack(xs[k])
    low2 = lax.broadcasted_iota(jnp.int32, (H, L), 1) < 64
    lhs = jnp.where(low2, et[H:d_model].astype(F32), -et[0:H].astype(F32)).astype(BF16)
    dl_ref[...] = jnp.dot(lhs, jnp.ones((L, L), BF16), preferred_element_type=F32)


class _Stats:
    def __init__(self, x_ref, d_model, chains=1):
        self.x_ref, self.d_model = x_ref, d_model
        self.pos = 0
        self.x0 = None
        self.a1 = [None] * chains
        self.a2 = [None] * chains
        self.pending = []
        self.result = None

    def left(self):
        return STEPS - self.pos

    def advance(self, n):
        if self.x0 is None:
            self.x0 = self.x_ref[0:16, :].astype(F32)[0:1, :]
        for _ in range(n):
            if not self.pending:
                r0 = self.pos * 8
                t = self.x_ref[r0:r0 + 16, :].astype(F32) - self.x0
                self.pending = [t[0:8], t[8:16]]
            t = self.pending.pop(0)
            c = self.pos % len(self.a1)
            self.a1[c] = t if self.a1[c] is None else self.a1[c] + t
            self.a2[c] = t * t if self.a2[c] is None else self.a2[c] + t * t
            self.pos += 1
        return self.a2[0]

    def finish(self):
        if self.result is None:
            self.advance(self.left())
            a1 = functools.reduce(lambda u, v: u + v, self.a1)
            a2 = functools.reduce(lambda u, v: u + v, self.a2)
            s1 = jnp.sum(a1, axis=0, keepdims=True) * (1.0 / self.d_model)
            s2 = jnp.sum(a2, axis=0, keepdims=True) * (1.0 / self.d_model)
            var = jnp.maximum(s2 - s1 * s1, 0.0)
            self.result = (self.x0 + s1, lax.rsqrt(var + EPS))
        return self.result


def _signed_add(cur, v, sign):
    if cur is None:
        return v, sign
    val, cur_sign = cur
    if cur_sign == 1:
        return (val + v if sign == 1 else val - v), 1
    return (v - val, 1) if sign == 1 else (val + v, -1)


class _Unit:
    def __init__(self, xs_ref, os_ref, ref, dl_ref, c0, d_model, gate_row):
        self.xs_ref, self.os_ref, self.ref, self.dl_ref = xs_ref, os_ref, ref, dl_ref
        self.c0, self.d_model, self.gate_row = c0, d_model, gate_row
        self.stats = {}
        self.cache = {}
        self.queue = []
        self.on_store = None

    def col(self, pair, j):
        return self.c0 + (pair + 2 * j) * L

    def tile_stats(self, pair, j, chains=1):
        if (pair, j) not in self.stats:
            self.stats[pair, j] = _Stats(
                self.xs_ref.at[:, pl.ds(self.col(pair, j), L)], self.d_model, chains)
        return self.stats[pair, j]

    def norm(self, pair, j):
        return self.tile_stats(pair, j).finish()

    def x(self, pair, k, j, r0, r1):
        c = self.col(pair, j)
        return self.xs_ref[k * KH + r0:k * KH + r1, c:c + L].astype(F32)

    def hat(self, pair, k, j, r0, r1):
        m, r = self.norm(pair, j)
        return (self.x(pair, k, j, r0, r1) - m) * r

    def tail(self, pair, j):
        if ("tail", pair, j) not in self.cache:
            self.cache["tail", pair, j] = self.hat(pair, 2, j, 0, 64)
        return self.cache["tail", pair, j]

    def cross(self, pair, ka, kb, r0, r1):
        (ma, ra), (mb, rb) = self.norm(pair, 0), self.norm(pair, 1)
        if ("mr", pair) not in self.cache:
            self.cache["mr", pair] = ma * ra + mb * rb
        return (self.x(pair, ka, 0, r0, r1) * ra + self.x(pair, kb, 1, r0, r1) * rb
                - self.cache["mr", pair])

    def rhs(self, pair, name, raw=None):
        row = lax.broadcasted_iota(jnp.int32, (16, L), 0)
        ones = jnp.where(row < 2, 1.0, 0.0)

        def cat(*parts):
            return jnp.concatenate(parts, axis=0)

        if name == "R1":
            return cat(ones, jnp.zeros((48, L), F32), self.cross(pair, 0, 1, KS, KH))
        if name == "R6":
            return cat(self.tail(pair, 1), self.cross(pair, 0, 0, KS, KH))
        if name == "R7":
            return cat(self.tail(pair, 0), self.cross(pair, 1, 1, KS, KH))
        prod, r0 = name[:2], (0 if name[2] == "a" else L)
        if prod in ("S3", "S4"):
            j = 1 if prod == "S3" else 0
            diff = self.x(pair, 1 - j, j, r0, r0 + L) - self.x(pair, j, j, r0, r0 + L)
            if raw == "P":
                return diff
            if raw == "Q":
                return diff + self.norm(pair, 0)[1] * 0.0
            return diff * self.norm(pair, j)[1]
        main = {"S1": lambda a, b: self.cross(pair, 0, 1, a, b),
                "S2": lambda a, b: self.hat(pair, 0, 0, a, b),
                "S5": lambda a, b: self.hat(pair, 1, 1, a, b),
                "S6": lambda a, b: self.cross(pair, 0, 0, a, b),
                "S7": lambda a, b: self.cross(pair, 1, 1, a, b)}[prod]
        if r0 == 0:
            return main(0, L)
        rest = {"S1": lambda: ones,
                "S2": lambda: self.hat(pair, 1, 1, KS, KH),
                "S5": lambda: self.hat(pair, 0, 0, KS, KH),
                "S6": lambda: self.tail(pair, 1),
                "S7": lambda: self.tail(pair, 0)}[prod]
        return cat(main(L, KS), rest())

    def rhs2(self, prod, k):
        def h(kk, pair):
            if ("h", prod, kk, pair) not in self.cache:
                self.cache["h", prod, kk, pair] = self.rhs(pair, prod + "ab"[kk])
            return self.cache["h", prod, kk, pair]

        return {1: lambda: h(0, 0) + h(1, 1), 2: lambda: h(0, 0),
                3: lambda: h(0, 1) - h(1, 1), 4: lambda: h(1, 0) - h(0, 0),
                5: lambda: h(1, 1), 6: lambda: h(0, 0) + h(0, 1),
                7: lambda: h(1, 0) + h(1, 1)}[k]()

    def run(self, schedule, before_token):
        acc, count, done = {}, {}, {}
        acc2, count2, part = {}, {}, {}

        def add(pair, half, name, v):
            for key, sign in USES[name]:
                k = (pair, half, key)
                acc[k] = _signed_add(acc.get(k), v, sign)
                count[k] = count.get(k, 0) + 1
                if count[k] == TERMS[key]:
                    val, val_sign = acc[k]
                    assert val_sign == 1
                    done[k] = val
                    if (1 - pair, half, key) in done:
                        r0 = (0 if key[0] == "1" else H) + half * Q
                        c = self.col(0, int(key[1]) - 1)
                        both = jnp.concatenate(
                            [done[0, half, key], done[1, half, key]], axis=1)
                        self.os_ref[r0:r0 + Q, c:c + 2 * L] = both.astype(BF16)
                        if self.on_store is not None:
                            self.on_store(r0, c)

        def add_full(pair, name, v):
            add(pair, 0, name, v[0:Q])
            add(pair, 1, name, v[Q:H])

        for pos, (token, steps) in enumerate(schedule):
            before_token(pos)
            gate = None
            while steps > 0 and self.queue:
                n = min(steps, self.queue[0].left())
                gate = self.queue[0].advance(n)
                steps -= n
                if self.queue[0].left() == 0:
                    gate = jnp.broadcast_to(self.queue.pop(0).finish()[1], (8, L))

            def dot(name, q, gate=gate):
                if gate is not None:
                    g0 = self.gate_row if q.shape[0] > self.gate_row else 0
                    parts = [q[0:g0]] if g0 else []
                    parts.append(q[g0:g0 + 8] + gate * 0.0)
                    if g0 + 8 < q.shape[0]:
                        parts.append(q[g0 + 8:])
                    q = jnp.concatenate(parts, axis=0)
                p = pltpu.bitcast(self.ref[name][...], BF16)[:, 0:q.shape[0]]
                return jnp.dot(p, q.astype(BF16), preferred_element_type=F32)

            if ":" not in token:
                prod, k = token[:2], int(token[3])
                v = dot(token, self.rhs2(prod, k))
                for half, pair, sign in USES2[k]:
                    kk = (prod, half, pair)
                    acc2[kk] = _signed_add(acc2.get(kk), v, sign)
                    count2[kk] = count2.get(kk, 0) + 1
                    if count2[kk] == TERMS2[half, pair]:
                        val, val_sign = acc2[kk]
                        assert val_sign == 1
                        add(pair, half, prod, val)
                continue
            pair, name = "AB".index(token[0]), token[2:]
            if name == "D":
                add_full(pair, "D", self.dl_ref[...])
                continue
            if name == "V3":
                add_full(pair, "S3", part.pop((pair, "S3")) * self.norm(pair, 1)[1])
                continue
            raw = name[0] if name[0] in "PQ" else None
            name = "S" + name[1:] if raw else name
            v = dot(name, self.rhs(pair, name, raw))
            prod = name[:2]
            if prod[0] == "R":
                add_full(pair, prod, v)
            elif (pair, prod) not in part:
                part[pair, prod] = v
            elif raw:
                part[pair, prod] = v + part[pair, prod]
            else:
                add_full(pair, prod, v + part.pop((pair, prod)))
        assert len(done) == 16


def _forward(cfg, x, g, b, w):
    B, S, D = x.shape
    assert D == 2 * H == KM + 64 == 8 * STEPS
    plan = cfg["plan"]
    ups = B // UNIT
    n_units = S * ups
    assert sum(u * n for u, n, _ in plan) == n_units
    n_chunks = sum(n for _, n, _ in plan)
    names = LONG + SHORT
    used = {t[2:].replace("P", "S").replace("Q", "S")
            for sched in (cfg["steady"], *cfg["cold"]) for t, _ in sched if ":" in t}
    fine, per_unit = cfg["write_fine"], cfg["bulk_per_unit"]
    gs, rb = cfg["bulk_slices"], cfg["bulk_rows"]
    nrb = D // rb

    assert nrb == 2 * per_unit and gs * ups == 8
    per_slot = per_unit // len(cfg["bulk_at"])
    assert per_slot * len(cfg["bulk_at"]) == per_unit

    def issued(u, lo=jnp.minimum, hi=jnp.maximum):
        def ready(v):
            return 2 * (lo(v, fine) >> 3)
        n = lo(lo(u - cfg["write_start"] + 1, ready(u)), ready(u - 1) + 1)
        return hi(n, 0)

    loop_start = sum(u * n for u, n, _ in plan[:-1])
    table = {u: issued(u, min, max) for u in range(loop_start - 1, n_units)}
    assert table[loop_start - 1] == 0 and fine >= loop_start and fine % (gs * ups) == 0
    assert all(0 <= table[u] - table[u - 1] <= 1 for u in range(loop_start, n_units))
    assert all(table[u] <= 2 * (u // (gs * ups)) for u in table)
    assert table[n_units - 1] == 2 * fine // (gs * ups)
    assert all(n == 1 for _, n, _ in plan[:-1]) and plan[-1][2] and plan[-2][2]

    xt = jnp.transpose(x, (1, 2, 0))

    def kernel(x_hbm, g_hbm, b_hbm, w_hbm, o_hbm, xbuf, obuf, wbuf, gbuf, bbuf, *rest):
        ref = dict(zip(names, rest))
        dl_ref, isem, nsem, osem, wsem = rest[len(names):]

        def copies(sem, u, end, shift=0):
            res = []
            while u < end:
                s, r = divmod(u, ups)
                if r == 0 and end - u >= ups:
                    idx = (pl.ds(s + shift, (end - u) // ups),)
                    u += (end - u) // ups * ups
                else:
                    idx = (s + shift, slice(None), pl.ds(r * UNIT, UNIT))
                    u += 1
                res.append(pltpu.make_async_copy(x_hbm.at[idx], xbuf.at[idx], sem))
            return res

        def write_back(*idx):
            pltpu.make_async_copy(obuf.at[idx], o_hbm.at[idx], osem.at[0]).start()

        def w_rows(r0, r1, k):
            rows = pl.ds(r0, r1 - r0)
            return pltpu.make_async_copy(w_hbm.at[rows], wbuf.at[rows], wsem.at[k])

        cg = pltpu.make_async_copy(g_hbm, gbuf, wsem.at[1])
        cb = pltpu.make_async_copy(b_hbm, bbuf, wsem.at[2])
        w_first = [w_rows(0, L, 0), w_rows(KH, KH + L, 0)]
        w_rest = [w_rows(L, KH, 3), w_rows(KH + L, D, 3)]
        for c in [cg, cb] + w_first + w_rest:
            c.start()
        cg.wait()
        cb.wait()
        j = u0 = 0
        handed = False
        for nu, count, hand in plan:
            for _ in range(count):
                for c in copies(isem.at[j], u0 + handed, u0 + nu):
                    c.start()
                if hand and u0 + nu < n_units:
                    for c in copies(nsem.at[j], u0 + nu, u0 + nu + 1):
                        c.start()
                j += 1
                u0 += nu
                handed = hand
        for c in w_first:
            c.wait()
        keep = _prep_first(gbuf, wbuf, ref, used, D)
        for c in w_rest:
            c.wait()
        _prep_rest(gbuf, bbuf, wbuf, ref, dl_ref, used, keep, D)

        def make_unit(s, c0):
            return _Unit(xbuf.at[s], obuf.at[s], ref, dl_ref, c0, D, cfg["gate_row"])

        def do_chunk(j, u0, nu, shift, stats_in, hand, in_loop):
            for c in copies(isem.at[j], u0 + (stats_in is not None), u0 + nu, shift):
                c.wait()
            if hand:
                s_next, r_next = divmod(u0 + nu, ups)
                if in_loop:
                    exists = s_next + shift < S
                    s_next = jnp.minimum(s_next + shift, S - 1)

                    @pl.when(exists)
                    def _():
                        copies(nsem.at[j], r_next, r_next + 1, s_next)[0].wait()
                else:
                    copies(nsem.at[j], u0 + nu, u0 + nu + 1)[0].wait()
            where = [(u // ups + shift, (u % ups) * UNIT) for u in range(u0, u0 + nu)]
            units = [make_unit(s, c0) for s, c0 in where]
            if stats_in is None:
                units[0].tile_stats(0, 0, chains=2)
                units[0].queue = [units[0].tile_stats(1, 0), units[0].tile_stats(1, 1)]
            else:
                for n, key in enumerate(TILE_ORDER[1:]):
                    units[0].tile_stats(*key).result = stats_in[2 * n:2 * n + 2]
                head = units[0].tile_stats(*TILE_ORDER[0])
                head.x0, head.a1, head.a2 = stats_in[6], [stats_in[7]], [stats_in[8]]
                head.pos = STEPS
            for p in range(nu - 1):
                units[p].queue += [units[p + 1].tile_stats(*key) for key in TILE_ORDER]
            if hand:
                ahead = make_unit(s_next, r_next * UNIT)
                units[-1].queue += [ahead.tile_stats(*key)
                                    for key in TILE_ORDER[1:] + TILE_ORDER[:1]]

            for p, (s, c0) in enumerate(where):
                if p == 0:
                    schedule = cfg["cold"][j] if stats_in is None else cfg["warm"]
                else:
                    schedule = cfg["last"] if (hand and p == nu - 1) else cfg["steady"]
                if not in_loop:
                    units[p].run(schedule, lambda pos: None)
                    continue
                u = u0 + p + shift * ups
                k0, k1 = issued(u - 1), issued(u)

                def delayed(pos, k0=k0, k1=k1):
                    if pos in cfg["bulk_at"]:
                        first = cfg["bulk_at"].index(pos) * per_slot
                        for i in range(first, first + per_slot):
                            row = (k0 & 1) * (per_unit * rb) + i * rb
                            pl.when(k0 < k1)(functools.partial(
                                write_back, pl.ds((k0 >> 1) * gs, gs),
                                pl.ds(pl.multiple_of(row, 8), rb)))

                now = u >= fine
                if p == nu - 1:
                    now = now & (u < n_units - 1)

                    def on_store(r0, c, s=s, u=u):
                        pl.when(u == n_units - 1)(functools.partial(
                            write_back, s, pl.ds(r0, Q), pl.ds(c, 2 * L)))
                    units[p].on_store = on_store
                units[p].run(schedule, delayed)

                @pl.when(now)
                def _(s=s, c0=c0):
                    for c in range(c0, c0 + UNIT, L):
                        write_back(s, slice(None), pl.ds(c, L))

            if not hand:
                return None
            head = ahead.tile_stats(*TILE_ORDER[0])
            assert head.left() == 0
            return (*[v for key in TILE_ORDER[1:] for v in ahead.norm(*key)],
                    head.x0, head.a1[0], head.a2[0])

        j = u0 = 0
        stats = None
        for nu, count, hand in plan:
            if count == 1:
                stats = do_chunk(j, u0, nu, 0, stats, hand, False)
            else:
                assert nu % ups == 0 and u0 % ups == 0

                def body(it, carry, j=j, u0=u0, nu=nu):
                    return do_chunk(j + it, u0, nu, it * (nu // ups), carry, True, True)
                lax.fori_loop(0, count, body, stats)
            j += count
            u0 += nu * count
        pltpu.make_async_copy(obuf, o_hbm, osem.at[0]).wait()

    out = pl.pallas_call(
        kernel,
        in_specs=[pl.BlockSpec(memory_space=pl.ANY)] * 4,
        out_specs=pl.BlockSpec(memory_space=pl.ANY),
        out_shape=jax.ShapeDtypeStruct((S, D, B), x.dtype),
        scratch_shapes=[
            pltpu.VMEM((S, D, B), BF16),
            pltpu.VMEM((S, D, B), BF16),
            pltpu.VMEM((D, D), BF16),
            pltpu.VMEM((D,), BF16),
            pltpu.VMEM((D,), BF16),
            *[pltpu.VMEM(((H if n in LONG else Q) // 2, L), U32) for n in names],
            pltpu.VMEM((H, L), F32),
            pltpu.SemaphoreType.DMA((n_chunks,)),
            pltpu.SemaphoreType.DMA((n_chunks,)),
            pltpu.SemaphoreType.DMA((1,)),
            pltpu.SemaphoreType.DMA((4,)),
        ],
        compiler_params=pltpu.CompilerParams(
            vmem_limit_bytes=110 * 1024 * 1024,
            disable_bounds_checks=True,
            disable_semaphore_checks=True,
        ),
    )(xt, g, b, w)
    return jnp.transpose(out, (2, 0, 1))


@jax.jit
def pallas_standalone__layernorm_linear__sampling_kernel(
    x: jax.Array,
    g: jax.Array,
    b: jax.Array,
    w: jax.Array,
):
    return _forward(CONFIG, x, g, b, w)
```

```python
import functools

import jax
import jax.numpy as jnp
from jax import lax
import jax.experimental.pallas as pl
import jax.experimental.pallas.tpu as pltpu

EPS = 1e-5
F32 = jnp.float32
BF16 = jnp.bfloat16
U32 = jnp.uint32

L = 128
H = 288
Q = 144
KH = 256
KS = 192
KM = 2 * KH
UNIT = 512
STEPS = 72

LONG = tuple("S%d%s" % (i, h) for i in range(1, 8) for h in "ab") + ("R1", "R6", "R7")
LEVEL2 = ("S2", "S3", "S4", "S5")
SHORT = tuple("%sm%d" % (p, k) for p in LEVEL2 for k in range(1, 8))
USES = {
    "S1": (("11", 1), ("22", 1)), "S2": (("21", 1), ("22", -1)),
    "S3": (("12", 1), ("22", 1)), "S4": (("11", 1), ("21", 1)),
    "S5": (("11", -1), ("12", 1)), "S6": (("22", 1),), "S7": (("11", 1),),
    "R1": (("12", 1), ("21", 1)), "R6": (("12", 1),), "R7": (("21", 1),),
    "D": (("21", 1), ("22", 1)),
}
TERMS = {"11": 4, "12": 4, "21": 5, "22": 5}
USES2 = {1: ((0, 0, 1), (1, 1, 1)), 2: ((1, 0, 1), (1, 1, -1)), 3: ((0, 1, 1), (1, 1, 1)),
         4: ((0, 0, 1), (1, 0, 1)), 5: ((0, 0, -1), (0, 1, 1)), 6: ((1, 1, 1),),
         7: ((0, 0, 1),)}
TERMS2 = {(0, 0): 4, (0, 1): 2, (1, 0): 2, (1, 1): 4}
TILE_ORDER = ((0, 0), (1, 0), (0, 1), (1, 1))

_ROWS = ("S4m1 S4m7 S4m6 S4m2", "S4m4 S4m3 S4m5 S2m1", "S2m6 S2m2 S2m4 S2m3",
         "S2m5 S2m7 S3m4 S3m2", "S3m5 S3m3 S3m1 S3m6", "A:D B:D S3m7 S5m1 S5m7 S5m6",
         "A:R7 B:R7 S5m2 S5m4", "S5m3 S5m5", "A:S1a A:S1b B:S1a B:S1b",
         "A:R1 B:R1 A:R6 B:R6", "A:S7a A:S7b B:S7a B:S7b", "A:S6a A:S6b B:S6a B:S6b")
_ROWS_COLD = ("A:S4a A:S4b A:S2a A:Q3a", "A:P3b A:S5a A:V3 A:D A:S2b A:R7",
              "A:S5b A:R1 A:R6 A:S1a", "A:S1b A:S7a A:S7b A:S6a", "A:S6b B:S4a B:S4b B:S2a",
              "B:S3a B:S3b B:S5a B:D B:S2b", "B:R7 B:S5b B:R1 B:R6",
              "B:S1a B:S1b B:S7a B:S7b", "B:S6a B:S6b")
_ROWS_COLD0 = ("A:S4a A:S4b A:Q3a A:Q3b", "B:P4a B:P4b B:P3a B:P3b",
               "A:V3 A:D A:R7 A:R1 A:R6 A:S1a", "A:S1b A:S7a A:S7b A:S6a",
               "A:S6b B:V4 B:V3 B:D B:R7 B:R1 B:R6", "S2m2 S2m4 S2m3 S2m5",
               "S2m6 S2m1 S2m7 S5m1", "S5m7 S5m6 S5m2 S5m4", "B:S1a B:S1b S5m3 S5m5",
               "B:S7a B:S7b B:S6a B:S6b")


def _schedule(rows, weights):
    out = []
    for row, steps in zip(rows, weights, strict=True):
        toks = row.split()
        passes = [t for t in toks if not (t.endswith(":D") or ":V" in t)]
        for t in toks:
            n = 0
            if t in passes:
                k = passes.index(t)
                n = steps * (k + 1) // len(passes) - steps * k // len(passes)
            out.append((t, n))
    return tuple(out)


CONFIG = dict(
    plan=((1, 1, False), (2, 1, False), (4, 1, True), (7, 1, True), (10, 5, True)),
    steady=_schedule(_ROWS, (12, 20, 36, 12, 20, 12, 24, 8, 24, 36, 32, 52)),
    warm=_schedule(_ROWS, (0, 28, 16, 12, 28, 20, 8, 32, 20, 36, 48, 40)),
    last=_schedule(_ROWS, (12, 36, 28, 12, 28, 20, 12, 16, 16, 28, 28, 52)),
    cold=(_schedule(_ROWS_COLD0, (0, 12, 44, 48, 20, 0, 8, 0, 12, 0)),
          _schedule(_ROWS_COLD, (0, 12, 60, 60, 40, 88, 64, 76, 32)),
          _schedule(_ROWS_COLD, (0, 36, 60, 36, 76, 64, 64, 84, 12))),
    gate_row=112,
    write_start=30,
    write_fine=48,
    bulk_slices=4,
    bulk_rows=24,
    bulk_per_unit=12,
    bulk_at=(4, 8, 20, 32, 36, 41),
)


def _pack(v):
    return pltpu.bitcast(v.astype(BF16), U32)


def _prep_first(g_ref, w_ref, ref, used, d_model, rows=16):
    g = g_ref[...].astype(F32).reshape(1, d_model)
    wt = jnp.concatenate([w_ref[0:L, :], w_ref[KH:KH + L, :]], axis=0).T
    keep = {}
    for r0 in range(0, H, rows):
        a11, a12, a21, a22 = [
            wt[h * H + r0:h * H + r0 + rows, k * L:(k + 1) * L].astype(F32)
            * g[:, k * KH:k * KH + L] for h in range(2) for k in range(2)]
        xs = (a11 + a22, a21 + a22, a11, a22, a11 + a12, a21 - a11, a12 - a22)
        for k in range(7):
            name = "S%da" % (k + 1)
            if name in used:
                ref[name][r0 // 2:(r0 + rows) // 2, :] = _pack(xs[k])
            keep[name, r0] = xs[k]
    for r0 in range(0, Q, rows):
        for p in LEVEL2:
            x11, x21 = keep[p + "a", r0], keep[p + "a", Q + r0]
            ref[p + "m3"][r0 // 2:(r0 + rows) // 2, :] = _pack(x11)
            ref[p + "m6"][r0 // 2:(r0 + rows) // 2, :] = _pack(x21 - x11)
    return keep


def _prep_rest(g_ref, b_ref, w_ref, ref, dl_ref, used, keep, d_model, rows=16):
    w = w_ref[...]
    g = g_ref[...].astype(F32).reshape(1, d_model)
    wt = jnp.concatenate([w[L:KH], w[KH + L:KM]], axis=0).T
    gt = jnp.concatenate([g[:, KM:d_model]] * 2, axis=1)
    at = jnp.concatenate([w[KM:d_model]] * 2, axis=0).T
    brow = jnp.broadcast_to(b_ref[...].astype(F32).reshape(1, d_model), (16, d_model))
    drow = jnp.dot(brow.astype(BF16), w, preferred_element_type=F32)
    row = lax.broadcasted_iota(jnp.int32, (16, d_model), 0)
    lo = drow - drow.astype(BF16).astype(F32)
    e = jnp.where(row == 0, drow, jnp.where(row == 1, lo, 0.0))
    z = jnp.zeros((48, d_model), F32)
    et = jnp.concatenate([e, z, e, z], axis=0).astype(BF16).T
    low = lax.broadcasted_iota(jnp.int32, (rows, L), 1) < 64

    def sel(p, q):
        return jnp.where(low, p, q)

    def level1(r0):
        a11, a12, a21, a22 = [
            wt[h * H + r0:h * H + r0 + rows, k * L:(k + 1) * L].astype(F32)
            * g[:, k * KH + L:(k + 1) * KH] for h in range(2) for k in range(2)]
        at1 = at[r0:r0 + rows].astype(F32) * gt
        at2 = at[H + r0:H + r0 + rows].astype(F32) * gt
        e1 = et[r0:r0 + rows].astype(F32)
        s2, s5, s6, s7 = a21 + a22, a11 + a12, a21 - a11, a12 - a22
        xs = (sel(a11 + a22, e1), sel(s2, -s2), sel(a11, a21), sel(a22, a12),
              sel(s5, -s5), sel(s6, at2), sel(s7, at1))
        res = {"S%db" % (k + 1): xs[k] for k in range(7)}
        res["R1"] = sel(e1, a21 + a12)
        res["R6"] = sel(at1, -s6)
        res["R7"] = sel(at2, -s7)
        for name in res:
            if name in used:
                ref[name][r0 // 2:(r0 + rows) // 2, :] = _pack(res[name])
        return res

    for r0 in range(0, Q, rows):
        u, v = level1(r0), level1(Q + r0)
        for p in LEVEL2:
            x11, x12 = keep[p + "a", r0], u[p + "b"]
            x21, x22 = keep[p + "a", Q + r0], v[p + "b"]
            xs = {1: x11 + x22, 2: x21 + x22, 4: x22, 5: x11 + x12, 7: x12 - x22}
            for k in xs:
                ref["%sm%d" % (p, k)][r0 // 2:(r0 + rows) // 2, :] = _pack(xs[k])
    low2 = lax.broadcasted_iota(jnp.int32, (H, L), 1) < 64
    lhs = jnp.where(low2, et[H:d_model].astype(F32), -et[0:H].astype(F32)).astype(BF16)
    dl_ref[...] = jnp.dot(lhs, jnp.ones((L, L), BF16), preferred_element_type=F32)


class _Stats:
    def __init__(self, x_ref, d_model, chains=1):
        self.x_ref, self.d_model = x_ref, d_model
        self.pos = 0
        self.x0 = None
        self.a1 = [None] * chains
        self.a2 = [None] * chains
        self.pending = []
        self.result = None

    def left(self):
        return STEPS - self.pos

    def advance(self, n):
        if self.x0 is None:
            self.x0 = self.x_ref[0:16, :].astype(F32)[0:1, :]
        for _ in range(n):
            if not self.pending:
                r0 = self.pos * 8
                t = self.x_ref[r0:r0 + 16, :].astype(F32) - self.x0
                self.pending = [t[0:8], t[8:16]]
            t = self.pending.pop(0)
            c = self.pos % len(self.a1)
            self.a1[c] = t if self.a1[c] is None else self.a1[c] + t
            self.a2[c] = t * t if self.a2[c] is None else self.a2[c] + t * t
            self.pos += 1
        return self.a2[0]

    def finish(self):
        if self.result is None:
            self.advance(self.left())
            a1 = functools.reduce(lambda u, v: u + v, self.a1)
            a2 = functools.reduce(lambda u, v: u + v, self.a2)
            s1 = jnp.sum(a1, axis=0, keepdims=True) * (1.0 / self.d_model)
            s2 = jnp.sum(a2, axis=0, keepdims=True) * (1.0 / self.d_model)
            var = jnp.maximum(s2 - s1 * s1, 0.0)
            self.result = (self.x0 + s1, lax.rsqrt(var + EPS))
        return self.result


def _signed_add(cur, v, sign):
    if cur is None:
        return v, sign
    val, cur_sign = cur
    if cur_sign == 1:
        return (val + v if sign == 1 else val - v), 1
    return (v - val, 1) if sign == 1 else (val + v, -1)


class _Unit:
    def __init__(self, xs_ref, os_ref, ref, dl_ref, c0, d_model, gate_row):
        self.xs_ref, self.os_ref, self.ref, self.dl_ref = xs_ref, os_ref, ref, dl_ref
        self.c0, self.d_model, self.gate_row = c0, d_model, gate_row
        self.stats = {}
        self.cache = {}
        self.queue = []
        self.on_store = None

    def col(self, pair, j):
        return self.c0 + (pair + 2 * j) * L

    def tile_stats(self, pair, j, chains=1):
        if (pair, j) not in self.stats:
            self.stats[pair, j] = _Stats(
                self.xs_ref.at[:, pl.ds(self.col(pair, j), L)], self.d_model, chains)
        return self.stats[pair, j]

    def norm(self, pair, j):
        return self.tile_stats(pair, j).finish()

    def x(self, pair, k, j, r0, r1):
        c = self.col(pair, j)
        return self.xs_ref[k * KH + r0:k * KH + r1, c:c + L].astype(F32)

    def hat(self, pair, k, j, r0, r1):
        m, r = self.norm(pair, j)
        return (self.x(pair, k, j, r0, r1) - m) * r

    def tail(self, pair, j):
        if ("tail", pair, j) not in self.cache:
            self.cache["tail", pair, j] = self.hat(pair, 2, j, 0, 64)
        return self.cache["tail", pair, j]

    def cross(self, pair, ka, kb, r0, r1):
        (ma, ra), (mb, rb) = self.norm(pair, 0), self.norm(pair, 1)
        if ("mr", pair) not in self.cache:
            self.cache["mr", pair] = ma * ra + mb * rb
        return (self.x(pair, ka, 0, r0, r1) * ra + self.x(pair, kb, 1, r0, r1) * rb
                - self.cache["mr", pair])

    def rhs(self, pair, name, raw=None):
        row = lax.broadcasted_iota(jnp.int32, (16, L), 0)
        ones = jnp.where(row < 2, 1.0, 0.0)

        def cat(*parts):
            return jnp.concatenate(parts, axis=0)

        if name == "R1":
            return cat(ones, jnp.zeros((48, L), F32), self.cross(pair, 0, 1, KS, KH))
        if name == "R6":
            return cat(self.tail(pair, 1), self.cross(pair, 0, 0, KS, KH))
        if name == "R7":
            return cat(self.tail(pair, 0), self.cross(pair, 1, 1, KS, KH))
        prod, r0 = name[:2], (0 if name[2] == "a" else L)
        if prod in ("S3", "S4"):
            j = 1 if prod == "S3" else 0
            diff = self.x(pair, 1 - j, j, r0, r0 + L) - self.x(pair, j, j, r0, r0 + L)
            if raw == "P":
                return diff
            if raw == "Q":
                return diff + jnp.minimum(self.norm(pair, 0)[1], 0.0)
            return diff * self.norm(pair, j)[1]
        main = {"S1": lambda a, b: self.cross(pair, 0, 1, a, b),
                "S2": lambda a, b: self.hat(pair, 0, 0, a, b),
                "S5": lambda a, b: self.hat(pair, 1, 1, a, b),
                "S6": lambda a, b: self.cross(pair, 0, 0, a, b),
                "S7": lambda a, b: self.cross(pair, 1, 1, a, b)}[prod]
        if r0 == 0:
            return main(0, L)
        rest = {"S1": lambda: ones,
                "S2": lambda: self.hat(pair, 1, 1, KS, KH),
                "S5": lambda: self.hat(pair, 0, 0, KS, KH),
                "S6": lambda: self.tail(pair, 1),
                "S7": lambda: self.tail(pair, 0)}[prod]
        return cat(main(L, KS), rest())

    def rhs2(self, prod, k):
        def h(kk, pair):
            if ("h", prod, kk, pair) not in self.cache:
                self.cache["h", prod, kk, pair] = self.rhs(pair, prod + "ab"[kk])
            return self.cache["h", prod, kk, pair]

        return {1: lambda: h(0, 0) + h(1, 1), 2: lambda: h(0, 0),
                3: lambda: h(0, 1) - h(1, 1), 4: lambda: h(1, 0) - h(0, 0),
                5: lambda: h(1, 1), 6: lambda: h(0, 0) + h(0, 1),
                7: lambda: h(1, 0) + h(1, 1)}[k]()

    def run(self, schedule, before_token):
        acc, count, done = {}, {}, {}
        acc2, count2, part = {}, {}, {}

        def add(pair, half, name, v):
            for key, sign in USES[name]:
                k = (pair, half, key)
                acc[k] = _signed_add(acc.get(k), v, sign)
                count[k] = count.get(k, 0) + 1
                if count[k] == TERMS[key]:
                    val, val_sign = acc[k]
                    assert val_sign == 1
                    done[k] = val
                    if (1 - pair, half, key) in done:
                        r0 = (0 if key[0] == "1" else H) + half * Q
                        c = self.col(0, int(key[1]) - 1)
                        both = jnp.concatenate(
                            [done[0, half, key], done[1, half, key]], axis=1)
                        self.os_ref[r0:r0 + Q, c:c + 2 * L] = both.astype(BF16)
                        if self.on_store is not None:
                            self.on_store(r0, c)

        def add_full(pair, name, v):
            add(pair, 0, name, v[0:Q])
            add(pair, 1, name, v[Q:H])

        for pos, (token, steps) in enumerate(schedule):
            before_token(pos)
            gate = None
            while steps > 0 and self.queue:
                n = min(steps, self.queue[0].left())
                gate = self.queue[0].advance(n)
                steps -= n
                if self.queue[0].left() == 0:
                    gate = jnp.broadcast_to(self.queue.pop(0).finish()[1], (8, L))

            def dot(name, q, gate=gate):
                if gate is not None:
                    g0 = self.gate_row if q.shape[0] > self.gate_row else 0
                    parts = [q[0:g0]] if g0 else []
                    parts.append(q[g0:g0 + 8] + jnp.minimum(gate, 0.0))
                    if g0 + 8 < q.shape[0]:
                        parts.append(q[g0 + 8:])
                    q = jnp.concatenate(parts, axis=0)
                p = pltpu.bitcast(self.ref[name][...], BF16)[:, 0:q.shape[0]]
                return jnp.dot(p, q.astype(BF16), preferred_element_type=F32)

            if ":" not in token:
                prod, k = token[:2], int(token[3])
                v = dot(token, self.rhs2(prod, k))
                for half, pair, sign in USES2[k]:
                    kk = (prod, half, pair)
                    acc2[kk] = _signed_add(acc2.get(kk), v, sign)
                    count2[kk] = count2.get(kk, 0) + 1
                    if count2[kk] == TERMS2[half, pair]:
                        val, val_sign = acc2[kk]
                        assert val_sign == 1
                        add(pair, half, prod, val)
                continue
            pair, name = "AB".index(token[0]), token[2:]
            if name == "D":
                add_full(pair, "D", self.dl_ref[...])
                continue
            if name[0] == "V":
                prod = "S" + name[1]
                scale = self.norm(pair, 1 if prod == "S3" else 0)[1]
                add_full(pair, prod, part.pop((pair, prod)) * scale)
                continue
            raw = name[0] if name[0] in "PQ" else None
            name = "S" + name[1:] if raw else name
            v = dot(name, self.rhs(pair, name, raw))
            prod = name[:2]
            if prod[0] == "R":
                add_full(pair, prod, v)
            elif (pair, prod) not in part:
                part[pair, prod] = v
            elif raw:
                part[pair, prod] = v + part[pair, prod]
            else:
                add_full(pair, prod, v + part.pop((pair, prod)))
        assert len(done) == 16


def _forward(cfg, x, g, b, w):
    B, S, D = x.shape
    assert D == 2 * H == KM + 64 == 8 * STEPS
    plan = cfg["plan"]
    ups = B // UNIT
    n_units = S * ups
    assert sum(u * n for u, n, _ in plan) == n_units
    n_chunks = sum(n for _, n, _ in plan)
    names = LONG + SHORT
    used = {t[2:].replace("P", "S").replace("Q", "S")
            for sched in (cfg["steady"], *cfg["cold"]) for t, _ in sched if ":" in t}
    fine, per_unit = cfg["write_fine"], cfg["bulk_per_unit"]
    gs, rb = cfg["bulk_slices"], cfg["bulk_rows"]
    nrb = D // rb

    assert nrb == 2 * per_unit and gs * ups == 8
    per_slot = per_unit // len(cfg["bulk_at"])
    assert per_slot * len(cfg["bulk_at"]) == per_unit

    def issued(u, lo=jnp.minimum, hi=jnp.maximum):
        def ready(v):
            return 2 * (lo(v, fine) >> 3)
        n = lo(lo(u - cfg["write_start"] + 1, ready(u)), ready(u - 1) + 1)
        return hi(n, 0)

    loop_start = sum(u * n for u, n, _ in plan[:-1])
    table = {u: issued(u, min, max) for u in range(loop_start - 1, n_units)}
    assert table[loop_start - 1] == 0 and fine >= loop_start and fine % (gs * ups) == 0
    assert all(0 <= table[u] - table[u - 1] <= 1 for u in range(loop_start, n_units))
    assert all(table[u] <= 2 * (u // (gs * ups)) for u in table)
    assert table[n_units - 1] == 2 * fine // (gs * ups)
    assert all(n == 1 for _, n, _ in plan[:-1]) and plan[-1][2] and plan[-2][2]

    xt = jnp.transpose(x, (1, 2, 0))

    def kernel(x_hbm, g_hbm, b_hbm, w_hbm, o_hbm, xbuf, obuf, wbuf, gbuf, bbuf, *rest):
        ref = dict(zip(names, rest))
        dl_ref, isem, nsem, osem, wsem = rest[len(names):]

        def copies(sem, u, end, shift=0):
            res = []
            while u < end:
                s, r = divmod(u, ups)
                if r == 0 and end - u >= ups:
                    idx = (pl.ds(s + shift, (end - u) // ups), slice(None), pl.ds(0, B))
                    u += (end - u) // ups * ups
                else:
                    idx = (s + shift, slice(None), pl.ds(r * UNIT, UNIT))
                    u += 1
                res.append(pltpu.make_async_copy(x_hbm.at[idx], xbuf.at[idx], sem))
            return res

        def write_back(*idx):
            pltpu.make_async_copy(obuf.at[idx], o_hbm.at[idx], osem.at[0]).start()

        def w_rows(r0, r1, k):
            rows = pl.ds(r0, r1 - r0)
            return pltpu.make_async_copy(w_hbm.at[rows], wbuf.at[rows], wsem.at[k])

        cg = pltpu.make_async_copy(g_hbm, gbuf, wsem.at[1])
        cb = pltpu.make_async_copy(b_hbm, bbuf, wsem.at[2])
        w_first = [w_rows(0, L, 0), w_rows(KH, KH + L, 0)]
        w_rest = [w_rows(L, KH, 3), w_rows(KH + L, D, 3)]
        for c in [cg, cb] + w_first + w_rest:
            c.start()
        cg.wait()
        cb.wait()
        j = u0 = 0
        handed = False
        for nu, count, hand in plan:
            for _ in range(count):
                for c in copies(isem.at[j], u0 + handed, u0 + nu):
                    c.start()
                if hand and u0 + nu < n_units:
                    for c in copies(nsem.at[j], u0 + nu, u0 + nu + 1):
                        c.start()
                j += 1
                u0 += nu
                handed = hand
        for c in w_first:
            c.wait()
        keep = _prep_first(gbuf, wbuf, ref, used, D)
        for c in w_rest:
            c.wait()
        _prep_rest(gbuf, bbuf, wbuf, ref, dl_ref, used, keep, D)

        def make_unit(s, c0):
            return _Unit(xbuf.at[s], obuf.at[s], ref, dl_ref, c0, D, cfg["gate_row"])

        def do_chunk(j, u0, nu, shift, stats_in, hand, in_loop):
            for c in copies(isem.at[j], u0 + (stats_in is not None), u0 + nu, shift):
                c.wait()
            if hand:
                s_next, r_next = divmod(u0 + nu, ups)
                if in_loop:
                    exists = s_next + shift < S
                    s_next = jnp.minimum(s_next + shift, S - 1)

                    @pl.when(exists)
                    def _():
                        copies(nsem.at[j], r_next, r_next + 1, s_next)[0].wait()
                else:
                    copies(nsem.at[j], u0 + nu, u0 + nu + 1)[0].wait()
            where = [(u // ups + shift, (u % ups) * UNIT) for u in range(u0, u0 + nu)]
            units = [make_unit(s, c0) for s, c0 in where]
            if stats_in is None:
                units[0].tile_stats(0, 0, chains=2)
                units[0].queue = [units[0].tile_stats(1, 0), units[0].tile_stats(1, 1)]
            else:
                for n, key in enumerate(TILE_ORDER[1:]):
                    units[0].tile_stats(*key).result = stats_in[2 * n:2 * n + 2]
                head = units[0].tile_stats(*TILE_ORDER[0])
                head.x0, head.a1, head.a2 = stats_in[6], [stats_in[7]], [stats_in[8]]
                head.pos = STEPS
            for p in range(nu - 1):
                units[p].queue += [units[p + 1].tile_stats(*key) for key in TILE_ORDER]
            if hand:
                ahead = make_unit(s_next, r_next * UNIT)
                units[-1].queue += [ahead.tile_stats(*key)
                                    for key in TILE_ORDER[1:] + TILE_ORDER[:1]]

            for p, (s, c0) in enumerate(where):
                if p == 0:
                    schedule = cfg["cold"][j] if stats_in is None else cfg["warm"]
                else:
                    schedule = cfg["last"] if (hand and p == nu - 1) else cfg["steady"]
                if not in_loop:
                    units[p].run(schedule, lambda pos: None)
                    continue
                u = u0 + p + shift * ups
                k0, k1 = issued(u - 1), issued(u)

                def delayed(pos, k0=k0, k1=k1):
                    if pos in cfg["bulk_at"]:
                        first = cfg["bulk_at"].index(pos) * per_slot
                        for i in range(first, first + per_slot):
                            row = (k0 & 1) * (per_unit * rb) + i * rb
                            pl.when(k0 < k1)(functools.partial(
                                write_back, pl.ds((k0 >> 1) * gs, gs),
                                pl.ds(pl.multiple_of(row, 8), rb)))

                now = u >= fine
                if p == nu - 1:
                    now = now & (u < n_units - 1)

                    def on_store(r0, c, s=s, u=u):
                        pl.when(u == n_units - 1)(functools.partial(
                            write_back, s, pl.ds(r0, Q), pl.ds(c, 2 * L)))
                    units[p].on_store = on_store
                units[p].run(schedule, delayed)

                @pl.when(now)
                def _(s=s, c0=c0):
                    for c in range(c0, c0 + UNIT, L):
                        write_back(s, slice(None), pl.ds(c, L))

            if not hand:
                return None
            head = ahead.tile_stats(*TILE_ORDER[0])
            assert head.left() == 0
            return (*[v for key in TILE_ORDER[1:] for v in ahead.norm(*key)],
                    head.x0, head.a1[0], head.a2[0])

        j = u0 = 0
        stats = None
        for nu, count, hand in plan:
            if count == 1:
                stats = do_chunk(j, u0, nu, 0, stats, hand, False)
            else:
                assert nu % ups == 0 and u0 % ups == 0

                def body(it, carry, j=j, u0=u0, nu=nu):
                    return do_chunk(j + it, u0, nu, it * (nu // ups), carry, True, True)
                lax.fori_loop(0, count, body, stats)
            j += count
            u0 += nu * count
        pltpu.make_async_copy(obuf, o_hbm, osem.at[0]).wait()

    out = pl.pallas_call(
        kernel,
        in_specs=[pl.BlockSpec(memory_space=pl.ANY)] * 4,
        out_specs=pl.BlockSpec(memory_space=pl.ANY),
        out_shape=jax.ShapeDtypeStruct((S, D, B), x.dtype),
        scratch_shapes=[
            pltpu.VMEM((S, D, B + 2 * L), BF16),
            pltpu.VMEM((S, D, B), BF16),
            pltpu.VMEM((D, D), BF16),
            pltpu.VMEM((D,), BF16),
            pltpu.VMEM((D,), BF16),
            *[pltpu.VMEM(((H if n in LONG else Q) // 2, L), U32) for n in names],
            pltpu.VMEM((H, L), F32),
            pltpu.SemaphoreType.DMA((n_chunks,)),
            pltpu.SemaphoreType.DMA((n_chunks,)),
            pltpu.SemaphoreType.DMA((1,)),
            pltpu.SemaphoreType.DMA((4,)),
        ],
        compiler_params=pltpu.CompilerParams(
            vmem_limit_bytes=110 * 1024 * 1024,
            disable_bounds_checks=True,
            disable_semaphore_checks=True,
        ),
    )(xt, g, b, w)
    return jnp.transpose(out, (2, 0, 1))


@jax.jit
def pallas_standalone__layernorm_linear__sampling_kernel(
    x: jax.Array,
    g: jax.Array,
    b: jax.Array,
    w: jax.Array,
):
    return _forward(CONFIG, x, g, b, w)
```

```python
import functools

import jax
import jax.numpy as jnp
from jax import lax
import jax.experimental.pallas as pl
import jax.experimental.pallas.tpu as pltpu

EPS = 1e-5
F32 = jnp.float32
BF16 = jnp.bfloat16
U32 = jnp.uint32

L = 128
H = 288
Q = 144
KH = 256
KS = 192
KM = 2 * KH
UNIT = 512
STEPS = 72

LONG = tuple("S%d%s" % (i, h) for i in range(1, 8) for h in "ab") + ("R1", "R6", "R7")
LEVEL2 = ("S2", "S3", "S4", "S5")
SHORT = tuple("%sm%d" % (p, k) for p in LEVEL2 for k in range(1, 8))
USES = {
    "S1": (("11", 1), ("22", 1)), "S2": (("21", 1), ("22", -1)),
    "S3": (("12", 1), ("22", 1)), "S4": (("11", 1), ("21", 1)),
    "S5": (("11", -1), ("12", 1)), "S6": (("22", 1),), "S7": (("11", 1),),
    "R1": (("12", 1), ("21", 1)), "R6": (("12", 1),), "R7": (("21", 1),),
    "D": (("21", 1), ("22", 1)),
}
TERMS = {"11": 4, "12": 4, "21": 5, "22": 5}
USES2 = {1: ((0, 0, 1), (1, 1, 1)), 2: ((1, 0, 1), (1, 1, -1)), 3: ((0, 1, 1), (1, 1, 1)),
         4: ((0, 0, 1), (1, 0, 1)), 5: ((0, 0, -1), (0, 1, 1)), 6: ((1, 1, 1),),
         7: ((0, 0, 1),)}
TERMS2 = {(0, 0): 4, (0, 1): 2, (1, 0): 2, (1, 1): 4}
TILE_ORDER = ((0, 0), (1, 0), (0, 1), (1, 1))

_ROWS = ("S4m1 S4m7 S4m6 S4m2", "S4m4 S4m3 S4m5 S2m1", "S2m6 S2m2 S2m4 S2m3",
         "S2m5 S2m7 S3m4 S3m2", "S3m5 S3m3 S3m1 S3m6", "A:D B:D S3m7 S5m1 S5m7 S5m6",
         "A:R7 B:R7 S5m2 S5m4", "S5m3 S5m5", "A:S1a A:S1b B:S1a B:S1b",
         "A:R1 B:R1 A:R6 B:R6", "A:S7a A:S7b B:S7a B:S7b", "A:S6a A:S6b B:S6a B:S6b")
_ROWS_COLD = ("A:D A:S1a A:S1b A:R7 A:R1", "A:R6 A:S7a A:S7b A:S6a", "S4m1 S4m7 S4m6 S4m2",
              "S4m4 S4m3 S4m5 S2m1", "S2m6 S2m2 S2m4 S2m3", "S2m5 S2m7 S3m4 S3m2",
              "S3m5 S3m3 S3m1 S3m6", "B:D S3m7 S5m1 S5m7 S5m6", "A:S6b B:R7 S5m2 S5m4",
              "S5m3 S5m5", "B:S1a B:S1b B:R1 B:R6", "B:S7a B:S7b B:S6a B:S6b")
_ROWS_COLD0 = ("A:S4a A:S4b A:Q3a A:Q3b", "B:P4a B:P4b B:P3a B:P3b",
               "A:V3 A:D A:R7 A:R1 A:R6 A:S1a", "A:S1b A:S7a A:S7b A:S6a",
               "A:S6b B:V4 B:V3 B:D B:R7 B:R1 B:R6", "S2m2 S2m4 S2m3 S2m5",
               "S2m6 S2m1 S2m7 S5m1", "S5m7 S5m6 S5m2 S5m4", "B:S1a B:S1b S5m3 S5m5",
               "B:S7a B:S7b B:S6a B:S6b")


def _schedule(rows, weights):
    out = []
    for row, steps in zip(rows, weights, strict=True):
        toks = row.split()
        passes = [t for t in toks if not (t.endswith(":D") or ":V" in t)]
        for t in toks:
            n = 0
            if t in passes:
                k = passes.index(t)
                n = steps * (k + 1) // len(passes) - steps * k // len(passes)
            out.append((t, n))
    return tuple(out)


CONFIG = dict(
    plan=((1, 1, False), (2, 1, False), (4, 1, True), (7, 1, True), (10, 5, True)),
    steady=_schedule(_ROWS, (12, 20, 36, 12, 20, 12, 24, 8, 24, 36, 32, 52)),
    warm=_schedule(_ROWS, (0, 28, 16, 12, 28, 20, 8, 32, 20, 36, 48, 40)),
    last=_schedule(_ROWS, (12, 36, 28, 12, 28, 20, 12, 16, 16, 28, 28, 52)),
    cold=(_schedule(_ROWS_COLD0, (0, 16, 0, 32, 0, 4, 56, 4, 0, 32)),
          _schedule(_ROWS_COLD, (0, 60, 64, 20, 36, 36, 28, 16, 28, 16, 52, 76)),
          _schedule(_ROWS_COLD, (0, 56, 64, 20, 28, 24, 20, 40, 28, 24, 56, 72))),
    gate_row=112,
    write_start=30,
    write_fine=48,
    bulk_slices=4,
    bulk_rows=24,
    bulk_per_unit=12,
    bulk_at=(4, 8, 20, 32, 36, 41),
)


def _pack(v):
    return pltpu.bitcast(v.astype(BF16), U32)


def _prep_first(g_ref, w_ref, ref, used, d_model, rows=16):
    g = g_ref[...].astype(F32).reshape(1, d_model)
    wt = jnp.concatenate([w_ref[0:L, :], w_ref[KH:KH + L, :]], axis=0).T
    keep = {}
    for r0 in range(0, H, rows):
        a11, a12, a21, a22 = [
            wt[h * H + r0:h * H + r0 + rows, k * L:(k + 1) * L].astype(F32)
            * g[:, k * KH:k * KH + L] for h in range(2) for k in range(2)]
        xs = (a11 + a22, a21 + a22, a11, a22, a11 + a12, a21 - a11, a12 - a22)
        for k in range(7):
            name = "S%da" % (k + 1)
            if name in used:
                ref[name][r0 // 2:(r0 + rows) // 2, :] = _pack(xs[k])
            keep[name, r0] = xs[k]
    for r0 in range(0, Q, rows):
        for p in LEVEL2:
            x11, x21 = keep[p + "a", r0], keep[p + "a", Q + r0]
            ref[p + "m3"][r0 // 2:(r0 + rows) // 2, :] = _pack(x11)
            ref[p + "m6"][r0 // 2:(r0 + rows) // 2, :] = _pack(x21 - x11)
    return keep


def _prep_rest(g_ref, b_ref, w_ref, ref, dl_ref, used, keep, d_model, rows=16):
    w = w_ref[...]
    g = g_ref[...].astype(F32).reshape(1, d_model)
    wt = jnp.concatenate([w[L:KH], w[KH + L:KM]], axis=0).T
    gt = jnp.concatenate([g[:, KM:d_model]] * 2, axis=1)
    at = jnp.concatenate([w[KM:d_model]] * 2, axis=0).T
    brow = jnp.broadcast_to(b_ref[...].astype(F32).reshape(1, d_model), (16, d_model))
    drow = jnp.dot(brow.astype(BF16), w, preferred_element_type=F32)
    row = lax.broadcasted_iota(jnp.int32, (16, d_model), 0)
    lo = drow - drow.astype(BF16).astype(F32)
    e = jnp.where(row == 0, drow, jnp.where(row == 1, lo, 0.0))
    z = jnp.zeros((48, d_model), F32)
    et = jnp.concatenate([e, z, e, z], axis=0).astype(BF16).T
    low = lax.broadcasted_iota(jnp.int32, (rows, L), 1) < 64

    def sel(p, q):
        return jnp.where(low, p, q)

    def level1(r0):
        a11, a12, a21, a22 = [
            wt[h * H + r0:h * H + r0 + rows, k * L:(k + 1) * L].astype(F32)
            * g[:, k * KH + L:(k + 1) * KH] for h in range(2) for k in range(2)]
        at1 = at[r0:r0 + rows].astype(F32) * gt
        at2 = at[H + r0:H + r0 + rows].astype(F32) * gt
        e1 = et[r0:r0 + rows].astype(F32)
        s2, s5, s6, s7 = a21 + a22, a11 + a12, a21 - a11, a12 - a22
        xs = (sel(a11 + a22, e1), sel(s2, -s2), sel(a11, a21), sel(a22, a12),
              sel(s5, -s5), sel(s6, at2), sel(s7, at1))
        res = {"S%db" % (k + 1): xs[k] for k in range(7)}
        res["R1"] = sel(e1, a21 + a12)
        res["R6"] = sel(at1, -s6)
        res["R7"] = sel(at2, -s7)
        for name in res:
            if name in used:
                ref[name][r0 // 2:(r0 + rows) // 2, :] = _pack(res[name])
        return res

    for r0 in range(0, Q, rows):
        u, v = level1(r0), level1(Q + r0)
        for p in LEVEL2:
            x11, x12 = keep[p + "a", r0], u[p + "b"]
            x21, x22 = keep[p + "a", Q + r0], v[p + "b"]
            xs = {1: x11 + x22, 2: x21 + x22, 4: x22, 5: x11 + x12, 7: x12 - x22}
            for k in xs:
                ref["%sm%d" % (p, k)][r0 // 2:(r0 + rows) // 2, :] = _pack(xs[k])
    low2 = lax.broadcasted_iota(jnp.int32, (H, L), 1) < 64
    lhs = jnp.where(low2, et[H:d_model].astype(F32), -et[0:H].astype(F32)).astype(BF16)
    dl_ref[...] = jnp.dot(lhs, jnp.ones((L, L), BF16), preferred_element_type=F32)


class _Stats:
    def __init__(self, x_ref, d_model, chains=1):
        self.x_ref, self.d_model = x_ref, d_model
        self.pos = 0
        self.x0 = None
        self.a1 = [None] * chains
        self.a2 = [None] * chains
        self.pending = []
        self.result = None

    def left(self):
        return STEPS - self.pos

    def advance(self, n):
        if self.x0 is None:
            self.x0 = self.x_ref[0:16, :].astype(F32)[0:1, :]
        for _ in range(n):
            if not self.pending:
                r0 = self.pos * 8
                t = self.x_ref[r0:r0 + 16, :].astype(F32) - self.x0
                self.pending = [t[0:8], t[8:16]]
            t = self.pending.pop(0)
            c = self.pos % len(self.a1)
            self.a1[c] = t if self.a1[c] is None else self.a1[c] + t
            self.a2[c] = t * t if self.a2[c] is None else self.a2[c] + t * t
            self.pos += 1
        return self.a2[0]

    def finish(self):
        if self.result is None:
            self.advance(self.left())
            a1 = functools.reduce(lambda u, v: u + v, self.a1)
            a2 = functools.reduce(lambda u, v: u + v, self.a2)
            s1 = jnp.sum(a1, axis=0, keepdims=True) * (1.0 / self.d_model)
            s2 = jnp.sum(a2, axis=0, keepdims=True) * (1.0 / self.d_model)
            var = jnp.maximum(s2 - s1 * s1, 0.0)
            self.result = (self.x0 + s1, lax.rsqrt(var + EPS))
        return self.result


def _signed_add(cur, v, sign):
    if cur is None:
        return v, sign
    val, cur_sign = cur
    if cur_sign == 1:
        return (val + v if sign == 1 else val - v), 1
    return (v - val, 1) if sign == 1 else (val + v, -1)


class _Unit:
    def __init__(self, xs_ref, os_ref, ref, dl_ref, c0, d_model, gate_row):
        self.xs_ref, self.os_ref, self.ref, self.dl_ref = xs_ref, os_ref, ref, dl_ref
        self.c0, self.d_model, self.gate_row = c0, d_model, gate_row
        self.stats = {}
        self.cache = {}
        self.queue = []
        self.on_store = None

    def col(self, pair, j):
        return self.c0 + (pair + 2 * j) * L

    def tile_stats(self, pair, j, chains=1):
        if (pair, j) not in self.stats:
            self.stats[pair, j] = _Stats(
                self.xs_ref.at[:, pl.ds(self.col(pair, j), L)], self.d_model, chains)
        return self.stats[pair, j]

    def norm(self, pair, j):
        return self.tile_stats(pair, j).finish()

    def x(self, pair, k, j, r0, r1):
        c = self.col(pair, j)
        return self.xs_ref[k * KH + r0:k * KH + r1, c:c + L].astype(F32)

    def hat(self, pair, k, j, r0, r1):
        m, r = self.norm(pair, j)
        return (self.x(pair, k, j, r0, r1) - m) * r

    def tail(self, pair, j):
        if ("tail", pair, j) not in self.cache:
            self.cache["tail", pair, j] = self.hat(pair, 2, j, 0, 64)
        return self.cache["tail", pair, j]

    def cross(self, pair, ka, kb, r0, r1):
        (ma, ra), (mb, rb) = self.norm(pair, 0), self.norm(pair, 1)
        if ("mr", pair) not in self.cache:
            self.cache["mr", pair] = ma * ra + mb * rb
        return (self.x(pair, ka, 0, r0, r1) * ra + self.x(pair, kb, 1, r0, r1) * rb
                - self.cache["mr", pair])

    def rhs(self, pair, name, raw=None):
        row = lax.broadcasted_iota(jnp.int32, (16, L), 0)
        ones = jnp.where(row < 2, 1.0, 0.0)

        def cat(*parts):
            return jnp.concatenate(parts, axis=0)

        if name == "R1":
            return cat(ones, jnp.zeros((48, L), F32), self.cross(pair, 0, 1, KS, KH))
        if name == "R6":
            return cat(self.tail(pair, 1), self.cross(pair, 0, 0, KS, KH))
        if name == "R7":
            return cat(self.tail(pair, 0), self.cross(pair, 1, 1, KS, KH))
        prod, r0 = name[:2], (0 if name[2] == "a" else L)
        if prod in ("S3", "S4"):
            j = 1 if prod == "S3" else 0
            diff = self.x(pair, 1 - j, j, r0, r0 + L) - self.x(pair, j, j, r0, r0 + L)
            if raw == "P":
                return diff
            if raw == "Q":
                return diff + jnp.minimum(self.norm(pair, 0)[1], 0.0)
            return diff * self.norm(pair, j)[1]
        main = {"S1": lambda a, b: self.cross(pair, 0, 1, a, b),
                "S2": lambda a, b: self.hat(pair, 0, 0, a, b),
                "S5": lambda a, b: self.hat(pair, 1, 1, a, b),
                "S6": lambda a, b: self.cross(pair, 0, 0, a, b),
                "S7": lambda a, b: self.cross(pair, 1, 1, a, b)}[prod]
        if r0 == 0:
            return main(0, L)
        rest = {"S1": lambda: ones,
                "S2": lambda: self.hat(pair, 1, 1, KS, KH),
                "S5": lambda: self.hat(pair, 0, 0, KS, KH),
                "S6": lambda: self.tail(pair, 1),
                "S7": lambda: self.tail(pair, 0)}[prod]
        return cat(main(L, KS), rest())

    def rhs2(self, prod, k):
        def h(kk, pair):
            if ("h", prod, kk, pair) not in self.cache:
                self.cache["h", prod, kk, pair] = self.rhs(pair, prod + "ab"[kk])
            return self.cache["h", prod, kk, pair]

        return {1: lambda: h(0, 0) + h(1, 1), 2: lambda: h(0, 0),
                3: lambda: h(0, 1) - h(1, 1), 4: lambda: h(1, 0) - h(0, 0),
                5: lambda: h(1, 1), 6: lambda: h(0, 0) + h(0, 1),
                7: lambda: h(1, 0) + h(1, 1)}[k]()

    def run(self, schedule, before_token):
        acc, count, done = {}, {}, {}
        acc2, count2, part = {}, {}, {}

        def add(pair, half, name, v):
            for key, sign in USES[name]:
                k = (pair, half, key)
                acc[k] = _signed_add(acc.get(k), v, sign)
                count[k] = count.get(k, 0) + 1
                if count[k] == TERMS[key]:
                    val, val_sign = acc[k]
                    assert val_sign == 1
                    done[k] = val
                    if (1 - pair, half, key) in done:
                        r0 = (0 if key[0] == "1" else H) + half * Q
                        c = self.col(0, int(key[1]) - 1)
                        both = jnp.concatenate(
                            [done[0, half, key], done[1, half, key]], axis=1)
                        self.os_ref[r0:r0 + Q, c:c + 2 * L] = both.astype(BF16)
                        if self.on_store is not None:
                            self.on_store(r0, c)

        def add_full(pair, name, v):
            add(pair, 0, name, v[0:Q])
            add(pair, 1, name, v[Q:H])

        for pos, (token, steps) in enumerate(schedule):
            before_token(pos)
            gate = None
            while steps > 0 and self.queue:
                n = min(steps, self.queue[0].left())
                gate = self.queue[0].advance(n)
                steps -= n
                if self.queue[0].left() == 0:
                    gate = jnp.broadcast_to(self.queue.pop(0).finish()[1], (8, L))

            def dot(name, q, gate=gate):
                if gate is not None:
                    g0 = self.gate_row if q.shape[0] > self.gate_row else 0
                    parts = [q[0:g0]] if g0 else []
                    parts.append(q[g0:g0 + 8] + jnp.minimum(gate, 0.0))
                    if g0 + 8 < q.shape[0]:
                        parts.append(q[g0 + 8:])
                    q = jnp.concatenate(parts, axis=0)
                p = pltpu.bitcast(self.ref[name][...], BF16)[:, 0:q.shape[0]]
                return jnp.dot(p, q.astype(BF16), preferred_element_type=F32)

            if ":" not in token:
                prod, k = token[:2], int(token[3])
                v = dot(token, self.rhs2(prod, k))
                for half, pair, sign in USES2[k]:
                    kk = (prod, half, pair)
                    acc2[kk] = _signed_add(acc2.get(kk), v, sign)
                    count2[kk] = count2.get(kk, 0) + 1
                    if count2[kk] == TERMS2[half, pair]:
                        val, val_sign = acc2[kk]
                        assert val_sign == 1
                        add(pair, half, prod, val)
                continue
            pair, name = "AB".index(token[0]), token[2:]
            if name == "D":
                add_full(pair, "D", self.dl_ref[...])
                continue
            if name[0] == "V":
                prod = "S" + name[1]
                scale = self.norm(pair, 1 if prod == "S3" else 0)[1]
                add_full(pair, prod, part.pop((pair, prod)) * scale)
                continue
            raw = name[0] if name[0] in "PQ" else None
            name = "S" + name[1:] if raw else name
            v = dot(name, self.rhs(pair, name, raw))
            prod = name[:2]
            if prod[0] == "R":
                add_full(pair, prod, v)
            elif (pair, prod) not in part:
                part[pair, prod] = v
            elif raw:
                part[pair, prod] = v + part[pair, prod]
            else:
                add_full(pair, prod, v + part.pop((pair, prod)))
        assert len(done) == 16


def _forward(cfg, x, g, b, w):
    B, S, D = x.shape
    assert D == 2 * H == KM + 64 == 8 * STEPS
    plan = cfg["plan"]
    ups = B // UNIT
    n_units = S * ups
    assert sum(u * n for u, n, _ in plan) == n_units
    n_chunks = sum(n for _, n, _ in plan)
    names = LONG + SHORT
    used = {t[2:].replace("P", "S").replace("Q", "S")
            for sched in (cfg["steady"], *cfg["cold"]) for t, _ in sched if ":" in t}
    fine, per_unit = cfg["write_fine"], cfg["bulk_per_unit"]
    gs, rb = cfg["bulk_slices"], cfg["bulk_rows"]
    nrb = D // rb

    assert nrb == 2 * per_unit and gs * ups == 8
    per_slot = per_unit // len(cfg["bulk_at"])
    assert per_slot * len(cfg["bulk_at"]) == per_unit

    def issued(u, lo=jnp.minimum, hi=jnp.maximum):
        def ready(v):
            return 2 * (lo(v, fine) >> 3)
        n = lo(lo(u - cfg["write_start"] + 1, ready(u)), ready(u - 1) + 1)
        return hi(n, 0)

    loop_start = sum(u * n for u, n, _ in plan[:-1])
    table = {u: issued(u, min, max) for u in range(loop_start - 1, n_units)}
    assert table[loop_start - 1] == 0 and fine >= loop_start and fine % (gs * ups) == 0
    assert all(0 <= table[u] - table[u - 1] <= 1 for u in range(loop_start, n_units))
    assert all(table[u] <= 2 * (u // (gs * ups)) for u in table)
    assert table[n_units - 1] == 2 * fine // (gs * ups)
    assert all(n == 1 for _, n, _ in plan[:-1]) and plan[-1][2] and plan[-2][2]

    xt = jnp.transpose(x, (1, 2, 0))

    def kernel(x_hbm, g_hbm, b_hbm, w_hbm, o_hbm, xbuf, obuf, wbuf, gbuf, bbuf, *rest):
        ref = dict(zip(names, rest))
        dl_ref, isem, nsem, osem, wsem = rest[len(names):]

        def copies(sem, u, end, shift=0):
            res = []
            while u < end:
                s, r = divmod(u, ups)
                if r == 0 and end - u >= ups:
                    idx = (pl.ds(s + shift, (end - u) // ups), slice(None), pl.ds(0, B))
                    u += (end - u) // ups * ups
                else:
                    idx = (s + shift, slice(None), pl.ds(r * UNIT, UNIT))
                    u += 1
                res.append(pltpu.make_async_copy(x_hbm.at[idx], xbuf.at[idx], sem))
            return res

        def write_back(*idx):
            pltpu.make_async_copy(obuf.at[idx], o_hbm.at[idx], osem.at[0]).start()

        def w_rows(r0, r1, k):
            rows = pl.ds(r0, r1 - r0)
            return pltpu.make_async_copy(w_hbm.at[rows], wbuf.at[rows], wsem.at[k])

        cg = pltpu.make_async_copy(g_hbm, gbuf, wsem.at[1])
        cb = pltpu.make_async_copy(b_hbm, bbuf, wsem.at[2])
        w_first = [w_rows(0, L, 0), w_rows(KH, KH + L, 0)]
        w_rest = [w_rows(L, KH, 3), w_rows(KH + L, D, 3)]
        for c in [cg, cb] + w_first + w_rest:
            c.start()
        cg.wait()
        cb.wait()
        j = u0 = 0
        handed = False
        for nu, count, hand in plan:
            for _ in range(count):
                for c in copies(isem.at[j], u0 + handed, u0 + nu):
                    c.start()
                if hand and u0 + nu < n_units:
                    for c in copies(nsem.at[j], u0 + nu, u0 + nu + 1):
                        c.start()
                j += 1
                u0 += nu
                handed = hand
        for c in w_first:
            c.wait()
        keep = _prep_first(gbuf, wbuf, ref, used, D)
        for c in w_rest:
            c.wait()
        _prep_rest(gbuf, bbuf, wbuf, ref, dl_ref, used, keep, D)

        def make_unit(s, c0):
            return _Unit(xbuf.at[s], obuf.at[s], ref, dl_ref, c0, D, cfg["gate_row"])

        def do_chunk(j, u0, nu, shift, stats_in, hand, in_loop):
            for c in copies(isem.at[j], u0 + (stats_in is not None), u0 + nu, shift):
                c.wait()
            if hand:
                s_next, r_next = divmod(u0 + nu, ups)
                if in_loop:
                    exists = s_next + shift < S
                    s_next = jnp.minimum(s_next + shift, S - 1)

                    @pl.when(exists)
                    def _():
                        copies(nsem.at[j], r_next, r_next + 1, s_next)[0].wait()
                else:
                    copies(nsem.at[j], u0 + nu, u0 + nu + 1)[0].wait()
            where = [(u // ups + shift, (u % ups) * UNIT) for u in range(u0, u0 + nu)]
            units = [make_unit(s, c0) for s, c0 in where]
            if stats_in is None:
                units[0].tile_stats(0, 0, chains=2)
                units[0].queue = [units[0].tile_stats(1, 0), units[0].tile_stats(1, 1)]
            else:
                for n, key in enumerate(TILE_ORDER[1:]):
                    units[0].tile_stats(*key).result = stats_in[2 * n:2 * n + 2]
                head = units[0].tile_stats(*TILE_ORDER[0])
                head.x0, head.a1, head.a2 = stats_in[6], [stats_in[7]], [stats_in[8]]
                head.pos = STEPS
            for p in range(nu - 1):
                units[p].queue += [units[p + 1].tile_stats(*key) for key in TILE_ORDER]
            if hand:
                ahead = make_unit(s_next, r_next * UNIT)
                units[-1].queue += [ahead.tile_stats(*key)
                                    for key in TILE_ORDER[1:] + TILE_ORDER[:1]]

            for p, (s, c0) in enumerate(where):
                if p == 0:
                    schedule = cfg["cold"][j] if stats_in is None else cfg["warm"]
                else:
                    schedule = cfg["last"] if (hand and p == nu - 1) else cfg["steady"]
                if not in_loop:
                    units[p].run(schedule, lambda pos: None)
                    continue
                u = u0 + p + shift * ups
                k0, k1 = issued(u - 1), issued(u)

                def delayed(pos, k0=k0, k1=k1):
                    if pos in cfg["bulk_at"]:
                        first = cfg["bulk_at"].index(pos) * per_slot
                        for i in range(first, first + per_slot):
                            row = (k0 & 1) * (per_unit * rb) + i * rb
                            pl.when(k0 < k1)(functools.partial(
                                write_back, pl.ds((k0 >> 1) * gs, gs),
                                pl.ds(pl.multiple_of(row, 8), rb)))

                now = u >= fine
                if p == nu - 1:
                    now = now & (u < n_units - 1)

                    def on_store(r0, c, s=s, u=u):
                        pl.when(u == n_units - 1)(functools.partial(
                            write_back, s, pl.ds(r0, Q), pl.ds(c, 2 * L)))
                    units[p].on_store = on_store
                units[p].run(schedule, delayed)

                @pl.when(now)
                def _(s=s, c0=c0):
                    for c in range(c0, c0 + UNIT, L):
                        write_back(s, slice(None), pl.ds(c, L))

            if not hand:
                return None
            head = ahead.tile_stats(*TILE_ORDER[0])
            assert head.left() == 0
            return (*[v for key in TILE_ORDER[1:] for v in ahead.norm(*key)],
                    head.x0, head.a1[0], head.a2[0])

        j = u0 = 0
        stats = None
        for nu, count, hand in plan:
            if count == 1:
                stats = do_chunk(j, u0, nu, 0, stats, hand, False)
            else:
                assert nu % ups == 0 and u0 % ups == 0

                def body(it, carry, j=j, u0=u0, nu=nu):
                    return do_chunk(j + it, u0, nu, it * (nu // ups), carry, True, True)
                lax.fori_loop(0, count, body, stats)
            j += count
            u0 += nu * count
        pltpu.make_async_copy(obuf, o_hbm, osem.at[0]).wait()

    out = pl.pallas_call(
        kernel,
        in_specs=[pl.BlockSpec(memory_space=pl.ANY)] * 4,
        out_specs=pl.BlockSpec(memory_space=pl.ANY),
        out_shape=jax.ShapeDtypeStruct((S, D, B), x.dtype),
        scratch_shapes=[
            pltpu.VMEM((S, D, B + 2 * L), BF16),
            pltpu.VMEM((S, D, B), BF16),
            pltpu.VMEM((D, D), BF16),
            pltpu.VMEM((D,), BF16),
            pltpu.VMEM((D,), BF16),
            *[pltpu.VMEM(((H if n in LONG else Q) // 2, L), U32) for n in names],
            pltpu.VMEM((H, L), F32),
            pltpu.SemaphoreType.DMA((n_chunks,)),
            pltpu.SemaphoreType.DMA((n_chunks,)),
            pltpu.SemaphoreType.DMA((1,)),
            pltpu.SemaphoreType.DMA((4,)),
        ],
        compiler_params=pltpu.CompilerParams(
            vmem_limit_bytes=110 * 1024 * 1024,
            disable_bounds_checks=True,
            disable_semaphore_checks=True,
        ),
    )(xt, g, b, w)
    return jnp.transpose(out, (2, 0, 1))


@jax.jit
def pallas_standalone__layernorm_linear__sampling_kernel(
    x: jax.Array,
    g: jax.Array,
    b: jax.Array,
    w: jax.Array,
):
    return _forward(CONFIG, x, g, b, w)
```

```python
import functools

import jax
import jax.numpy as jnp
from jax import lax
import jax.experimental.pallas as pl
import jax.experimental.pallas.tpu as pltpu

EPS = 1e-5
F32 = jnp.float32
BF16 = jnp.bfloat16
U32 = jnp.uint32

L = 128
H = 288
Q = 144
KH = 256
KS = 192
KM = 2 * KH
UNIT = 512
STEPS = 72

LONG = tuple("S%d%s" % (i, h) for i in range(1, 8) for h in "ab") + ("R1", "R6", "R7")
LEVEL2 = ("S2", "S3", "S4", "S5")
SWAPPED = ("S2", "S5")
SHORT = tuple("%sm%d" % (p, k) for p in LEVEL2 for k in range(1, 8))
USES = {
    "S1": (("11", 1), ("22", 1)), "S2": (("21", 1), ("22", -1)),
    "S3": (("12", 1), ("22", 1)), "S4": (("11", 1), ("21", 1)),
    "S5": (("11", -1), ("12", 1)), "S6": (("22", 1),), "S7": (("11", 1),),
    "R1": (("12", 1), ("21", 1)), "R6": (("12", 1),), "R7": (("21", 1),),
    "D": (("21", 1), ("22", 1)),
}
TERMS = {"11": 4, "12": 4, "21": 5, "22": 5}
USES2 = {1: ((0, 0, 1), (1, 1, 1)), 2: ((1, 0, 1), (1, 1, -1)), 3: ((0, 1, 1), (1, 1, 1)),
         4: ((0, 0, 1), (1, 0, 1)), 5: ((0, 0, -1), (0, 1, 1)), 6: ((1, 1, 1),),
         7: ((0, 0, 1),)}
TERMS2 = {(0, 0): 4, (0, 1): 2, (1, 0): 2, (1, 1): 4}
TILE_ORDER = ((0, 0), (1, 0), (0, 1), (1, 1))

_ROWS = ("S4m1 S4m7 S4m6 S4m2", "A:D B:D S4m4 S4m3 S4m5 S5m6", "S5m2 S5m4 S5m3 S5m5",
         "S5m1 S5m7 S3m4 S3m2", "S3m5 S3m3 S3m1 S3m6", "S3m7 S2m1 S2m7 S2m6",
         "A:R7 B:R7 S2m2 S2m4", "S2m3 S2m5", "A:S1a A:S1b B:S1a B:S1b",
         "A:R1 B:R1 A:R6 B:R6", "A:S7a A:S7b B:S7a B:S7b", "A:S6a A:S6b B:S6a B:S6b")
_ROWS_COLD = ("A:D A:S1a A:S1b A:R7 A:R1", "A:R6 A:S7a A:S7b A:S6a", "S4m1 S4m7 S4m6 S4m2",
              "S4m4 S4m3 S4m5 S2m1", "S2m6 S2m2 S2m4 S2m3", "S2m5 S2m7 S3m4 S3m2",
              "S3m5 S3m3 S3m1 S3m6", "B:D S3m7 S5m1 S5m7 S5m6", "A:S6b B:R7 S5m2 S5m4",
              "S5m3 S5m5", "B:S1a B:S1b B:R1 B:R6", "B:S7a B:S7b B:S6a B:S6b")
_ROWS_COLD0 = ("A:S4a A:S4b A:Q3a A:Q3b", "B:P4a B:P4b B:P3a B:P3b",
               "A:V3 A:D A:R7 A:R1 A:R6 A:S1a", "A:S1b A:S7a A:S7b A:S6a",
               "A:S6b B:V4 B:V3 B:D B:R7 B:R1 B:R6", "S2m2 S2m4 S2m3 S2m5",
               "S2m6 S2m1 S2m7 S5m1", "S5m7 S5m6 S5m2 S5m4", "B:S1a B:S1b S5m3 S5m5",
               "B:S7a B:S7b B:S6a B:S6b")


def _schedule(rows, weights):
    out = []
    for row, steps in zip(rows, weights, strict=True):
        toks = row.split()
        passes = [t for t in toks if not (t.endswith(":D") or ":V" in t)]
        for t in toks:
            n = 0
            if t in passes:
                k = passes.index(t)
                n = steps * (k + 1) // len(passes) - steps * k // len(passes)
            out.append((t, n))
    return tuple(out)


CONFIG = dict(
    plan=((1, 1, False), (2, 1, False), (4, 1, True), (7, 1, True), (10, 5, True)),
    steady=_schedule(_ROWS, (4, 20, 40, 12, 20, 12, 24, 20, 28, 24, 32, 52)),
    warm=_schedule(_ROWS, (0, 28, 28, 0, 68, 20, 8, 20, 32, 20, 48, 16)),
    last=_schedule(_ROWS, (12, 36, 24, 12, 20, 28, 12, 24, 12, 28, 28, 52)),
    cold=(_schedule(_ROWS_COLD0, (0, 16, 0, 32, 0, 4, 56, 4, 0, 32)),
          _schedule(_ROWS_COLD, (0, 60, 64, 20, 36, 36, 28, 16, 28, 16, 52, 76)),
          _schedule(_ROWS_COLD, (0, 56, 64, 20, 28, 24, 20, 40, 28, 24, 56, 72))),
    gate_row=120,
    write_start=30,
    write_fine=48,
    bulk_slices=4,
    bulk_rows=24,
    bulk_per_unit=12,
    bulk_at=(3, 7, 11, 12, 17, 18, 21, 25, 26, 28, 37, 42),
)


def _pack(v):
    return pltpu.bitcast(v.astype(BF16), U32)


def _prep_first(g_ref, w_ref, ref, used, d_model, rows=16):
    g = g_ref[...].astype(F32).reshape(1, d_model)
    wt = jnp.concatenate([w_ref[0:L, :], w_ref[KH:KH + L, :]], axis=0).T
    keep = {}
    for r0 in range(0, H, rows):
        a11, a12, a21, a22 = [
            wt[h * H + r0:h * H + r0 + rows, k * L:(k + 1) * L].astype(F32)
            * g[:, k * KH:k * KH + L] for h in range(2) for k in range(2)]
        xs = (a11 + a22, a21 + a22, a11, a22, a11 + a12, a21 - a11, a12 - a22)
        for k in range(7):
            name = "S%da" % (k + 1)
            if name in used:
                ref[name][r0 // 2:(r0 + rows) // 2, :] = _pack(xs[k])
            keep[name, r0] = xs[k]
    for r0 in range(0, Q, rows):
        for p in LEVEL2:
            x11, x21 = keep[p + "a", r0], keep[p + "a", Q + r0]
            if p in SWAPPED:
                x11, x21 = x21, x11
            ref[p + "m3"][r0 // 2:(r0 + rows) // 2, :] = _pack(x11)
            ref[p + "m6"][r0 // 2:(r0 + rows) // 2, :] = _pack(x21 - x11)
    return keep


def _prep_rest(g_ref, b_ref, w_ref, ref, dl_ref, used, keep, d_model, rows=16):
    w = w_ref[...]
    g = g_ref[...].astype(F32).reshape(1, d_model)
    wt = jnp.concatenate([w[L:KH], w[KH + L:KM]], axis=0).T
    gt = jnp.concatenate([g[:, KM:d_model]] * 2, axis=1)
    at = jnp.concatenate([w[KM:d_model]] * 2, axis=0).T
    brow = jnp.broadcast_to(b_ref[...].astype(F32).reshape(1, d_model), (16, d_model))
    drow = jnp.dot(brow.astype(BF16), w, preferred_element_type=F32)
    row = lax.broadcasted_iota(jnp.int32, (16, d_model), 0)
    lo = drow - drow.astype(BF16).astype(F32)
    e = jnp.where(row == 0, drow, jnp.where(row == 1, lo, 0.0))
    z = jnp.zeros((48, d_model), F32)
    et = jnp.concatenate([e, z, e, z], axis=0).astype(BF16).T
    low = lax.broadcasted_iota(jnp.int32, (rows, L), 1) < 64

    def sel(p, q):
        return jnp.where(low, p, q)

    def level1(r0):
        a11, a12, a21, a22 = [
            wt[h * H + r0:h * H + r0 + rows, k * L:(k + 1) * L].astype(F32)
            * g[:, k * KH + L:(k + 1) * KH] for h in range(2) for k in range(2)]
        at1 = at[r0:r0 + rows].astype(F32) * gt
        at2 = at[H + r0:H + r0 + rows].astype(F32) * gt
        e1 = et[r0:r0 + rows].astype(F32)
        s2, s5, s6, s7 = a21 + a22, a11 + a12, a21 - a11, a12 - a22
        xs = (sel(a11 + a22, e1), sel(s2, -s2), sel(a11, a21), sel(a22, a12),
              sel(s5, -s5), sel(s6, at2), sel(s7, at1))
        res = {"S%db" % (k + 1): xs[k] for k in range(7)}
        res["R1"] = sel(e1, a21 + a12)
        res["R6"] = sel(at1, -s6)
        res["R7"] = sel(at2, -s7)
        for name in res:
            if name in used:
                ref[name][r0 // 2:(r0 + rows) // 2, :] = _pack(res[name])
        return res

    for r0 in range(0, Q, rows):
        u, v = level1(r0), level1(Q + r0)
        for p in LEVEL2:
            x11, x12 = keep[p + "a", r0], u[p + "b"]
            x21, x22 = keep[p + "a", Q + r0], v[p + "b"]
            if p in SWAPPED:
                x11, x12, x21, x22 = x21, x22, x11, x12
            xs = {1: x11 + x22, 2: x21 + x22, 4: x22, 5: x11 + x12, 7: x12 - x22}
            for k in xs:
                ref["%sm%d" % (p, k)][r0 // 2:(r0 + rows) // 2, :] = _pack(xs[k])
    low2 = lax.broadcasted_iota(jnp.int32, (H, L), 1) < 64
    lhs = jnp.where(low2, et[H:d_model].astype(F32), -et[0:H].astype(F32)).astype(BF16)
    dl_ref[...] = jnp.dot(lhs, jnp.ones((L, L), BF16), preferred_element_type=F32)


class _Stats:
    def __init__(self, x_ref, d_model, chains=1):
        self.x_ref, self.d_model = x_ref, d_model
        self.pos = 0
        self.x0 = None
        self.a1 = [None] * chains
        self.a2 = [None] * chains
        self.pending = []
        self.result = None

    def left(self):
        return STEPS - self.pos

    def advance(self, n):
        if self.x0 is None:
            self.x0 = self.x_ref[0:16, :].astype(F32)[0:1, :]
        for _ in range(n):
            if not self.pending:
                r0 = self.pos * 8
                t = self.x_ref[r0:r0 + 16, :].astype(F32) - self.x0
                self.pending = [t[0:8], t[8:16]]
            t = self.pending.pop(0)
            c = self.pos % len(self.a1)
            self.a1[c] = t if self.a1[c] is None else self.a1[c] + t
            self.a2[c] = t * t if self.a2[c] is None else self.a2[c] + t * t
            self.pos += 1
        return self.a2[0]

    def finish(self):
        if self.result is None:
            self.advance(self.left())
            a1 = functools.reduce(lambda u, v: u + v, self.a1)
            a2 = functools.reduce(lambda u, v: u + v, self.a2)
            s1 = jnp.sum(a1, axis=0, keepdims=True) * (1.0 / self.d_model)
            s2 = jnp.sum(a2, axis=0, keepdims=True) * (1.0 / self.d_model)
            var = jnp.maximum(s2 - s1 * s1, 0.0)
            self.result = (self.x0 + s1, lax.rsqrt(var + EPS))
        return self.result


def _signed_add(cur, v, sign):
    if cur is None:
        return v, sign
    val, cur_sign = cur
    if cur_sign == 1:
        return (val + v if sign == 1 else val - v), 1
    return (v - val, 1) if sign == 1 else (val + v, -1)


class _Unit:
    def __init__(self, xs_ref, os_ref, ref, dl_ref, c0, d_model, gate_row):
        self.xs_ref, self.os_ref, self.ref, self.dl_ref = xs_ref, os_ref, ref, dl_ref
        self.c0, self.d_model, self.gate_row = c0, d_model, gate_row
        self.stats = {}
        self.cache = {}
        self.queue = []
        self.on_store = None

    def col(self, pair, j):
        return self.c0 + (pair + 2 * j) * L

    def tile_stats(self, pair, j, chains=1):
        if (pair, j) not in self.stats:
            self.stats[pair, j] = _Stats(
                self.xs_ref.at[:, pl.ds(self.col(pair, j), L)], self.d_model, chains)
        return self.stats[pair, j]

    def norm(self, pair, j):
        return self.tile_stats(pair, j).finish()

    def x(self, pair, k, j, r0, r1):
        c = self.col(pair, j)
        return self.xs_ref[k * KH + r0:k * KH + r1, c:c + L].astype(F32)

    def hat(self, pair, k, j, r0, r1):
        m, r = self.norm(pair, j)
        return (self.x(pair, k, j, r0, r1) - m) * r

    def tail(self, pair, j):
        if ("tail", pair, j) not in self.cache:
            self.cache["tail", pair, j] = self.hat(pair, 2, j, 0, 64)
        return self.cache["tail", pair, j]

    def cross(self, pair, ka, kb, r0, r1):
        (ma, ra), (mb, rb) = self.norm(pair, 0), self.norm(pair, 1)
        if ("mr", pair) not in self.cache:
            self.cache["mr", pair] = ma * ra + mb * rb
        return (self.x(pair, ka, 0, r0, r1) * ra + self.x(pair, kb, 1, r0, r1) * rb
                - self.cache["mr", pair])

    def rhs(self, pair, name, raw=None):
        row = lax.broadcasted_iota(jnp.int32, (16, L), 0)
        ones = jnp.where(row < 2, 1.0, 0.0)

        def cat(*parts):
            return jnp.concatenate(parts, axis=0)

        if name == "R1":
            return cat(ones, jnp.zeros((48, L), F32), self.cross(pair, 0, 1, KS, KH))
        if name == "R6":
            return cat(self.tail(pair, 1), self.cross(pair, 0, 0, KS, KH))
        if name == "R7":
            return cat(self.tail(pair, 0), self.cross(pair, 1, 1, KS, KH))
        prod, r0 = name[:2], (0 if name[2] == "a" else L)
        if prod in ("S3", "S4"):
            j = 1 if prod == "S3" else 0
            diff = self.x(pair, 1 - j, j, r0, r0 + L) - self.x(pair, j, j, r0, r0 + L)
            if raw == "P":
                return diff
            if raw == "Q":
                return diff + jnp.minimum(self.norm(pair, 0)[1], 0.0)
            return diff * self.norm(pair, j)[1]
        main = {"S1": lambda a, b: self.cross(pair, 0, 1, a, b),
                "S2": lambda a, b: self.hat(pair, 0, 0, a, b),
                "S5": lambda a, b: self.hat(pair, 1, 1, a, b),
                "S6": lambda a, b: self.cross(pair, 0, 0, a, b),
                "S7": lambda a, b: self.cross(pair, 1, 1, a, b)}[prod]
        if r0 == 0:
            return main(0, L)
        rest = {"S1": lambda: ones,
                "S2": lambda: self.hat(pair, 1, 1, KS, KH),
                "S5": lambda: self.hat(pair, 0, 0, KS, KH),
                "S6": lambda: self.tail(pair, 1),
                "S7": lambda: self.tail(pair, 0)}[prod]
        return cat(main(L, KS), rest())

    def rhs2(self, prod, k):
        def h(kk, pair):
            if ("h", prod, kk, pair) not in self.cache:
                self.cache["h", prod, kk, pair] = self.rhs(pair, prod + "ab"[kk])
            return self.cache["h", prod, kk, pair]

        return {1: lambda: h(0, 0) + h(1, 1), 2: lambda: h(0, 0),
                3: lambda: h(0, 1) - h(1, 1), 4: lambda: h(1, 0) - h(0, 0),
                5: lambda: h(1, 1), 6: lambda: h(0, 0) + h(0, 1),
                7: lambda: h(1, 0) + h(1, 1)}[k]()

    def run(self, schedule, before_token):
        acc, count, done = {}, {}, {}
        acc2, count2, part = {}, {}, {}

        def add(pair, half, name, v):
            for key, sign in USES[name]:
                k = (pair, half, key)
                acc[k] = _signed_add(acc.get(k), v, sign)
                count[k] = count.get(k, 0) + 1
                if count[k] == TERMS[key]:
                    val, val_sign = acc[k]
                    assert val_sign == 1
                    done[k] = val
                    if (1 - pair, half, key) in done:
                        r0 = (0 if key[0] == "1" else H) + half * Q
                        c = self.col(0, int(key[1]) - 1)
                        both = jnp.concatenate(
                            [done[0, half, key], done[1, half, key]], axis=1)
                        self.os_ref[r0:r0 + Q, c:c + 2 * L] = both.astype(BF16)
                        if self.on_store is not None:
                            self.on_store(r0, c)

        def add_full(pair, name, v):
            add(pair, 0, name, v[0:Q])
            add(pair, 1, name, v[Q:H])

        for pos, (token, steps) in enumerate(schedule):
            before_token(pos)
            gate = None
            while steps > 0 and self.queue:
                n = min(steps, self.queue[0].left())
                gate = self.queue[0].advance(n)
                steps -= n
                if self.queue[0].left() == 0:
                    gate = jnp.broadcast_to(self.queue.pop(0).finish()[1], (8, L))

            def dot(name, q, gate=gate):
                if gate is not None:
                    g0 = self.gate_row if q.shape[0] > self.gate_row else 0
                    parts = [q[0:g0]] if g0 else []
                    parts.append(q[g0:g0 + 8] + jnp.minimum(gate, 0.0))
                    if g0 + 8 < q.shape[0]:
                        parts.append(q[g0 + 8:])
                    q = jnp.concatenate(parts, axis=0)
                p = pltpu.bitcast(self.ref[name][...], BF16)[:, 0:q.shape[0]]
                return jnp.dot(p, q.astype(BF16), preferred_element_type=F32)

            if ":" not in token:
                prod, k = token[:2], int(token[3])
                v = dot(token, self.rhs2(prod, k))
                for half, pair, sign in USES2[k]:
                    kk = (prod, half, pair)
                    acc2[kk] = _signed_add(acc2.get(kk), v, sign)
                    count2[kk] = count2.get(kk, 0) + 1
                    if count2[kk] == TERMS2[half, pair]:
                        val, val_sign = acc2[kk]
                        assert val_sign == 1
                        add(pair, 1 - half if prod in SWAPPED else half, prod, val)
                continue
            pair, name = "AB".index(token[0]), token[2:]
            if name == "D":
                add_full(pair, "D", self.dl_ref[...])
                continue
            if name[0] == "V":
                prod = "S" + name[1]
                scale = self.norm(pair, 1 if prod == "S3" else 0)[1]
                add_full(pair, prod, part.pop((pair, prod)) * scale)
                continue
            raw = name[0] if name[0] in "PQ" else None
            name = "S" + name[1:] if raw else name
            v = dot(name, self.rhs(pair, name, raw))
            prod = name[:2]
            if prod[0] == "R":
                add_full(pair, prod, v)
            elif (pair, prod) not in part:
                part[pair, prod] = v
            elif raw:
                part[pair, prod] = v + part[pair, prod]
            else:
                add_full(pair, prod, v + part.pop((pair, prod)))
        assert len(done) == 16


def _forward(cfg, x, g, b, w):
    B, S, D = x.shape
    assert D == 2 * H == KM + 64 == 8 * STEPS
    plan = cfg["plan"]
    ups = B // UNIT
    n_units = S * ups
    assert sum(u * n for u, n, _ in plan) == n_units
    n_chunks = sum(n for _, n, _ in plan)
    names = LONG + SHORT
    used = {t[2:].replace("P", "S").replace("Q", "S")
            for sched in (cfg["steady"], *cfg["cold"]) for t, _ in sched if ":" in t}
    fine, per_unit = cfg["write_fine"], cfg["bulk_per_unit"]
    gs, rb = cfg["bulk_slices"], cfg["bulk_rows"]
    nrb = D // rb

    assert nrb == 2 * per_unit and gs * ups == 8
    per_slot = per_unit // len(cfg["bulk_at"])
    assert per_slot * len(cfg["bulk_at"]) == per_unit

    def issued(u, lo=jnp.minimum, hi=jnp.maximum):
        def ready(v):
            return 2 * (lo(v, fine) >> 3)
        n = lo(lo(u - cfg["write_start"] + 1, ready(u)), ready(u - 1) + 1)
        return hi(n, 0)

    loop_start = sum(u * n for u, n, _ in plan[:-1])
    table = {u: issued(u, min, max) for u in range(loop_start - 1, n_units)}
    assert table[loop_start - 1] == 0 and fine >= loop_start and fine % (gs * ups) == 0
    assert all(0 <= table[u] - table[u - 1] <= 1 for u in range(loop_start, n_units))
    assert all(table[u] <= 2 * (u // (gs * ups)) for u in table)
    assert table[n_units - 1] == 2 * fine // (gs * ups)
    assert all(n == 1 for _, n, _ in plan[:-1]) and plan[-1][2] and plan[-2][2]

    xt = jnp.transpose(x, (1, 2, 0))

    def kernel(x_hbm, g_hbm, b_hbm, w_hbm, o_hbm, xbuf, obuf, wbuf, gbuf, bbuf, *rest):
        ref = dict(zip(names, rest))
        dl_ref, isem, nsem, osem, wsem = rest[len(names):]

        def copies(sem, u, end, shift=0):
            res = []
            while u < end:
                s, r = divmod(u, ups)
                if r == 0 and end - u >= ups:
                    idx = (pl.ds(s + shift, (end - u) // ups), slice(None), pl.ds(0, B))
                    u += (end - u) // ups * ups
                else:
                    idx = (s + shift, slice(None), pl.ds(r * UNIT, UNIT))
                    u += 1
                res.append(pltpu.make_async_copy(x_hbm.at[idx], xbuf.at[idx], sem))
            return res

        def write_back(*idx):
            pltpu.make_async_copy(obuf.at[idx], o_hbm.at[idx], osem.at[0]).start()

        def w_rows(r0, r1, k):
            rows = pl.ds(r0, r1 - r0)
            return pltpu.make_async_copy(w_hbm.at[rows], wbuf.at[rows], wsem.at[k])

        cg = pltpu.make_async_copy(g_hbm, gbuf, wsem.at[1])
        cb = pltpu.make_async_copy(b_hbm, bbuf, wsem.at[2])
        w_first = [w_rows(0, L, 0), w_rows(KH, KH + L, 0)]
        w_rest = [w_rows(L, KH, 3), w_rows(KH + L, D, 3)]
        for c in [cg, cb] + w_first + w_rest:
            c.start()
        cg.wait()
        cb.wait()
        j = u0 = 0
        handed = False
        for nu, count, hand in plan:
            for _ in range(count):
                for c in copies(isem.at[j], u0 + handed, u0 + nu):
                    c.start()
                if hand and u0 + nu < n_units:
                    for c in copies(nsem.at[j], u0 + nu, u0 + nu + 1):
                        c.start()
                j += 1
                u0 += nu
                handed = hand
        for c in w_first:
            c.wait()
        keep = _prep_first(gbuf, wbuf, ref, used, D)
        for c in w_rest:
            c.wait()
        _prep_rest(gbuf, bbuf, wbuf, ref, dl_ref, used, keep, D)

        def make_unit(s, c0):
            return _Unit(xbuf.at[s], obuf.at[s], ref, dl_ref, c0, D, cfg["gate_row"])

        def do_chunk(j, u0, nu, shift, stats_in, hand, in_loop):
            for c in copies(isem.at[j], u0 + (stats_in is not None), u0 + nu, shift):
                c.wait()
            if hand:
                s_next, r_next = divmod(u0 + nu, ups)
                if in_loop:
                    exists = s_next + shift < S
                    s_next = jnp.minimum(s_next + shift, S - 1)

                    @pl.when(exists)
                    def _():
                        copies(nsem.at[j], r_next, r_next + 1, s_next)[0].wait()
                else:
                    copies(nsem.at[j], u0 + nu, u0 + nu + 1)[0].wait()
            where = [(u // ups + shift, (u % ups) * UNIT) for u in range(u0, u0 + nu)]
            units = [make_unit(s, c0) for s, c0 in where]
            if stats_in is None:
                units[0].tile_stats(0, 0, chains=2)
                units[0].queue = [units[0].tile_stats(1, 0), units[0].tile_stats(1, 1)]
            else:
                for n, key in enumerate(TILE_ORDER[1:]):
                    units[0].tile_stats(*key).result = stats_in[2 * n:2 * n + 2]
                head = units[0].tile_stats(*TILE_ORDER[0])
                head.x0, head.a1, head.a2 = stats_in[6], [stats_in[7]], [stats_in[8]]
                head.pos = STEPS
            for p in range(nu - 1):
                units[p].queue += [units[p + 1].tile_stats(*key) for key in TILE_ORDER]
            if hand:
                ahead = make_unit(s_next, r_next * UNIT)
                units[-1].queue += [ahead.tile_stats(*key)
                                    for key in TILE_ORDER[1:] + TILE_ORDER[:1]]

            for p, (s, c0) in enumerate(where):
                if p == 0:
                    schedule = cfg["cold"][j] if stats_in is None else cfg["warm"]
                else:
                    schedule = cfg["last"] if (hand and p == nu - 1) else cfg["steady"]
                if not in_loop:
                    units[p].run(schedule, lambda pos: None)
                    continue
                u = u0 + p + shift * ups
                k0, k1 = issued(u - 1), issued(u)

                def delayed(pos, k0=k0, k1=k1):
                    if pos in cfg["bulk_at"]:
                        first = cfg["bulk_at"].index(pos) * per_slot
                        for i in range(first, first + per_slot):
                            row = (k0 & 1) * (per_unit * rb) + i * rb
                            pl.when(k0 < k1)(functools.partial(
                                write_back, pl.ds((k0 >> 1) * gs, gs),
                                pl.ds(pl.multiple_of(row, 8), rb)))

                now = u >= fine
                if p == nu - 1:
                    now = now & (u < n_units - 1)

                    def on_store(r0, c, s=s, u=u):
                        pl.when(u == n_units - 1)(functools.partial(
                            write_back, s, pl.ds(r0, Q), pl.ds(c, 2 * L)))
                    units[p].on_store = on_store
                units[p].run(schedule, delayed)

                @pl.when(now)
                def _(s=s, c0=c0):
                    for c in range(c0, c0 + UNIT, L):
                        write_back(s, slice(None), pl.ds(c, L))

            if not hand:
                return None
            head = ahead.tile_stats(*TILE_ORDER[0])
            assert head.left() == 0
            return (*[v for key in TILE_ORDER[1:] for v in ahead.norm(*key)],
                    head.x0, head.a1[0], head.a2[0])

        j = u0 = 0
        stats = None
        for nu, count, hand in plan:
            if count == 1:
                stats = do_chunk(j, u0, nu, 0, stats, hand, False)
            else:
                assert nu % ups == 0 and u0 % ups == 0

                def body(it, carry, j=j, u0=u0, nu=nu):
                    return do_chunk(j + it, u0, nu, it * (nu // ups), carry, True, True)
                lax.fori_loop(0, count, body, stats)
            j += count
            u0 += nu * count
        pltpu.make_async_copy(obuf, o_hbm, osem.at[0]).wait()

    out = pl.pallas_call(
        kernel,
        in_specs=[pl.BlockSpec(memory_space=pl.ANY)] * 4,
        out_specs=pl.BlockSpec(memory_space=pl.ANY),
        out_shape=jax.ShapeDtypeStruct((S, D, B), x.dtype),
        scratch_shapes=[
            pltpu.VMEM((S, D, B + 2 * L), BF16),
            pltpu.VMEM((S, D, B), BF16),
            pltpu.VMEM((D, D), BF16),
            pltpu.VMEM((D,), BF16),
            pltpu.VMEM((D,), BF16),
            *[pltpu.VMEM(((H if n in LONG else Q) // 2, L), U32) for n in names],
            pltpu.VMEM((H, L), F32),
            pltpu.SemaphoreType.DMA((n_chunks,)),
            pltpu.SemaphoreType.DMA((n_chunks,)),
            pltpu.SemaphoreType.DMA((1,)),
            pltpu.SemaphoreType.DMA((4,)),
        ],
        compiler_params=pltpu.CompilerParams(
            vmem_limit_bytes=110 * 1024 * 1024,
            disable_bounds_checks=True,
            disable_semaphore_checks=True,
        ),
    )(xt, g, b, w)
    return jnp.transpose(out, (2, 0, 1))


@jax.jit
def pallas_standalone__layernorm_linear__sampling_kernel(
    x: jax.Array,
    g: jax.Array,
    b: jax.Array,
    w: jax.Array,
):
    return _forward(CONFIG, x, g, b, w)
```

```python
import functools

import jax
import jax.numpy as jnp
from jax import lax
import jax.experimental.pallas as pl
import jax.experimental.pallas.tpu as pltpu

EPS = 1e-5
F32 = jnp.float32
BF16 = jnp.bfloat16
U32 = jnp.uint32

L = 128
H = 288
Q = 144
KH = 256
KS = 192
KM = 2 * KH
UNIT = 512
STEPS = 72

LONG = tuple("S%d%s" % (i, h) for i in range(1, 8) for h in "ab") + ("R1", "R6", "R7")
LEVEL2 = ("S2", "S3", "S4", "S5")
SWAPPED = ("S2", "S5")
SHORT = tuple("%sm%d" % (p, k) for p in LEVEL2 for k in range(1, 8))
USES = {
    "S1": (("11", 1), ("22", 1)), "S2": (("21", 1), ("22", -1)),
    "S3": (("12", 1), ("22", 1)), "S4": (("11", 1), ("21", 1)),
    "S5": (("11", -1), ("12", 1)), "S6": (("22", 1),), "S7": (("11", 1),),
    "R1": (("12", 1), ("21", 1)), "R6": (("12", 1),), "R7": (("21", 1),),
    "D": (("21", 1), ("22", 1)),
}
TERMS = {"11": 4, "12": 4, "21": 5, "22": 5}
USES2 = {1: ((0, 0, 1), (1, 1, 1)), 2: ((1, 0, 1), (1, 1, -1)), 3: ((0, 1, 1), (1, 1, 1)),
         4: ((0, 0, 1), (1, 0, 1)), 5: ((0, 0, -1), (0, 1, 1)), 6: ((1, 1, 1),),
         7: ((0, 0, 1),)}
TERMS2 = {(0, 0): 4, (0, 1): 2, (1, 0): 2, (1, 1): 4}
TILE_ORDER = ((0, 0), (1, 0), (0, 1), (1, 1))

_ROWS = ("S4m1 S4m7 S4m6 S4m2", "A:D B:D S4m4 S4m3 S4m5 S5m6", "S5m2 S5m4 S5m3 S5m5",
         "S5m1 S5m7 S3m4 S3m2", "S3m5 S3m3 S3m1 S3m6", "S3m7 S2m1 S2m7 S2m6",
         "A:R7 B:R7 S2m2 S2m4", "S2m3 S2m5", "A:S1a A:S1b B:S1a B:S1b",
         "A:R1 B:R1 A:R6 B:R6", "A:S7a A:S7b B:S7a B:S7b", "A:S6a A:S6b B:S6a B:S6b")
_ROWS_COLD = ("A:D A:S1a A:S1b A:R7 A:R1", "A:R6 A:S7a A:S7b A:S6a", "S4m1 S4m7 S4m6 S4m2",
              "S4m4 S4m3 S4m5 S2m1", "S2m6 S2m2 S2m4 S2m3", "S2m5 S2m7 S3m4 S3m2",
              "S3m5 S3m3 S3m1 S3m6", "B:D S3m7 S5m1 S5m7 S5m6", "A:S6b B:R7 S5m2 S5m4",
              "S5m3 S5m5", "B:S1a B:S1b B:R1 B:R6", "B:S7a B:S7b B:S6a B:S6b")
_ROWS_COLD0 = ("A:S4a A:S4b A:Q3a A:Q3b", "B:P4a B:P4b B:P3a B:P3b",
               "A:V3 A:D A:R7 A:R1 A:R6 A:S1a", "A:S1b A:S7a A:S7b A:S6a",
               "A:S6b B:V4 B:V3 B:D B:R7 B:R1 B:R6", "S2m2 S2m4 S2m3 S2m5",
               "S2m6 S2m1 S2m7 S5m1", "S5m7 S5m6 S5m2 S5m4", "B:S1a B:S1b S5m3 S5m5",
               "B:S7a B:S7b B:S6a B:S6b")


def _schedule(rows, weights):
    out = []
    for row, steps in zip(rows, weights, strict=True):
        toks = row.split()
        passes = [t for t in toks if not (t.endswith(":D") or ":V" in t)]
        for t in toks:
            n = 0
            if t in passes:
                k = passes.index(t)
                n = steps * (k + 1) // len(passes) - steps * k // len(passes)
            out.append((t, n))
    return tuple(out)


CONFIG = dict(
    plan=((1, 1, False), (2, 1, False), (4, 1, True), (7, 1, True), (10, 5, True)),
    ramp=(_schedule(_ROWS, (0, 8, 48, 24, 20, 8, 16, 32, 48, 0, 32, 52)),
          _schedule(_ROWS, (0, 20, 40, 12, 24, 4, 28, 20, 32, 24, 32, 52)),
          _schedule(_ROWS, (24, 36, 12, 12, 32, 16, 12, 24, 12, 28, 28, 52))),
    loop=(_schedule(_ROWS, (0, 28, 28, 0, 68, 20, 8, 20, 32, 20, 48, 16)),
          _schedule(_ROWS, (4, 20, 40, 12, 20, 12, 24, 20, 28, 24, 32, 52)),
          _schedule(_ROWS, (12, 36, 24, 12, 20, 28, 12, 24, 12, 28, 28, 52))),
    cold=(_schedule(_ROWS_COLD0, (0, 16, 0, 44, 0, 4, 56, 0, 4, 20)),
          _schedule(_ROWS_COLD, (0, 60, 64, 16, 36, 36, 40, 16, 28, 16, 56, 64)),
          _schedule(_ROWS_COLD, (0, 56, 64, 20, 28, 24, 20, 40, 28, 24, 56, 72))),
    gate_row=120,
    write_start=30,
    write_fine=48,
    bulk_slices=4,
    bulk_rows=24,
    bulk_per_unit=12,
    bulk_at=(3, 7, 11, 12, 17, 18, 21, 25, 26, 28, 37, 42),
)


def _pack(v):
    return pltpu.bitcast(v.astype(BF16), U32)


def _prep_first(g_ref, w_ref, ref, used, d_model, rows=16):
    g = g_ref[...].astype(F32).reshape(1, d_model)
    wt = jnp.concatenate([w_ref[0:L, :], w_ref[KH:KH + L, :]], axis=0).T
    keep = {}
    for r0 in range(0, H, rows):
        a11, a12, a21, a22 = [
            wt[h * H + r0:h * H + r0 + rows, k * L:(k + 1) * L].astype(F32)
            * g[:, k * KH:k * KH + L] for h in range(2) for k in range(2)]
        xs = (a11 + a22, a21 + a22, a11, a22, a11 + a12, a21 - a11, a12 - a22)
        for k in range(7):
            name = "S%da" % (k + 1)
            if name in used:
                ref[name][r0 // 2:(r0 + rows) // 2, :] = _pack(xs[k])
            keep[name, r0] = xs[k]
    for r0 in range(0, Q, rows):
        for p in LEVEL2:
            x11, x21 = keep[p + "a", r0], keep[p + "a", Q + r0]
            if p in SWAPPED:
                x11, x21 = x21, x11
            ref[p + "m3"][r0 // 2:(r0 + rows) // 2, :] = _pack(x11)
            ref[p + "m6"][r0 // 2:(r0 + rows) // 2, :] = _pack(x21 - x11)
    return keep


def _prep_rest(g_ref, b_ref, w_ref, ref, dl_ref, used, keep, d_model, rows=16):
    w = w_ref[...]
    g = g_ref[...].astype(F32).reshape(1, d_model)
    wt = jnp.concatenate([w[L:KH], w[KH + L:KM]], axis=0).T
    gt = jnp.concatenate([g[:, KM:d_model]] * 2, axis=1)
    at = jnp.concatenate([w[KM:d_model]] * 2, axis=0).T
    brow = jnp.broadcast_to(b_ref[...].astype(F32).reshape(1, d_model), (16, d_model))
    drow = jnp.dot(brow.astype(BF16), w, preferred_element_type=F32)
    row = lax.broadcasted_iota(jnp.int32, (16, d_model), 0)
    lo = drow - drow.astype(BF16).astype(F32)
    e = jnp.where(row == 0, drow, jnp.where(row == 1, lo, 0.0))
    z = jnp.zeros((48, d_model), F32)
    et = jnp.concatenate([e, z, e, z], axis=0).astype(BF16).T
    low = lax.broadcasted_iota(jnp.int32, (rows, L), 1) < 64

    def sel(p, q):
        return jnp.where(low, p, q)

    def level1(r0):
        a11, a12, a21, a22 = [
            wt[h * H + r0:h * H + r0 + rows, k * L:(k + 1) * L].astype(F32)
            * g[:, k * KH + L:(k + 1) * KH] for h in range(2) for k in range(2)]
        at1 = at[r0:r0 + rows].astype(F32) * gt
        at2 = at[H + r0:H + r0 + rows].astype(F32) * gt
        e1 = et[r0:r0 + rows].astype(F32)
        s2, s5, s6, s7 = a21 + a22, a11 + a12, a21 - a11, a12 - a22
        xs = (sel(a11 + a22, e1), sel(s2, -s2), sel(a11, a21), sel(a22, a12),
              sel(s5, -s5), sel(s6, at2), sel(s7, at1))
        res = {"S%db" % (k + 1): xs[k] for k in range(7)}
        res["R1"] = sel(e1, a21 + a12)
        res["R6"] = sel(at1, -s6)
        res["R7"] = sel(at2, -s7)
        for name in res:
            if name in used:
                ref[name][r0 // 2:(r0 + rows) // 2, :] = _pack(res[name])
        return res

    for r0 in range(0, Q, rows):
        u, v = level1(r0), level1(Q + r0)
        for p in LEVEL2:
            x11, x12 = keep[p + "a", r0], u[p + "b"]
            x21, x22 = keep[p + "a", Q + r0], v[p + "b"]
            if p in SWAPPED:
                x11, x12, x21, x22 = x21, x22, x11, x12
            xs = {1: x11 + x22, 2: x21 + x22, 4: x22, 5: x11 + x12, 7: x12 - x22}
            for k in xs:
                ref["%sm%d" % (p, k)][r0 // 2:(r0 + rows) // 2, :] = _pack(xs[k])
    low2 = lax.broadcasted_iota(jnp.int32, (H, L), 1) < 64
    lhs = jnp.where(low2, et[H:d_model].astype(F32), -et[0:H].astype(F32)).astype(BF16)
    dl_ref[...] = jnp.dot(lhs, jnp.ones((L, L), BF16), preferred_element_type=F32)


class _Stats:
    def __init__(self, x_ref, d_model, chains=1):
        self.x_ref, self.d_model = x_ref, d_model
        self.pos = 0
        self.x0 = None
        self.a1 = [None] * chains
        self.a2 = [None] * chains
        self.pending = []
        self.result = None

    def left(self):
        return STEPS - self.pos

    def advance(self, n):
        if self.x0 is None:
            self.x0 = self.x_ref[0:16, :].astype(F32)[0:1, :]
        for _ in range(n):
            if not self.pending:
                r0 = self.pos * 8
                t = self.x_ref[r0:r0 + 16, :].astype(F32) - self.x0
                self.pending = [t[0:8], t[8:16]]
            t = self.pending.pop(0)
            c = self.pos % len(self.a1)
            self.a1[c] = t if self.a1[c] is None else self.a1[c] + t
            self.a2[c] = t * t if self.a2[c] is None else self.a2[c] + t * t
            self.pos += 1
        return self.a2[0]

    def finish(self):
        if self.result is None:
            self.advance(self.left())
            a1 = functools.reduce(lambda u, v: u + v, self.a1)
            a2 = functools.reduce(lambda u, v: u + v, self.a2)
            s1 = jnp.sum(a1, axis=0, keepdims=True) * (1.0 / self.d_model)
            s2 = jnp.sum(a2, axis=0, keepdims=True) * (1.0 / self.d_model)
            var = jnp.maximum(s2 - s1 * s1, 0.0)
            self.result = (self.x0 + s1, lax.rsqrt(var + EPS))
        return self.result


def _signed_add(cur, v, sign):
    if cur is None:
        return v, sign
    val, cur_sign = cur
    if cur_sign == 1:
        return (val + v if sign == 1 else val - v), 1
    return (v - val, 1) if sign == 1 else (val + v, -1)


class _Unit:
    def __init__(self, xs_ref, os_ref, ref, dl_ref, c0, d_model, gate_row):
        self.xs_ref, self.os_ref, self.ref, self.dl_ref = xs_ref, os_ref, ref, dl_ref
        self.c0, self.d_model, self.gate_row = c0, d_model, gate_row
        self.stats = {}
        self.cache = {}
        self.queue = []
        self.on_store = None

    def col(self, pair, j):
        return self.c0 + (pair + 2 * j) * L

    def tile_stats(self, pair, j, chains=1):
        if (pair, j) not in self.stats:
            self.stats[pair, j] = _Stats(
                self.xs_ref.at[:, pl.ds(self.col(pair, j), L)], self.d_model, chains)
        return self.stats[pair, j]

    def norm(self, pair, j):
        return self.tile_stats(pair, j).finish()

    def x(self, pair, k, j, r0, r1):
        c = self.col(pair, j)
        return self.xs_ref[k * KH + r0:k * KH + r1, c:c + L].astype(F32)

    def hat(self, pair, k, j, r0, r1):
        m, r = self.norm(pair, j)
        return (self.x(pair, k, j, r0, r1) - m) * r

    def tail(self, pair, j):
        if ("tail", pair, j) not in self.cache:
            self.cache["tail", pair, j] = self.hat(pair, 2, j, 0, 64)
        return self.cache["tail", pair, j]

    def cross(self, pair, ka, kb, r0, r1):
        (ma, ra), (mb, rb) = self.norm(pair, 0), self.norm(pair, 1)
        if ("mr", pair) not in self.cache:
            self.cache["mr", pair] = ma * ra + mb * rb
        return (self.x(pair, ka, 0, r0, r1) * ra + self.x(pair, kb, 1, r0, r1) * rb
                - self.cache["mr", pair])

    def rhs(self, pair, name, raw=None):
        row = lax.broadcasted_iota(jnp.int32, (16, L), 0)
        ones = jnp.where(row < 2, 1.0, 0.0)

        def cat(*parts):
            return jnp.concatenate(parts, axis=0)

        if name == "R1":
            return cat(ones, jnp.zeros((48, L), F32), self.cross(pair, 0, 1, KS, KH))
        if name == "R6":
            return cat(self.tail(pair, 1), self.cross(pair, 0, 0, KS, KH))
        if name == "R7":
            return cat(self.tail(pair, 0), self.cross(pair, 1, 1, KS, KH))
        prod, r0 = name[:2], (0 if name[2] == "a" else L)
        if prod in ("S3", "S4"):
            j = 1 if prod == "S3" else 0
            diff = self.x(pair, 1 - j, j, r0, r0 + L) - self.x(pair, j, j, r0, r0 + L)
            if raw == "P":
                return diff
            if raw == "Q":
                return diff + jnp.minimum(self.norm(pair, 0)[1], 0.0)
            return diff * self.norm(pair, j)[1]
        main = {"S1": lambda a, b: self.cross(pair, 0, 1, a, b),
                "S2": lambda a, b: self.hat(pair, 0, 0, a, b),
                "S5": lambda a, b: self.hat(pair, 1, 1, a, b),
                "S6": lambda a, b: self.cross(pair, 0, 0, a, b),
                "S7": lambda a, b: self.cross(pair, 1, 1, a, b)}[prod]
        if r0 == 0:
            return main(0, L)
        rest = {"S1": lambda: ones,
                "S2": lambda: self.hat(pair, 1, 1, KS, KH),
                "S5": lambda: self.hat(pair, 0, 0, KS, KH),
                "S6": lambda: self.tail(pair, 1),
                "S7": lambda: self.tail(pair, 0)}[prod]
        return cat(main(L, KS), rest())

    def rhs2(self, prod, k):
        def h(kk, pair):
            if ("h", prod, kk, pair) not in self.cache:
                self.cache["h", prod, kk, pair] = self.rhs(pair, prod + "ab"[kk])
            return self.cache["h", prod, kk, pair]

        return {1: lambda: h(0, 0) + h(1, 1), 2: lambda: h(0, 0),
                3: lambda: h(0, 1) - h(1, 1), 4: lambda: h(1, 0) - h(0, 0),
                5: lambda: h(1, 1), 6: lambda: h(0, 0) + h(0, 1),
                7: lambda: h(1, 0) + h(1, 1)}[k]()

    def run(self, schedule, before_token):
        acc, count, done = {}, {}, {}
        acc2, count2, part = {}, {}, {}

        def add(pair, half, name, v):
            for key, sign in USES[name]:
                k = (pair, half, key)
                acc[k] = _signed_add(acc.get(k), v, sign)
                count[k] = count.get(k, 0) + 1
                if count[k] == TERMS[key]:
                    val, val_sign = acc[k]
                    assert val_sign == 1
                    done[k] = val
                    if (1 - pair, half, key) in done:
                        r0 = (0 if key[0] == "1" else H) + half * Q
                        c = self.col(0, int(key[1]) - 1)
                        both = jnp.concatenate(
                            [done[0, half, key], done[1, half, key]], axis=1)
                        self.os_ref[r0:r0 + Q, c:c + 2 * L] = both.astype(BF16)
                        if self.on_store is not None:
                            self.on_store(r0, c)

        def add_full(pair, name, v):
            add(pair, 0, name, v[0:Q])
            add(pair, 1, name, v[Q:H])

        for pos, (token, steps) in enumerate(schedule):
            before_token(pos)
            gate = None
            while steps > 0 and self.queue:
                n = min(steps, self.queue[0].left())
                gate = self.queue[0].advance(n)
                steps -= n
                if self.queue[0].left() == 0:
                    gate = jnp.broadcast_to(self.queue.pop(0).finish()[1], (8, L))

            def dot(name, q, gate=gate):
                if gate is not None:
                    g0 = self.gate_row if q.shape[0] > self.gate_row else 0
                    parts = [q[0:g0]] if g0 else []
                    parts.append(q[g0:g0 + 8] + jnp.minimum(gate, 0.0))
                    if g0 + 8 < q.shape[0]:
                        parts.append(q[g0 + 8:])
                    q = jnp.concatenate(parts, axis=0)
                p = pltpu.bitcast(self.ref[name][...], BF16)[:, 0:q.shape[0]]
                return jnp.dot(p, q.astype(BF16), preferred_element_type=F32)

            if ":" not in token:
                prod, k = token[:2], int(token[3])
                v = dot(token, self.rhs2(prod, k))
                for half, pair, sign in USES2[k]:
                    kk = (prod, half, pair)
                    acc2[kk] = _signed_add(acc2.get(kk), v, sign)
                    count2[kk] = count2.get(kk, 0) + 1
                    if count2[kk] == TERMS2[half, pair]:
                        val, val_sign = acc2[kk]
                        assert val_sign == 1
                        add(pair, 1 - half if prod in SWAPPED else half, prod, val)
                continue
            pair, name = "AB".index(token[0]), token[2:]
            if name == "D":
                add_full(pair, "D", self.dl_ref[...])
                continue
            if name[0] == "V":
                prod = "S" + name[1]
                scale = self.norm(pair, 1 if prod == "S3" else 0)[1]
                add_full(pair, prod, part.pop((pair, prod)) * scale)
                continue
            raw = name[0] if name[0] in "PQ" else None
            name = "S" + name[1:] if raw else name
            v = dot(name, self.rhs(pair, name, raw))
            prod = name[:2]
            if prod[0] == "R":
                add_full(pair, prod, v)
            elif (pair, prod) not in part:
                part[pair, prod] = v
            elif raw:
                part[pair, prod] = v + part[pair, prod]
            else:
                add_full(pair, prod, v + part.pop((pair, prod)))
        assert len(done) == 16


def _forward(cfg, x, g, b, w):
    B, S, D = x.shape
    assert D == 2 * H == KM + 64 == 8 * STEPS
    plan = cfg["plan"]
    ups = B // UNIT
    n_units = S * ups
    assert sum(u * n for u, n, _ in plan) == n_units
    n_chunks = sum(n for _, n, _ in plan)
    names = LONG + SHORT
    used = {t[2:].replace("P", "S").replace("Q", "S")
            for sched in (*cfg["loop"], *cfg["cold"]) for t, _ in sched if ":" in t}
    fine, per_unit = cfg["write_fine"], cfg["bulk_per_unit"]
    gs, rb = cfg["bulk_slices"], cfg["bulk_rows"]
    nrb = D // rb

    assert nrb == 2 * per_unit and gs * ups == 8
    per_slot = per_unit // len(cfg["bulk_at"])
    assert per_slot * len(cfg["bulk_at"]) == per_unit

    def issued(u, lo=jnp.minimum, hi=jnp.maximum):
        def ready(v):
            return 2 * (lo(v, fine) >> 3)
        n = lo(lo(u - cfg["write_start"] + 1, ready(u)), ready(u - 1) + 1)
        return hi(n, 0)

    loop_start = sum(u * n for u, n, _ in plan[:-1])
    table = {u: issued(u, min, max) for u in range(loop_start - 1, n_units)}
    assert table[loop_start - 1] == 0 and fine >= loop_start and fine % (gs * ups) == 0
    assert all(0 <= table[u] - table[u - 1] <= 1 for u in range(loop_start, n_units))
    assert all(table[u] <= 2 * (u // (gs * ups)) for u in table)
    assert table[n_units - 1] == 2 * fine // (gs * ups)
    assert all(n == 1 for _, n, _ in plan[:-1]) and plan[-1][2] and plan[-2][2]

    xt = jnp.transpose(x, (1, 2, 0))

    def kernel(x_hbm, g_hbm, b_hbm, w_hbm, o_hbm, xbuf, obuf, wbuf, gbuf, bbuf, *rest):
        ref = dict(zip(names, rest))
        dl_ref, isem, nsem, osem, wsem = rest[len(names):]

        def copies(sem, u, end, shift=0):
            res = []
            while u < end:
                s, r = divmod(u, ups)
                if r == 0 and end - u >= ups:
                    idx = (pl.ds(s + shift, (end - u) // ups), slice(None), pl.ds(0, B))
                    u += (end - u) // ups * ups
                else:
                    idx = (s + shift, slice(None), pl.ds(r * UNIT, UNIT))
                    u += 1
                res.append(pltpu.make_async_copy(x_hbm.at[idx], xbuf.at[idx], sem))
            return res

        def write_back(*idx):
            pltpu.make_async_copy(obuf.at[idx], o_hbm.at[idx], osem.at[0]).start()

        def w_rows(r0, r1, k):
            rows = pl.ds(r0, r1 - r0)
            return pltpu.make_async_copy(w_hbm.at[rows], wbuf.at[rows], wsem.at[k])

        cg = pltpu.make_async_copy(g_hbm, gbuf, wsem.at[1])
        cb = pltpu.make_async_copy(b_hbm, bbuf, wsem.at[2])
        w_first = [w_rows(0, L, 0), w_rows(KH, KH + L, 0)]
        w_rest = [w_rows(L, KH, 3), w_rows(KH + L, D, 3)]
        for c in [cg, cb] + w_first + w_rest:
            c.start()
        cg.wait()
        cb.wait()
        j = u0 = 0
        handed = False
        for nu, count, hand in plan:
            for _ in range(count):
                for c in copies(isem.at[j], u0 + handed, u0 + nu):
                    c.start()
                if hand and u0 + nu < n_units:
                    for c in copies(nsem.at[j], u0 + nu, u0 + nu + 1):
                        c.start()
                j += 1
                u0 += nu
                handed = hand
        for c in w_first:
            c.wait()
        keep = _prep_first(gbuf, wbuf, ref, used, D)
        for c in w_rest:
            c.wait()
        _prep_rest(gbuf, bbuf, wbuf, ref, dl_ref, used, keep, D)

        def make_unit(s, c0):
            return _Unit(xbuf.at[s], obuf.at[s], ref, dl_ref, c0, D, cfg["gate_row"])

        def do_chunk(j, u0, nu, shift, stats_in, hand, in_loop):
            for c in copies(isem.at[j], u0 + (stats_in is not None), u0 + nu, shift):
                c.wait()
            if hand:
                s_next, r_next = divmod(u0 + nu, ups)
                if in_loop:
                    exists = s_next + shift < S
                    s_next = jnp.minimum(s_next + shift, S - 1)

                    @pl.when(exists)
                    def _():
                        copies(nsem.at[j], r_next, r_next + 1, s_next)[0].wait()
                else:
                    copies(nsem.at[j], u0 + nu, u0 + nu + 1)[0].wait()
            where = [(u // ups + shift, (u % ups) * UNIT) for u in range(u0, u0 + nu)]
            units = [make_unit(s, c0) for s, c0 in where]
            if stats_in is None:
                units[0].tile_stats(0, 0, chains=2)
                units[0].queue = [units[0].tile_stats(1, 0), units[0].tile_stats(1, 1)]
            else:
                for n, key in enumerate(TILE_ORDER[1:]):
                    units[0].tile_stats(*key).result = stats_in[2 * n:2 * n + 2]
                head = units[0].tile_stats(*TILE_ORDER[0])
                head.x0, head.a1, head.a2 = stats_in[6], [stats_in[7]], [stats_in[8]]
                head.pos = STEPS
            for p in range(nu - 1):
                units[p].queue += [units[p + 1].tile_stats(*key) for key in TILE_ORDER]
            if hand:
                ahead = make_unit(s_next, r_next * UNIT)
                units[-1].queue += [ahead.tile_stats(*key)
                                    for key in TILE_ORDER[1:] + TILE_ORDER[:1]]

            for p, (s, c0) in enumerate(where):
                if p == 0 and stats_in is None:
                    schedule = cfg["cold"][j]
                else:
                    place = 0 if p == 0 else (2 if (hand and p == nu - 1) else 1)
                    schedule = cfg["loop" if in_loop else "ramp"][place]
                if not in_loop:
                    units[p].run(schedule, lambda pos: None)
                    continue
                u = u0 + p + shift * ups
                k0, k1 = issued(u - 1), issued(u)

                def delayed(pos, k0=k0, k1=k1):
                    if pos in cfg["bulk_at"]:
                        first = cfg["bulk_at"].index(pos) * per_slot
                        for i in range(first, first + per_slot):
                            row = (k0 & 1) * (per_unit * rb) + i * rb
                            pl.when(k0 < k1)(functools.partial(
                                write_back, pl.ds((k0 >> 1) * gs, gs),
                                pl.ds(pl.multiple_of(row, 8), rb)))

                now = u >= fine
                if p == nu - 1:
                    now = now & (u < n_units - 1)

                    def on_store(r0, c, s=s, u=u):
                        pl.when(u == n_units - 1)(functools.partial(
                            write_back, s, pl.ds(r0, Q), pl.ds(c, 2 * L)))
                    units[p].on_store = on_store
                units[p].run(schedule, delayed)

                @pl.when(now)
                def _(s=s, c0=c0):
                    for c in range(c0, c0 + UNIT, L):
                        write_back(s, slice(None), pl.ds(c, L))

            if not hand:
                return None
            head = ahead.tile_stats(*TILE_ORDER[0])
            assert head.left() == 0
            return (*[v for key in TILE_ORDER[1:] for v in ahead.norm(*key)],
                    head.x0, head.a1[0], head.a2[0])

        j = u0 = 0
        stats = None
        for nu, count, hand in plan:
            if count == 1:
                stats = do_chunk(j, u0, nu, 0, stats, hand, False)
            else:
                assert nu % ups == 0 and u0 % ups == 0

                def body(it, carry, j=j, u0=u0, nu=nu):
                    return do_chunk(j + it, u0, nu, it * (nu // ups), carry, True, True)
                lax.fori_loop(0, count, body, stats)
            j += count
            u0 += nu * count
        pltpu.make_async_copy(obuf, o_hbm, osem.at[0]).wait()

    out = pl.pallas_call(
        kernel,
        in_specs=[pl.BlockSpec(memory_space=pl.ANY)] * 4,
        out_specs=pl.BlockSpec(memory_space=pl.ANY),
        out_shape=jax.ShapeDtypeStruct((S, D, B), x.dtype),
        scratch_shapes=[
            pltpu.VMEM((S, D, B + 2 * L), BF16),
            pltpu.VMEM((S, D, B), BF16),
            pltpu.VMEM((D, D), BF16),
            pltpu.VMEM((D,), BF16),
            pltpu.VMEM((D,), BF16),
            *[pltpu.VMEM(((H if n in LONG else Q) // 2, L), U32) for n in names],
            pltpu.VMEM((H, L), F32),
            pltpu.SemaphoreType.DMA((n_chunks,)),
            pltpu.SemaphoreType.DMA((n_chunks,)),
            pltpu.SemaphoreType.DMA((1,)),
            pltpu.SemaphoreType.DMA((4,)),
        ],
        compiler_params=pltpu.CompilerParams(
            vmem_limit_bytes=110 * 1024 * 1024,
            disable_bounds_checks=True,
            disable_semaphore_checks=True,
        ),
    )(xt, g, b, w)
    return jnp.transpose(out, (2, 0, 1))


@jax.jit
def pallas_standalone__layernorm_linear__sampling_kernel(
    x: jax.Array,
    g: jax.Array,
    b: jax.Array,
    w: jax.Array,
):
    return _forward(CONFIG, x, g, b, w)
```

```python
import functools

import jax
import jax.numpy as jnp
from jax import lax
import jax.experimental.pallas as pl
import jax.experimental.pallas.tpu as pltpu

EPS = 1e-5
F32 = jnp.float32
BF16 = jnp.bfloat16
U32 = jnp.uint32

L = 128
H = 288
Q = 144
KH = 256
KS = 192
KM = 2 * KH
UNIT = 512
STEPS = 72

LONG = tuple("S%d%s" % (i, h) for i in range(1, 8) for h in "ab") + ("R1", "R6", "R7")
LEVEL2 = ("S2", "S3", "S4", "S5")
SWAPPED = ("S2", "S5")
SHORT = tuple("%sm%d" % (p, k) for p in LEVEL2 for k in range(1, 8))
USES = {
    "S1": (("11", 1), ("22", -1)), "S2": (("21", 1), ("22", 1)),
    "S3": (("12", 1), ("22", 1)), "S4": (("11", 1), ("21", 1)),
    "S5": (("11", 1), ("12", 1)), "S6": (("22", 1),), "S7": (("11", 1),),
    "R1": (("12", -1), ("21", 1)), "R6": (("12", 1),), "R7": (("21", 1),),
    "D": (("21", 1), ("22", 1)),
}
TERMS = {"11": 4, "12": 4, "21": 5, "22": 5}
USES2 = {1: ((0, 0, 1), (1, 1, -1)), 2: ((1, 0, 1), (1, 1, 1)), 3: ((0, 1, 1), (1, 1, 1)),
         4: ((0, 0, 1), (1, 0, 1)), 5: ((0, 0, 1), (0, 1, 1)), 6: ((1, 1, 1),),
         7: ((0, 0, 1),)}
TERMS2 = {(0, 0): 4, (0, 1): 2, (1, 0): 2, (1, 1): 4}
TILE_ORDER = ((0, 0), (1, 0), (0, 1), (1, 1))

_ROWS = ("A:D B:D S4m6 S4m1 S4m7 S4m2", "S4m4 S4m3 S4m5 S5m6", "S5m2 S5m4 S5m3 S5m5",
         "S5m1 S5m7 S3m4 S3m2", "S3m5 S3m3 S3m1 S3m6", "S3m7 S2m1 S2m7 S2m6",
         "A:R7 B:R7 S2m4 S2m2", "S2m5 S2m3", "A:S1a A:S1b B:S1a B:S1b",
         "A:R1 B:R1 A:R6 B:R6", "A:S7a A:S7b B:S7a B:S7b", "A:S6a A:S6b B:S6a B:S6b")
_ROWS_COLD = ("A:D A:S1a A:S1b A:R7 A:R1", "A:R6 A:S7a A:S7b A:S6a", "S4m1 S4m7 S4m6 S4m2",
              "S4m4 S4m3 S4m5 S2m1", "S2m6 S2m2 S2m4 S2m3", "S2m5 S2m7 S3m4 S3m2",
              "S3m5 S3m3 S3m1 S3m6", "B:D S3m7 S5m1 S5m7 S5m6", "A:S6b B:R7 S5m2 S5m4",
              "S5m3 S5m5", "B:S1a B:S1b B:R1 B:R6", "B:S7a B:S7b B:S6a B:S6b")
_ROWS_COLD0 = ("A:S4a A:S4b A:Q3a A:Q3b", "B:P4a B:P4b B:P3a B:P3b",
               "A:V3 A:D A:R7 A:R1 A:R6 A:S1a", "A:S1b A:S7a A:S7b A:S6a",
               "A:S6b B:V4 B:V3 B:D B:R7 B:R1 B:R6", "S2m2 S2m4 S2m3 S2m5",
               "S2m6 S2m1 S2m7 S5m1", "S5m7 S5m6 S5m2 S5m4", "B:S1a B:S1b S5m3 S5m5",
               "B:S7a B:S7b B:S6a B:S6b")


def _schedule(rows, weights):
    out = []
    for row, steps in zip(rows, weights, strict=True):
        toks = row.split()
        passes = [t for t in toks if not (t.endswith(":D") or ":V" in t)]
        for t in toks:
            n = 0
            if t in passes:
                k = passes.index(t)
                n = steps * (k + 1) // len(passes) - steps * k // len(passes)
            out.append((t, n))
    return tuple(out)


CONFIG = dict(
    plan=((1, 1, False), (2, 1, False), (4, 1, True), (7, 1, True), (10, 5, True)),
    ramp=(_schedule(_ROWS, (0, 0, 44, 28, 8, 12, 20, 32, 60, 0, 28, 56)),
          _schedule(_ROWS, (4, 20, 40, 8, 28, 4, 28, 12, 32, 32, 28, 52)),
          _schedule(_ROWS, (32, 24, 12, 28, 24, 0, 12, 24, 20, 28, 28, 56))),
    loop=(_schedule(_ROWS, (0, 20, 28, 20, 64, 36, 12, 16, 20, 20, 52, 0)),
          _schedule(_ROWS, (12, 16, 40, 12, 20, 12, 20, 20, 28, 24, 28, 56)),
          _schedule(_ROWS, (12, 32, 24, 16, 20, 28, 12, 20, 12, 28, 32, 52))),
    cold=(_schedule(_ROWS_COLD0, (0, 20, 0, 56, 0, 8, 60, 0, 0, 0)),
          _schedule(_ROWS_COLD, (0, 60, 64, 16, 36, 36, 40, 0, 28, 28, 60, 64)),
          _schedule(_ROWS_COLD, (0, 56, 64, 20, 28, 24, 20, 40, 28, 24, 56, 72))),
    gate_row=120,
    write_start=30,
    write_fine=48,
    bulk_slices=4,
    bulk_rows=24,
    bulk_per_unit=12,
    bulk_at=(3, 11, 12, 17, 18, 21, 25, 26, 28, 36, 42, 46),
)


def _pack(v):
    return pltpu.bitcast(v.astype(BF16), U32)


def _prep_first(g_ref, w_ref, ref, used, d_model, rows=16):
    g = g_ref[...].astype(F32).reshape(1, d_model)
    wt = jnp.concatenate([w_ref[0:L, :], w_ref[KH:KH + L, :]], axis=0).T
    keep = {}
    for r0 in range(0, H, rows):
        a11, a12, a21, a22 = [
            wt[h * H + r0:h * H + r0 + rows, k * L:(k + 1) * L].astype(F32)
            * g[:, k * KH:k * KH + L] for h in range(2) for k in range(2)]
        xs = (a11 + a22, a21 + a22, a11, a22, a11 + a12, a11 - a21, a12 - a22)
        for k in range(7):
            name = "S%da" % (k + 1)
            if name in used:
                ref[name][r0 // 2:(r0 + rows) // 2, :] = _pack(xs[k])
            keep[name, r0] = xs[k]
    for r0 in range(0, Q, rows):
        for p in LEVEL2:
            x11, x21 = keep[p + "a", r0], keep[p + "a", Q + r0]
            if p in SWAPPED:
                x11, x21 = x21, x11
            ref[p + "m3"][r0 // 2:(r0 + rows) // 2, :] = _pack(x11)
            ref[p + "m6"][r0 // 2:(r0 + rows) // 2, :] = _pack(x11 - x21)
    return keep


def _prep_rest(g_ref, b_ref, w_ref, ref, dl_ref, used, keep, d_model, rows=16):
    w = w_ref[...]
    g = g_ref[...].astype(F32).reshape(1, d_model)
    wt = jnp.concatenate([w[L:KH], w[KH + L:KM]], axis=0).T
    gt = jnp.concatenate([g[:, KM:d_model]] * 2, axis=1)
    at = jnp.concatenate([w[KM:d_model]] * 2, axis=0).T
    brow = jnp.broadcast_to(b_ref[...].astype(F32).reshape(1, d_model), (16, d_model))
    drow = jnp.dot(brow.astype(BF16), w, preferred_element_type=F32)
    row = lax.broadcasted_iota(jnp.int32, (16, d_model), 0)
    lo = drow - drow.astype(BF16).astype(F32)
    e = jnp.where(row == 0, drow, jnp.where(row == 1, lo, 0.0))
    z = jnp.zeros((48, d_model), F32)
    et = jnp.concatenate([e, z, e, z], axis=0).astype(BF16).T
    low = lax.broadcasted_iota(jnp.int32, (rows, L), 1) < 64

    def sel(p, q):
        return jnp.where(low, p, q)

    def level1(r0):
        a11, a12, a21, a22 = [
            wt[h * H + r0:h * H + r0 + rows, k * L:(k + 1) * L].astype(F32)
            * g[:, k * KH + L:(k + 1) * KH] for h in range(2) for k in range(2)]
        at1 = at[r0:r0 + rows].astype(F32) * gt
        at2 = at[H + r0:H + r0 + rows].astype(F32) * gt
        e1 = et[r0:r0 + rows].astype(F32)
        s6, s7 = a11 - a21, a12 - a22
        xs = (sel(a11 + a22, e1), a21 + a22, sel(a11, a21), sel(a22, a12),
              a11 + a12, sel(s6, at2), sel(s7, at1))
        res = {"S%db" % (k + 1): xs[k] for k in range(7)}
        res["R1"] = sel(-e1, a21 + a12)
        res["R6"] = sel(at1, -s6)
        res["R7"] = sel(at2, -s7)
        for name in res:
            if name in used:
                ref[name][r0 // 2:(r0 + rows) // 2, :] = _pack(res[name])
        return res

    for r0 in range(0, Q, rows):
        u, v = level1(r0), level1(Q + r0)
        for p in LEVEL2:
            x11, x12 = keep[p + "a", r0], u[p + "b"]
            x21, x22 = keep[p + "a", Q + r0], v[p + "b"]
            if p in SWAPPED:
                x11, x12, x21, x22 = x21, x22, x11, x12
            xs = {1: x11 + x22, 2: x21 + x22, 4: x22, 5: x11 + x12, 7: x12 - x22}
            for k in xs:
                ref["%sm%d" % (p, k)][r0 // 2:(r0 + rows) // 2, :] = _pack(xs[k])
    low2 = lax.broadcasted_iota(jnp.int32, (H, L), 1) < 64
    lhs = jnp.where(low2, et[H:d_model], et[0:H])
    dl_ref[...] = jnp.dot(lhs, jnp.ones((L, L), BF16), preferred_element_type=F32)


class _Stats:
    def __init__(self, x_ref, d_model, chains=1):
        self.x_ref, self.d_model = x_ref, d_model
        self.pos = 0
        self.x0 = None
        self.a1 = [None] * chains
        self.a2 = [None] * chains
        self.pending = []
        self.result = None

    def left(self):
        return STEPS - self.pos

    def advance(self, n):
        if self.x0 is None:
            self.x0 = self.x_ref[0:16, :].astype(F32)[0:1, :]
        for _ in range(n):
            if not self.pending:
                r0 = self.pos * 8
                t = self.x_ref[r0:r0 + 16, :].astype(F32) - self.x0
                self.pending = [t[0:8], t[8:16]]
            t = self.pending.pop(0)
            c = self.pos % len(self.a1)
            self.a1[c] = t if self.a1[c] is None else self.a1[c] + t
            self.a2[c] = t * t if self.a2[c] is None else self.a2[c] + t * t
            self.pos += 1
        return self.a2[0]

    def finish(self):
        if self.result is None:
            self.advance(self.left())
            a1 = functools.reduce(lambda u, v: u + v, self.a1)
            a2 = functools.reduce(lambda u, v: u + v, self.a2)
            s1 = jnp.sum(a1, axis=0, keepdims=True) * (1.0 / self.d_model)
            s2 = jnp.sum(a2, axis=0, keepdims=True) * (1.0 / self.d_model)
            var = jnp.maximum(s2 - s1 * s1, 0.0)
            self.result = (self.x0 + s1, lax.rsqrt(var + EPS))
        return self.result


def _signed_add(cur, v, sign):
    if cur is None:
        return v, sign
    val, cur_sign = cur
    if cur_sign == 1:
        return (val + v if sign == 1 else val - v), 1
    return (v - val, 1) if sign == 1 else (val + v, -1)


class _Unit:
    def __init__(self, xs_ref, os_ref, ref, dl_ref, c0, d_model, gate_row):
        self.xs_ref, self.os_ref, self.ref, self.dl_ref = xs_ref, os_ref, ref, dl_ref
        self.c0, self.d_model, self.gate_row = c0, d_model, gate_row
        self.stats = {}
        self.cache = {}
        self.queue = []
        self.on_store = None

    def col(self, pair, j):
        return self.c0 + (pair + 2 * j) * L

    def tile_stats(self, pair, j, chains=1):
        if (pair, j) not in self.stats:
            self.stats[pair, j] = _Stats(
                self.xs_ref.at[:, pl.ds(self.col(pair, j), L)], self.d_model, chains)
        return self.stats[pair, j]

    def norm(self, pair, j):
        return self.tile_stats(pair, j).finish()

    def x(self, pair, k, j, r0, r1):
        c = self.col(pair, j)
        return self.xs_ref[k * KH + r0:k * KH + r1, c:c + L].astype(F32)

    def hat(self, pair, k, j, r0, r1):
        m, r = self.norm(pair, j)
        return (self.x(pair, k, j, r0, r1) - m) * r

    def tail(self, pair, j):
        if ("tail", pair, j) not in self.cache:
            self.cache["tail", pair, j] = self.hat(pair, 2, j, 0, 64)
        return self.cache["tail", pair, j]

    def cross(self, pair, ka, kb, r0, r1):
        (ma, ra), (mb, rb) = self.norm(pair, 0), self.norm(pair, 1)
        if ("mr", pair) not in self.cache:
            self.cache["mr", pair] = ma * ra - mb * rb
        return (self.x(pair, ka, 0, r0, r1) * ra - self.x(pair, kb, 1, r0, r1) * rb
                - self.cache["mr", pair])

    def rhs(self, pair, name, raw=None):
        row = lax.broadcasted_iota(jnp.int32, (16, L), 0)
        ones = jnp.where(row < 2, 1.0, 0.0)

        def cat(*parts):
            return jnp.concatenate(parts, axis=0)

        if name == "R1":
            return cat(ones, jnp.zeros((48, L), F32), self.cross(pair, 0, 1, KS, KH))
        if name == "R6":
            return cat(self.tail(pair, 1), self.cross(pair, 0, 0, KS, KH))
        if name == "R7":
            return cat(self.tail(pair, 0), self.cross(pair, 1, 1, KS, KH))
        prod, r0 = name[:2], (0 if name[2] == "a" else L)
        if prod in ("S3", "S4"):
            j = 1 if prod == "S3" else 0
            diff = self.x(pair, 1 - j, j, r0, r0 + L) - self.x(pair, j, j, r0, r0 + L)
            if raw == "P":
                return diff
            if raw == "Q":
                return diff + jnp.minimum(self.norm(pair, 0)[1], 0.0)
            return diff * self.norm(pair, j)[1]
        main = {"S1": lambda a, b: self.cross(pair, 0, 1, a, b),
                "S2": lambda a, b: self.hat(pair, 0, 0, a, b),
                "S5": lambda a, b: self.hat(pair, 1, 1, a, b),
                "S6": lambda a, b: self.cross(pair, 0, 0, a, b),
                "S7": lambda a, b: self.cross(pair, 1, 1, a, b)}[prod]
        if r0 == 0:
            return main(0, L)
        rest = {"S1": lambda: ones,
                "S2": lambda: self.hat(pair, 1, 1, KS, KH),
                "S5": lambda: self.hat(pair, 0, 0, KS, KH),
                "S6": lambda: self.tail(pair, 1),
                "S7": lambda: self.tail(pair, 0)}[prod]
        return cat(main(L, KS), rest())

    def rhs2(self, prod, k):
        def h(kk, pair):
            if ("h", prod, kk, pair) not in self.cache:
                self.cache["h", prod, kk, pair] = self.rhs(pair, prod + "ab"[kk])
            return self.cache["h", prod, kk, pair]

        return {1: lambda: h(0, 0) - h(1, 1), 2: lambda: h(0, 0),
                3: lambda: h(0, 1) - h(1, 1), 4: lambda: h(1, 0) - h(0, 0),
                5: lambda: h(1, 1), 6: lambda: h(0, 0) - h(0, 1),
                7: lambda: h(1, 0) - h(1, 1)}[k]()

    def run(self, schedule, before_token):
        acc, count, done = {}, {}, {}
        acc2, count2, part = {}, {}, {}

        def add(pair, half, name, v):
            for key, sign in USES[name]:
                k = (pair, half, key)
                acc[k] = _signed_add(acc.get(k), v, sign)
                count[k] = count.get(k, 0) + 1
                if count[k] == TERMS[key]:
                    val, val_sign = acc[k]
                    assert val_sign == 1
                    done[k] = val
                    if (1 - pair, half, key) in done:
                        r0 = (0 if key[0] == "1" else H) + half * Q
                        c = self.col(0, int(key[1]) - 1)
                        both = jnp.concatenate(
                            [done[0, half, key], done[1, half, key]], axis=1)
                        self.os_ref[r0:r0 + Q, c:c + 2 * L] = both.astype(BF16)
                        if self.on_store is not None:
                            self.on_store(r0, c)

        def add_full(pair, name, v):
            add(pair, 0, name, v[0:Q])
            add(pair, 1, name, v[Q:H])

        for pos, (token, steps) in enumerate(schedule):
            before_token(pos)
            gate = None
            while steps > 0 and self.queue:
                n = min(steps, self.queue[0].left())
                gate = self.queue[0].advance(n)
                steps -= n
                if self.queue[0].left() == 0:
                    gate = jnp.broadcast_to(self.queue.pop(0).finish()[1], (8, L))

            def dot(name, q, gate=gate):
                if gate is not None:
                    g0 = self.gate_row if q.shape[0] > self.gate_row else 0
                    parts = [q[0:g0]] if g0 else []
                    parts.append(q[g0:g0 + 8] + jnp.minimum(gate, 0.0))
                    if g0 + 8 < q.shape[0]:
                        parts.append(q[g0 + 8:])
                    q = jnp.concatenate(parts, axis=0)
                p = pltpu.bitcast(self.ref[name][...], BF16)[:, 0:q.shape[0]]
                return jnp.dot(p, q.astype(BF16), preferred_element_type=F32)

            if ":" not in token:
                prod, k = token[:2], int(token[3])
                v = dot(token, self.rhs2(prod, k))
                for half, pair, sign in USES2[k]:
                    kk = (prod, half, pair)
                    acc2[kk] = _signed_add(acc2.get(kk), v, sign)
                    count2[kk] = count2.get(kk, 0) + 1
                    if count2[kk] == TERMS2[half, pair]:
                        val, val_sign = acc2[kk]
                        assert val_sign == 1
                        add(pair, 1 - half if prod in SWAPPED else half, prod, val)
                continue
            pair, name = "AB".index(token[0]), token[2:]
            if name == "D":
                add_full(pair, "D", self.dl_ref[...])
                continue
            if name[0] == "V":
                prod = "S" + name[1]
                scale = self.norm(pair, 1 if prod == "S3" else 0)[1]
                add_full(pair, prod, part.pop((pair, prod)) * scale)
                continue
            raw = name[0] if name[0] in "PQ" else None
            name = "S" + name[1:] if raw else name
            v = dot(name, self.rhs(pair, name, raw))
            prod = name[:2]
            if prod[0] == "R":
                add_full(pair, prod, v)
            elif (pair, prod) not in part:
                part[pair, prod] = v
            elif raw:
                part[pair, prod] = v + part[pair, prod]
            else:
                add_full(pair, prod, v + part.pop((pair, prod)))
        assert len(done) == 16


def _forward(cfg, x, g, b, w):
    B, S, D = x.shape
    assert D == 2 * H == KM + 64 == 8 * STEPS
    plan = cfg["plan"]
    ups = B // UNIT
    n_units = S * ups
    assert sum(u * n for u, n, _ in plan) == n_units
    n_chunks = sum(n for _, n, _ in plan)
    names = LONG + SHORT
    used = {t[2:].replace("P", "S").replace("Q", "S")
            for sched in (*cfg["loop"], *cfg["cold"]) for t, _ in sched if ":" in t}
    fine, per_unit = cfg["write_fine"], cfg["bulk_per_unit"]
    gs, rb = cfg["bulk_slices"], cfg["bulk_rows"]
    nrb = D // rb

    assert nrb == 2 * per_unit and gs * ups == 8
    per_slot = per_unit // len(cfg["bulk_at"])
    assert per_slot * len(cfg["bulk_at"]) == per_unit

    def issued(u, lo=jnp.minimum, hi=jnp.maximum):
        def ready(v):
            return 2 * (lo(v, fine) >> 3)
        n = lo(lo(u - cfg["write_start"] + 1, ready(u)), ready(u - 1) + 1)
        return hi(n, 0)

    loop_start = sum(u * n for u, n, _ in plan[:-1])
    table = {u: issued(u, min, max) for u in range(loop_start - 1, n_units)}
    assert table[loop_start - 1] == 0 and fine >= loop_start and fine % (gs * ups) == 0
    assert all(0 <= table[u] - table[u - 1] <= 1 for u in range(loop_start, n_units))
    assert all(table[u] <= 2 * (u // (gs * ups)) for u in table)
    assert table[n_units - 1] == 2 * fine // (gs * ups)
    assert all(n == 1 for _, n, _ in plan[:-1]) and plan[-1][2] and plan[-2][2]

    xt = jnp.transpose(x, (1, 2, 0))

    def kernel(x_hbm, g_hbm, b_hbm, w_hbm, o_hbm, xbuf, obuf, wbuf, gbuf, bbuf, *rest):
        ref = dict(zip(names, rest))
        dl_ref, isem, nsem, osem, wsem = rest[len(names):]

        def copies(sem, u, end, shift=0):
            res = []
            while u < end:
                s, r = divmod(u, ups)
                if r == 0 and end - u >= ups:
                    idx = (pl.ds(s + shift, (end - u) // ups), slice(None), pl.ds(0, B))
                    u += (end - u) // ups * ups
                else:
                    idx = (s + shift, slice(None), pl.ds(r * UNIT, UNIT))
                    u += 1
                res.append(pltpu.make_async_copy(x_hbm.at[idx], xbuf.at[idx], sem))
            return res

        def write_back(*idx):
            pltpu.make_async_copy(obuf.at[idx], o_hbm.at[idx], osem.at[0]).start()

        def w_rows(r0, r1, k):
            rows = pl.ds(r0, r1 - r0)
            return pltpu.make_async_copy(w_hbm.at[rows], wbuf.at[rows], wsem.at[k])

        cg = pltpu.make_async_copy(g_hbm, gbuf, wsem.at[1])
        cb = pltpu.make_async_copy(b_hbm, bbuf, wsem.at[2])
        w_first = [w_rows(0, L, 0), w_rows(KH, KH + L, 0)]
        w_rest = [w_rows(L, KH, 3), w_rows(KH + L, D, 3)]
        for c in [cg, cb] + w_first + w_rest:
            c.start()
        cg.wait()
        cb.wait()
        j = u0 = 0
        handed = False
        for nu, count, hand in plan:
            for _ in range(count):
                for c in copies(isem.at[j], u0 + handed, u0 + nu):
                    c.start()
                if hand and u0 + nu < n_units:
                    for c in copies(nsem.at[j], u0 + nu, u0 + nu + 1):
                        c.start()
                j += 1
                u0 += nu
                handed = hand
        for c in w_first:
            c.wait()
        keep = _prep_first(gbuf, wbuf, ref, used, D)
        for c in w_rest:
            c.wait()
        _prep_rest(gbuf, bbuf, wbuf, ref, dl_ref, used, keep, D)

        def make_unit(s, c0):
            return _Unit(xbuf.at[s], obuf.at[s], ref, dl_ref, c0, D, cfg["gate_row"])

        def do_chunk(j, u0, nu, shift, stats_in, hand, in_loop):
            for c in copies(isem.at[j], u0 + (stats_in is not None), u0 + nu, shift):
                c.wait()
            if hand:
                s_next, r_next = divmod(u0 + nu, ups)
                if in_loop:
                    exists = s_next + shift < S
                    s_next = jnp.minimum(s_next + shift, S - 1)

                    @pl.when(exists)
                    def _():
                        copies(nsem.at[j], r_next, r_next + 1, s_next)[0].wait()
                else:
                    copies(nsem.at[j], u0 + nu, u0 + nu + 1)[0].wait()
            where = [(u // ups + shift, (u % ups) * UNIT) for u in range(u0, u0 + nu)]
            units = [make_unit(s, c0) for s, c0 in where]
            if stats_in is None:
                units[0].tile_stats(0, 0, chains=2)
                units[0].queue = [units[0].tile_stats(1, 0), units[0].tile_stats(1, 1)]
            else:
                for n, key in enumerate(TILE_ORDER[1:]):
                    units[0].tile_stats(*key).result = stats_in[2 * n:2 * n + 2]
                head = units[0].tile_stats(*TILE_ORDER[0])
                head.x0, head.a1, head.a2 = stats_in[6], [stats_in[7]], [stats_in[8]]
                head.pos = STEPS
            for p in range(nu - 1):
                units[p].queue += [units[p + 1].tile_stats(*key) for key in TILE_ORDER]
            if hand:
                ahead = make_unit(s_next, r_next * UNIT)
                units[-1].queue += [ahead.tile_stats(*key)
                                    for key in TILE_ORDER[1:] + TILE_ORDER[:1]]

            for p, (s, c0) in enumerate(where):
                if p == 0 and stats_in is None:
                    schedule = cfg["cold"][j]
                else:
                    place = 0 if p == 0 else (2 if (hand and p == nu - 1) else 1)
                    schedule = cfg["loop" if in_loop else "ramp"][place]
                if not in_loop:
                    units[p].run(schedule, lambda pos: None)
                    continue
                u = u0 + p + shift * ups
                k0, k1 = issued(u - 1), issued(u)

                def delayed(pos, k0=k0, k1=k1):
                    if pos in cfg["bulk_at"]:
                        first = cfg["bulk_at"].index(pos) * per_slot
                        for i in range(first, first + per_slot):
                            row = (k0 & 1) * (per_unit * rb) + i * rb
                            pl.when(k0 < k1)(functools.partial(
                                write_back, pl.ds((k0 >> 1) * gs, gs),
                                pl.ds(pl.multiple_of(row, 8), rb)))

                now = u >= fine
                if p == nu - 1:
                    now = now & (u < n_units - 1)

                    def on_store(r0, c, s=s, u=u):
                        pl.when(u == n_units - 1)(functools.partial(
                            write_back, s, pl.ds(r0, Q), pl.ds(c, 2 * L)))
                    units[p].on_store = on_store
                units[p].run(schedule, delayed)

                @pl.when(now)
                def _(s=s, c0=c0):
                    for c in range(c0, c0 + UNIT, L):
                        write_back(s, slice(None), pl.ds(c, L))

            if not hand:
                return None
            head = ahead.tile_stats(*TILE_ORDER[0])
            assert head.left() == 0
            return (*[v for key in TILE_ORDER[1:] for v in ahead.norm(*key)],
                    head.x0, head.a1[0], head.a2[0])

        j = u0 = 0
        stats = None
        for nu, count, hand in plan:
            if count == 1:
                stats = do_chunk(j, u0, nu, 0, stats, hand, False)
            else:
                assert nu % ups == 0 and u0 % ups == 0

                def body(it, carry, j=j, u0=u0, nu=nu):
                    return do_chunk(j + it, u0, nu, it * (nu // ups), carry, True, True)
                lax.fori_loop(0, count, body, stats)
            j += count
            u0 += nu * count
        pltpu.make_async_copy(obuf, o_hbm, osem.at[0]).wait()

    out = pl.pallas_call(
        kernel,
        in_specs=[pl.BlockSpec(memory_space=pl.ANY)] * 4,
        out_specs=pl.BlockSpec(memory_space=pl.ANY),
        out_shape=jax.ShapeDtypeStruct((S, D, B), x.dtype),
        scratch_shapes=[
            pltpu.VMEM((S, D, B + 2 * L), BF16),
            pltpu.VMEM((S, D, B), BF16),
            pltpu.VMEM((D, D), BF16),
            pltpu.VMEM((D,), BF16),
            pltpu.VMEM((D,), BF16),
            *[pltpu.VMEM(((H if n in LONG else Q) // 2, L), U32) for n in names],
            pltpu.VMEM((H, L), F32),
            pltpu.SemaphoreType.DMA((n_chunks,)),
            pltpu.SemaphoreType.DMA((n_chunks,)),
            pltpu.SemaphoreType.DMA((1,)),
            pltpu.SemaphoreType.DMA((4,)),
        ],
        compiler_params=pltpu.CompilerParams(
            vmem_limit_bytes=110 * 1024 * 1024,
            disable_bounds_checks=True,
            disable_semaphore_checks=True,
        ),
    )(xt, g, b, w)
    return jnp.transpose(out, (2, 0, 1))


@jax.jit
def pallas_standalone__layernorm_linear__sampling_kernel(
    x: jax.Array,
    g: jax.Array,
    b: jax.Array,
    w: jax.Array,
):
    return _forward(CONFIG, x, g, b, w)
```

```python
import functools

import jax
import jax.numpy as jnp
from jax import lax
import jax.experimental.pallas as pl
import jax.experimental.pallas.tpu as pltpu

EPS = 1e-5
F32 = jnp.float32
BF16 = jnp.bfloat16
U32 = jnp.uint32

L = 128
H = 288
Q = 144
KH = 256
KS = 192
KM = 2 * KH
UNIT = 512
STEPS = 72

LONG = tuple("S%d%s" % (i, h) for i in range(1, 8) for h in "ab") + ("R1", "R6", "R7")
LEVEL2 = ("S2", "S3", "S4", "S5")
SWAPPED = ("S2", "S5")
SHORT = tuple("%sm%d" % (p, k) for p in LEVEL2 for k in range(1, 8))
USES = {
    "S1": (("11", 1), ("22", -1)), "S2": (("21", 1), ("22", 1)),
    "S3": (("12", 1), ("22", 1)), "S4": (("11", 1), ("21", 1)),
    "S5": (("11", 1), ("12", 1)), "S6": (("22", 1),), "S7": (("11", 1),),
    "R1": (("12", -1), ("21", 1)), "R6": (("12", 1),), "R7": (("21", 1),),
    "D": (("21", 1), ("22", 1)),
}
TERMS = {"11": 4, "12": 4, "21": 5, "22": 5}
USES2 = {1: ((0, 0, 1), (1, 1, -1)), 2: ((1, 0, 1), (1, 1, 1)), 3: ((0, 1, 1), (1, 1, 1)),
         4: ((0, 0, 1), (1, 0, 1)), 5: ((0, 0, 1), (0, 1, 1)), 6: ((1, 1, 1),),
         7: ((0, 0, 1),)}
TERMS2 = {(0, 0): 4, (0, 1): 2, (1, 0): 2, (1, 1): 4}
TILE_ORDER = ((0, 0), (1, 0), (0, 1), (1, 1))

_ROWS = ("A:D B:D S4m6 S4m1 S4m7 S4m2", "S4m4 S4m3 S4m5 S5m6", "S5m2 S5m4 S5m3 S5m5",
         "S5m1 S5m7 S3m4 S3m2", "S3m5 S3m3 S3m1 S3m6", "S3m7 S2m1 S2m7 S2m6",
         "A:R7 B:R7 S2m4 S2m2", "S2m5 S2m3", "A:S1a A:S1b B:S1a B:S1b",
         "A:R1 B:R1 A:R6 B:R6", "A:S7a A:S7b B:S7a B:S7b", "A:S6a A:S6b B:S6a B:S6b")
_ROWS_COLD = ("A:D A:S1a A:S1b A:R7 A:R1", "A:R6 A:S7a A:S7b A:S6a", "S4m1 S4m7 S4m6 S4m2",
              "S4m4 S4m3 S4m5 S2m1", "S2m6 S2m2 S2m4 S2m3", "S2m5 S2m7 S3m4 S3m2",
              "S3m5 S3m3 S3m1 S3m6", "B:D S3m7 S5m1 S5m7 S5m6", "A:S6b B:R7 S5m2 S5m4",
              "S5m3 S5m5", "B:S1a B:S1b B:R1 B:R6", "B:S7a B:S7b B:S6a B:S6b")
_ROWS_COLD0 = ("A:S4a A:S4b A:Q3a A:Q3b", "B:P4a B:P4b B:P3a B:P3b",
               "A:V3 A:D A:R7 A:R1 A:R6 A:S1a", "A:S1b A:S7a A:S7b A:S6a",
               "A:S6b B:V4 B:V3 B:D B:R7 B:R1 B:R6", "S2m2 S2m4 S2m3 S2m5",
               "S2m6 S2m1 S2m7 S5m1", "S5m7 S5m6 S5m2 S5m4", "B:S1a B:S1b S5m3 S5m5",
               "B:S7a B:S7b B:S6a B:S6b")


def _schedule(rows, weights):
    out = []
    for row, steps in zip(rows, weights, strict=True):
        toks = row.split()
        passes = [t for t in toks if not (t.endswith(":D") or ":V" in t)]
        for t in toks:
            n = 0
            if t in passes:
                k = passes.index(t)
                n = steps * (k + 1) // len(passes) - steps * k // len(passes)
            out.append((t, n))
    return tuple(out)


CONFIG = dict(
    plan=((1, 1, False), (1, 1, True), (2, 1, True), (4, 1, True), (6, 1, True),
          (10, 5, True)),
    ramp=(_schedule(_ROWS, (0, 0, 40, 12, 20, 4, 4, 48, 60, 16, 32, 52)),
          _schedule(_ROWS, (4, 20, 40, 8, 24, 4, 28, 12, 32, 36, 28, 52)),
          _schedule(_ROWS, (32, 16, 20, 28, 24, 0, 12, 24, 20, 28, 28, 56))),
    loop=(_schedule(_ROWS, (0, 20, 28, 20, 64, 36, 12, 16, 20, 20, 52, 0)),
          _schedule(_ROWS, (12, 16, 40, 12, 20, 12, 20, 20, 28, 24, 28, 56)),
          _schedule(_ROWS, (12, 32, 24, 16, 20, 28, 12, 20, 12, 28, 32, 52))),
    cold=(_schedule(_ROWS_COLD0, (0, 20, 0, 56, 0, 0, 64, 0, 4, 0)),
          _schedule(_ROWS_COLD, (0, 56, 64, 20, 28, 24, 20, 40, 32, 20, 56, 72))),
    gate_row=120,
    write_start=30,
    write_fine=48,
    bulk_slices=4,
    bulk_rows=24,
    bulk_per_unit=12,
    bulk_at=(3, 11, 12, 17, 18, 21, 25, 26, 28, 36, 42, 46),
)


def _pack(v):
    return pltpu.bitcast(v.astype(BF16), U32)


def _prep_first(g_ref, w_ref, ref, used, d_model, rows=16):
    g = g_ref[...].astype(F32).reshape(1, d_model)
    wt = jnp.concatenate([w_ref[0:L, :], w_ref[KH:KH + L, :]], axis=0).T
    keep = {}
    for r0 in range(0, H, rows):
        a11, a12, a21, a22 = [
            wt[h * H + r0:h * H + r0 + rows, k * L:(k + 1) * L].astype(F32)
            * g[:, k * KH:k * KH + L] for h in range(2) for k in range(2)]
        xs = (a11 + a22, a21 + a22, a11, a22, a11 + a12, a11 - a21, a12 - a22)
        for k in range(7):
            name = "S%da" % (k + 1)
            if name in used:
                ref[name][r0 // 2:(r0 + rows) // 2, :] = _pack(xs[k])
            keep[name, r0] = xs[k]
    for r0 in range(0, Q, rows):
        for p in LEVEL2:
            x11, x21 = keep[p + "a", r0], keep[p + "a", Q + r0]
            if p in SWAPPED:
                x11, x21 = x21, x11
            ref[p + "m3"][r0 // 2:(r0 + rows) // 2, :] = _pack(x11)
            ref[p + "m6"][r0 // 2:(r0 + rows) // 2, :] = _pack(x11 - x21)
    return keep


def _prep_rest(g_ref, b_ref, w_ref, ref, dl_ref, used, keep, d_model, rows=16):
    w = w_ref[...]
    g = g_ref[...].astype(F32).reshape(1, d_model)
    wt = jnp.concatenate([w[L:KH], w[KH + L:KM]], axis=0).T
    gt = jnp.concatenate([g[:, KM:d_model]] * 2, axis=1)
    at = jnp.concatenate([w[KM:d_model]] * 2, axis=0).T
    brow = jnp.broadcast_to(b_ref[...].astype(F32).reshape(1, d_model), (16, d_model))
    drow = jnp.dot(brow.astype(BF16), w, preferred_element_type=F32)
    row = lax.broadcasted_iota(jnp.int32, (16, d_model), 0)
    lo = drow - drow.astype(BF16).astype(F32)
    e = jnp.where(row == 0, drow, jnp.where(row == 1, lo, 0.0))
    z = jnp.zeros((48, d_model), F32)
    et = jnp.concatenate([e, z, e, z], axis=0).astype(BF16).T
    low = lax.broadcasted_iota(jnp.int32, (rows, L), 1) < 64

    def sel(p, q):
        return jnp.where(low, p, q)

    def level1(r0):
        a11, a12, a21, a22 = [
            wt[h * H + r0:h * H + r0 + rows, k * L:(k + 1) * L].astype(F32)
            * g[:, k * KH + L:(k + 1) * KH] for h in range(2) for k in range(2)]
        at1 = at[r0:r0 + rows].astype(F32) * gt
        at2 = at[H + r0:H + r0 + rows].astype(F32) * gt
        e1 = et[r0:r0 + rows].astype(F32)
        s6, s7 = a11 - a21, a12 - a22
        xs = (sel(a11 + a22, e1), a21 + a22, sel(a11, a21), sel(a22, a12),
              a11 + a12, sel(s6, at2), sel(s7, at1))
        res = {"S%db" % (k + 1): xs[k] for k in range(7)}
        res["R1"] = sel(-e1, a21 + a12)
        res["R6"] = sel(at1, -s6)
        res["R7"] = sel(at2, -s7)
        for name in res:
            if name in used:
                ref[name][r0 // 2:(r0 + rows) // 2, :] = _pack(res[name])
        return res

    for r0 in range(0, Q, rows):
        u, v = level1(r0), level1(Q + r0)
        for p in LEVEL2:
            x11, x12 = keep[p + "a", r0], u[p + "b"]
            x21, x22 = keep[p + "a", Q + r0], v[p + "b"]
            if p in SWAPPED:
                x11, x12, x21, x22 = x21, x22, x11, x12
            xs = {1: x11 + x22, 2: x21 + x22, 4: x22, 5: x11 + x12, 7: x12 - x22}
            for k in xs:
                ref["%sm%d" % (p, k)][r0 // 2:(r0 + rows) // 2, :] = _pack(xs[k])
    low2 = lax.broadcasted_iota(jnp.int32, (H, L), 1) < 64
    lhs = jnp.where(low2, et[H:d_model], et[0:H])
    dl_ref[...] = jnp.dot(lhs, jnp.ones((L, L), BF16), preferred_element_type=F32)


class _Stats:
    def __init__(self, x_ref, d_model, chains=1):
        self.x_ref, self.d_model = x_ref, d_model
        self.pos = 0
        self.x0 = None
        self.a1 = [None] * chains
        self.a2 = [None] * chains
        self.pending = []
        self.result = None

    def left(self):
        return STEPS - self.pos

    def advance(self, n):
        if self.x0 is None:
            self.x0 = self.x_ref[0:16, :].astype(F32)[0:1, :]
        for _ in range(n):
            if not self.pending:
                r0 = self.pos * 8
                t = self.x_ref[r0:r0 + 16, :].astype(F32) - self.x0
                self.pending = [t[0:8], t[8:16]]
            t = self.pending.pop(0)
            c = self.pos % len(self.a1)
            self.a1[c] = t if self.a1[c] is None else self.a1[c] + t
            self.a2[c] = t * t if self.a2[c] is None else self.a2[c] + t * t
            self.pos += 1
        return self.a2[0]

    def finish(self):
        if self.result is None:
            self.advance(self.left())
            a1 = functools.reduce(lambda u, v: u + v, self.a1)
            a2 = functools.reduce(lambda u, v: u + v, self.a2)
            s1 = jnp.sum(a1, axis=0, keepdims=True) * (1.0 / self.d_model)
            s2 = jnp.sum(a2, axis=0, keepdims=True) * (1.0 / self.d_model)
            var = jnp.maximum(s2 - s1 * s1, 0.0)
            self.result = (self.x0 + s1, lax.rsqrt(var + EPS))
        return self.result


def _signed_add(cur, v, sign):
    if cur is None:
        return v, sign
    val, cur_sign = cur
    if cur_sign == 1:
        return (val + v if sign == 1 else val - v), 1
    return (v - val, 1) if sign == 1 else (val + v, -1)


class _Unit:
    def __init__(self, xs_ref, os_ref, ref, dl_ref, c0, d_model, gate_row):
        self.xs_ref, self.os_ref, self.ref, self.dl_ref = xs_ref, os_ref, ref, dl_ref
        self.c0, self.d_model, self.gate_row = c0, d_model, gate_row
        self.stats = {}
        self.cache = {}
        self.queue = []
        self.on_store = None

    def col(self, pair, j):
        return self.c0 + (pair + 2 * j) * L

    def tile_stats(self, pair, j, chains=1):
        if (pair, j) not in self.stats:
            self.stats[pair, j] = _Stats(
                self.xs_ref.at[:, pl.ds(self.col(pair, j), L)], self.d_model, chains)
        return self.stats[pair, j]

    def norm(self, pair, j):
        return self.tile_stats(pair, j).finish()

    def x(self, pair, k, j, r0, r1):
        c = self.col(pair, j)
        return self.xs_ref[k * KH + r0:k * KH + r1, c:c + L].astype(F32)

    def hat(self, pair, k, j, r0, r1):
        m, r = self.norm(pair, j)
        return (self.x(pair, k, j, r0, r1) - m) * r

    def tail(self, pair, j):
        if ("tail", pair, j) not in self.cache:
            self.cache["tail", pair, j] = self.hat(pair, 2, j, 0, 64)
        return self.cache["tail", pair, j]

    def cross(self, pair, ka, kb, r0, r1):
        (ma, ra), (mb, rb) = self.norm(pair, 0), self.norm(pair, 1)
        if ("mr", pair) not in self.cache:
            self.cache["mr", pair] = ma * ra - mb * rb
        return (self.x(pair, ka, 0, r0, r1) * ra - self.x(pair, kb, 1, r0, r1) * rb
                - self.cache["mr", pair])

    def rhs(self, pair, name, raw=None):
        row = lax.broadcasted_iota(jnp.int32, (16, L), 0)
        ones = jnp.where(row < 2, 1.0, 0.0)

        def cat(*parts):
            return jnp.concatenate(parts, axis=0)

        if name == "R1":
            return cat(ones, jnp.zeros((48, L), F32), self.cross(pair, 0, 1, KS, KH))
        if name == "R6":
            return cat(self.tail(pair, 1), self.cross(pair, 0, 0, KS, KH))
        if name == "R7":
            return cat(self.tail(pair, 0), self.cross(pair, 1, 1, KS, KH))
        prod, r0 = name[:2], (0 if name[2] == "a" else L)
        if prod in ("S3", "S4"):
            j = 1 if prod == "S3" else 0
            diff = self.x(pair, 1 - j, j, r0, r0 + L) - self.x(pair, j, j, r0, r0 + L)
            if raw == "P":
                return diff
            if raw == "Q":
                return diff + jnp.minimum(self.norm(pair, 0)[1], 0.0)
            return diff * self.norm(pair, j)[1]
        main = {"S1": lambda a, b: self.cross(pair, 0, 1, a, b),
                "S2": lambda a, b: self.hat(pair, 0, 0, a, b),
                "S5": lambda a, b: self.hat(pair, 1, 1, a, b),
                "S6": lambda a, b: self.cross(pair, 0, 0, a, b),
                "S7": lambda a, b: self.cross(pair, 1, 1, a, b)}[prod]
        if r0 == 0:
            return main(0, L)
        rest = {"S1": lambda: ones,
                "S2": lambda: self.hat(pair, 1, 1, KS, KH),
                "S5": lambda: self.hat(pair, 0, 0, KS, KH),
                "S6": lambda: self.tail(pair, 1),
                "S7": lambda: self.tail(pair, 0)}[prod]
        return cat(main(L, KS), rest())

    def rhs2(self, prod, k):
        def h(kk, pair):
            if ("h", prod, kk, pair) not in self.cache:
                self.cache["h", prod, kk, pair] = self.rhs(pair, prod + "ab"[kk])
            return self.cache["h", prod, kk, pair]

        return {1: lambda: h(0, 0) - h(1, 1), 2: lambda: h(0, 0),
                3: lambda: h(0, 1) - h(1, 1), 4: lambda: h(1, 0) - h(0, 0),
                5: lambda: h(1, 1), 6: lambda: h(0, 0) - h(0, 1),
                7: lambda: h(1, 0) - h(1, 1)}[k]()

    def run(self, schedule, before_token):
        acc, count, done = {}, {}, {}
        acc2, count2, part = {}, {}, {}

        def add(pair, half, name, v):
            for key, sign in USES[name]:
                k = (pair, half, key)
                acc[k] = _signed_add(acc.get(k), v, sign)
                count[k] = count.get(k, 0) + 1
                if count[k] == TERMS[key]:
                    val, val_sign = acc[k]
                    assert val_sign == 1
                    done[k] = val
                    if (1 - pair, half, key) in done:
                        r0 = (0 if key[0] == "1" else H) + half * Q
                        c = self.col(0, int(key[1]) - 1)
                        both = jnp.concatenate(
                            [done[0, half, key], done[1, half, key]], axis=1)
                        self.os_ref[r0:r0 + Q, c:c + 2 * L] = both.astype(BF16)
                        if self.on_store is not None:
                            self.on_store(r0, c)

        def add_full(pair, name, v):
            add(pair, 0, name, v[0:Q])
            add(pair, 1, name, v[Q:H])

        for pos, (token, steps) in enumerate(schedule):
            before_token(pos)
            gate = None
            while steps > 0 and self.queue:
                n = min(steps, self.queue[0].left())
                gate = self.queue[0].advance(n)
                steps -= n
                if self.queue[0].left() == 0:
                    gate = jnp.broadcast_to(self.queue.pop(0).finish()[1], (8, L))

            def dot(name, q, gate=gate):
                if gate is not None:
                    g0 = self.gate_row if q.shape[0] > self.gate_row else 0
                    parts = [q[0:g0]] if g0 else []
                    parts.append(q[g0:g0 + 8] + jnp.minimum(gate, 0.0))
                    if g0 + 8 < q.shape[0]:
                        parts.append(q[g0 + 8:])
                    q = jnp.concatenate(parts, axis=0)
                p = pltpu.bitcast(self.ref[name][...], BF16)[:, 0:q.shape[0]]
                return jnp.dot(p, q.astype(BF16), preferred_element_type=F32)

            if ":" not in token:
                prod, k = token[:2], int(token[3])
                v = dot(token, self.rhs2(prod, k))
                for half, pair, sign in USES2[k]:
                    kk = (prod, half, pair)
                    acc2[kk] = _signed_add(acc2.get(kk), v, sign)
                    count2[kk] = count2.get(kk, 0) + 1
                    if count2[kk] == TERMS2[half, pair]:
                        val, val_sign = acc2[kk]
                        assert val_sign == 1
                        add(pair, 1 - half if prod in SWAPPED else half, prod, val)
                continue
            pair, name = "AB".index(token[0]), token[2:]
            if name == "D":
                add_full(pair, "D", self.dl_ref[...])
                continue
            if name[0] == "V":
                prod = "S" + name[1]
                scale = self.norm(pair, 1 if prod == "S3" else 0)[1]
                add_full(pair, prod, part.pop((pair, prod)) * scale)
                continue
            raw = name[0] if name[0] in "PQ" else None
            name = "S" + name[1:] if raw else name
            v = dot(name, self.rhs(pair, name, raw))
            prod = name[:2]
            if prod[0] == "R":
                add_full(pair, prod, v)
            elif (pair, prod) not in part:
                part[pair, prod] = v
            elif raw:
                part[pair, prod] = v + part[pair, prod]
            else:
                add_full(pair, prod, v + part.pop((pair, prod)))
        assert len(done) == 16


def _forward(cfg, x, g, b, w):
    B, S, D = x.shape
    assert D == 2 * H == KM + 64 == 8 * STEPS
    plan = cfg["plan"]
    ups = B // UNIT
    n_units = S * ups
    assert sum(u * n for u, n, _ in plan) == n_units
    n_chunks = sum(n for _, n, _ in plan)
    names = LONG + SHORT
    used = {t[2:].replace("P", "S").replace("Q", "S")
            for sched in (*cfg["loop"], *cfg["cold"]) for t, _ in sched if ":" in t}
    fine, per_unit = cfg["write_fine"], cfg["bulk_per_unit"]
    gs, rb = cfg["bulk_slices"], cfg["bulk_rows"]
    nrb = D // rb

    assert nrb == 2 * per_unit and gs * ups == 8
    per_slot = per_unit // len(cfg["bulk_at"])
    assert per_slot * len(cfg["bulk_at"]) == per_unit

    def issued(u, lo=jnp.minimum, hi=jnp.maximum):
        def ready(v):
            return 2 * (lo(v, fine) >> 3)
        n = lo(lo(u - cfg["write_start"] + 1, ready(u)), ready(u - 1) + 1)
        return hi(n, 0)

    loop_start = sum(u * n for u, n, _ in plan[:-1])
    table = {u: issued(u, min, max) for u in range(loop_start - 1, n_units)}
    assert table[loop_start - 1] == 0 and fine >= loop_start and fine % (gs * ups) == 0
    assert all(0 <= table[u] - table[u - 1] <= 1 for u in range(loop_start, n_units))
    assert all(table[u] <= 2 * (u // (gs * ups)) for u in table)
    assert table[n_units - 1] == 2 * fine // (gs * ups)
    assert all(n == 1 for _, n, _ in plan[:-1]) and plan[-1][2] and plan[-2][2]

    xt = jnp.transpose(x, (1, 2, 0))

    def kernel(x_hbm, g_hbm, b_hbm, w_hbm, o_hbm, xbuf, obuf, wbuf, gbuf, bbuf, *rest):
        ref = dict(zip(names, rest))
        dl_ref, isem, nsem, osem, wsem = rest[len(names):]

        def copies(sem, u, end, shift=0):
            res = []
            while u < end:
                s, r = divmod(u, ups)
                if r == 0 and end - u >= ups:
                    idx = (pl.ds(s + shift, (end - u) // ups), slice(None), pl.ds(0, B))
                    u += (end - u) // ups * ups
                else:
                    idx = (s + shift, slice(None), pl.ds(r * UNIT, UNIT))
                    u += 1
                res.append(pltpu.make_async_copy(x_hbm.at[idx], xbuf.at[idx], sem))
            return res

        def write_back(*idx):
            pltpu.make_async_copy(obuf.at[idx], o_hbm.at[idx], osem.at[0]).start()

        def w_rows(r0, r1, k):
            rows = pl.ds(r0, r1 - r0)
            return pltpu.make_async_copy(w_hbm.at[rows], wbuf.at[rows], wsem.at[k])

        cg = pltpu.make_async_copy(g_hbm, gbuf, wsem.at[1])
        cb = pltpu.make_async_copy(b_hbm, bbuf, wsem.at[2])
        w_first = [w_rows(0, L, 0), w_rows(KH, KH + L, 0)]
        w_rest = [w_rows(L, KH, 3), w_rows(KH + L, D, 3)]
        for c in [cg, cb] + w_first + w_rest:
            c.start()
        cg.wait()
        cb.wait()
        j = u0 = 0
        handed = False
        for nu, count, hand in plan:
            for _ in range(count):
                for c in copies(isem.at[j], u0 + handed, u0 + nu):
                    c.start()
                if hand and u0 + nu < n_units:
                    for c in copies(nsem.at[j], u0 + nu, u0 + nu + 1):
                        c.start()
                j += 1
                u0 += nu
                handed = hand
        for c in w_first:
            c.wait()
        keep = _prep_first(gbuf, wbuf, ref, used, D)
        for c in w_rest:
            c.wait()
        _prep_rest(gbuf, bbuf, wbuf, ref, dl_ref, used, keep, D)

        def make_unit(s, c0):
            return _Unit(xbuf.at[s], obuf.at[s], ref, dl_ref, c0, D, cfg["gate_row"])

        def do_chunk(j, u0, nu, shift, stats_in, hand, in_loop):
            for c in copies(isem.at[j], u0 + (stats_in is not None), u0 + nu, shift):
                c.wait()
            if hand:
                s_next, r_next = divmod(u0 + nu, ups)
                if in_loop:
                    exists = s_next + shift < S
                    s_next = jnp.minimum(s_next + shift, S - 1)

                    @pl.when(exists)
                    def _():
                        copies(nsem.at[j], r_next, r_next + 1, s_next)[0].wait()
                else:
                    copies(nsem.at[j], u0 + nu, u0 + nu + 1)[0].wait()
            where = [(u // ups + shift, (u % ups) * UNIT) for u in range(u0, u0 + nu)]
            units = [make_unit(s, c0) for s, c0 in where]
            if stats_in is None:
                units[0].tile_stats(0, 0, chains=2)
                units[0].queue = [units[0].tile_stats(1, 0), units[0].tile_stats(1, 1)]
            else:
                for n, key in enumerate(TILE_ORDER[1:]):
                    units[0].tile_stats(*key).result = stats_in[2 * n:2 * n + 2]
                head = units[0].tile_stats(*TILE_ORDER[0])
                head.x0, head.a1, head.a2 = stats_in[6], [stats_in[7]], [stats_in[8]]
                head.pos = STEPS
            for p in range(nu - 1):
                units[p].queue += [units[p + 1].tile_stats(*key) for key in TILE_ORDER]
            if hand:
                ahead = make_unit(s_next, r_next * UNIT)
                units[-1].queue += [ahead.tile_stats(*key)
                                    for key in TILE_ORDER[1:] + TILE_ORDER[:1]]

            for p, (s, c0) in enumerate(where):
                if p == 0 and stats_in is None:
                    schedule = cfg["cold"][j]
                else:
                    place = 0 if p == 0 else (2 if (hand and p == nu - 1) else 1)
                    schedule = cfg["loop" if in_loop else "ramp"][place]
                if not in_loop:
                    units[p].run(schedule, lambda pos: None)
                    continue
                u = u0 + p + shift * ups
                k0, k1 = issued(u - 1), issued(u)

                def delayed(pos, k0=k0, k1=k1):
                    if pos in cfg["bulk_at"]:
                        first = cfg["bulk_at"].index(pos) * per_slot
                        for i in range(first, first + per_slot):
                            row = (k0 & 1) * (per_unit * rb) + i * rb
                            pl.when(k0 < k1)(functools.partial(
                                write_back, pl.ds((k0 >> 1) * gs, gs),
                                pl.ds(pl.multiple_of(row, 8), rb)))

                now = u >= fine
                if p == nu - 1:
                    now = now & (u < n_units - 1)

                    def on_store(r0, c, s=s, u=u):
                        pl.when(u == n_units - 1)(functools.partial(
                            write_back, s, pl.ds(r0, Q), pl.ds(c, 2 * L)))
                    units[p].on_store = on_store
                units[p].run(schedule, delayed)

                @pl.when(now)
                def _(s=s, c0=c0):
                    for c in range(c0, c0 + UNIT, L):
                        write_back(s, slice(None), pl.ds(c, L))

            if not hand:
                return None
            head = ahead.tile_stats(*TILE_ORDER[0])
            assert head.left() == 0
            return (*[v for key in TILE_ORDER[1:] for v in ahead.norm(*key)],
                    head.x0, head.a1[0], head.a2[0])

        j = u0 = 0
        stats = None
        for nu, count, hand in plan:
            if count == 1:
                stats = do_chunk(j, u0, nu, 0, stats, hand, False)
            else:
                assert nu % ups == 0 and u0 % ups == 0

                def body(it, carry, j=j, u0=u0, nu=nu):
                    return do_chunk(j + it, u0, nu, it * (nu // ups), carry, True, True)
                lax.fori_loop(0, count, body, stats)
            j += count
            u0 += nu * count
        pltpu.make_async_copy(obuf, o_hbm, osem.at[0]).wait()

    out = pl.pallas_call(
        kernel,
        in_specs=[pl.BlockSpec(memory_space=pl.ANY)] * 4,
        out_specs=pl.BlockSpec(memory_space=pl.ANY),
        out_shape=jax.ShapeDtypeStruct((S, D, B), x.dtype),
        scratch_shapes=[
            pltpu.VMEM((S, D, B + 2 * L), BF16),
            pltpu.VMEM((S, D, B), BF16),
            pltpu.VMEM((D, D), BF16),
            pltpu.VMEM((D,), BF16),
            pltpu.VMEM((D,), BF16),
            *[pltpu.VMEM(((H if n in LONG else Q) // 2, L), U32) for n in names],
            pltpu.VMEM((H, L), F32),
            pltpu.SemaphoreType.DMA((n_chunks,)),
            pltpu.SemaphoreType.DMA((n_chunks,)),
            pltpu.SemaphoreType.DMA((1,)),
            pltpu.SemaphoreType.DMA((4,)),
        ],
        compiler_params=pltpu.CompilerParams(
            vmem_limit_bytes=110 * 1024 * 1024,
            disable_bounds_checks=True,
            disable_semaphore_checks=True,
        ),
    )(xt, g, b, w)
    return jnp.transpose(out, (2, 0, 1))


@jax.jit
def pallas_standalone__layernorm_linear__sampling_kernel(
    x: jax.Array,
    g: jax.Array,
    b: jax.Array,
    w: jax.Array,
):
    return _forward(CONFIG, x, g, b, w)
```
